```python
import jax
import jax.numpy as jnp

def _softmax(x, axis=-1):
    return jax.nn.softmax(x, axis=axis)

def _gelu(x):
    return jax.nn.gelu(x, approximate=True)

def _silu(x):
    return jax.nn.silu(x)

def _sigmoid(x):
    return jax.nn.sigmoid(x)

def _layernorm(x, axis=-1, eps=1e-05):
    m = jnp.mean(x, axis=axis, keepdims=True)
    v = jnp.var(x, axis=axis, keepdims=True)
    return (x - m) / jnp.sqrt(v + eps)

def _scatter_add(tgt, idx, src, axis=0):
    return tgt.at[idx].add(src)

def _segment_sum(src, seg, n):
    return jax.ops.segment_sum(src, seg, n)

class _Rng:

    def __init__(self, key):
        self._k = key

    def _next(self):
        self._k, sub = jax.random.split(self._k)
        return sub

    def normal(self, shape):
        return jax.random.normal(self._next(), shape, dtype=jnp.bfloat16)

    def randint(self, lo, hi, shape):
        return jax.random.randint(self._next(), shape, lo, hi, dtype=jnp.int32)

    def uniform(self, shape, lo=0.0, hi=1.0):
        return jax.random.uniform(self._next(), shape, jnp.bfloat16, lo, hi)

    def permutation(self, n):
        return jax.random.permutation(self._next(), n)
kernel_name = 'gated_mix__memory_aug_recurrent_mem_tr__spectral_gfnet__prompt'

def setup_inputs():
    _rng = _Rng(jax.random.key(int.from_bytes(__import__("os").urandom(4), "little")))
    _w = lambda a: (lambda t: t.astype(jnp.bfloat16) if jnp.issubdtype(t.dtype, jnp.floating) else t)(jnp.asarray(a))

    def _A_setup():
        B, S, Dm = (1, 2048, 1024)
        H, Dh = (32, 128)
        M, seg = (8, 32)
        seg = min(seg, S)
        S = S // seg * seg
        return {'x': _w((lambda *s: _rng.normal(s) * 0.05)(B, S, Dm)), 'mem0': _w((lambda *s: _rng.normal(s) * 0.05)(B, M, Dm)), 'Wq': _w((lambda *s: _rng.normal(s) * 0.05)(Dm, H, Dh) * Dm ** (-0.5)), 'Wk': _w((lambda *s: _rng.normal(s) * 0.05)(Dm, H, Dh) * Dm ** (-0.5)), 'Wv': _w((lambda *s: _rng.normal(s) * 0.05)(Dm, H, Dh) * Dm ** (-0.5)), 'Wo': _w((lambda *s: _rng.normal(s) * 0.05)(H, Dh, Dm) * (H * Dh) ** (-0.5)), 'seg_len': seg}
    _A_in = _A_setup()

    def _B_setup():
        B, S, D = (1, 2048, 1024)
        Df = D // 2 + 1
        return {'x': _w((lambda *s: _rng.normal(s) * 0.05)(B, S, D)), 'w_r': _w((lambda *s: _rng.normal(s) * 0.05)(S, Df) * 0.02), 'w_i': _w((lambda *s: _rng.normal(s) * 0.05)(S, Df) * 0.02)}
    _B_in = _B_setup()
    return {'A_x': _A_in['x'], 'A_mem0': _A_in['mem0'], 'A_Wq': _A_in['Wq'], 'A_Wk': _A_in['Wk'], 'A_Wv': _A_in['Wv'], 'A_Wo': _A_in['Wo'], 'A_seg_len': _A_in['seg_len'], 'B_x': _B_in['x'], 'B_w_r': _B_in['w_r'], 'B_w_i': _B_in['w_i'], 'gate_w': _w((lambda *s: _rng.normal(s) * 0.05)(1024))}

def reference(A_x, A_mem0, A_Wq, A_Wk, A_Wv, A_Wo, A_seg_len, B_x, B_w_r, B_w_i, gate_w):

    def _A_ref(x, mem0, Wq, Wk, Wv, Wo, seg_len):
        B, S, Dm = x.shape
        H, Dh = (Wq.shape[1], Wq.shape[2])
        M = mem0.shape[1]
        scale = Dh ** (-0.5)
        n_seg = S // seg_len
        L = M + seg_len
        idx = jnp.arange(L)
        mask = (idx[:, None] < M) | (idx[:, None] >= idx[None, :])
        mem = mem0
        outs = []
        for s in range(n_seg):
            xs = x[:, s * seg_len:(s + 1) * seg_len, :].copy()
            h = jnp.concatenate([mem, xs], axis=1)
            q = jnp.einsum('btd,dhe->bhte', h, Wq)
            k = jnp.einsum('btd,dhe->bhte', h, Wk)
            v = jnp.einsum('btd,dhe->bhte', h, Wv)
            scores = jnp.einsum('bhqe,bhke->bhqk', q, k) * scale
            scores = jnp.where(mask[None, None], scores, -1000000000.0)
            p = _softmax(scores, axis=-1)
            o = jnp.einsum('bhqk,bhke->bhqe', p, v)
            o = jnp.einsum('bhte,hed->btd', o, Wo)
            mem = o[:, :M, :].copy()
            outs.append(o[:, M:, :])
        return jnp.concatenate(outs, axis=1)

    def _B_ref(x, w_r, w_i):
        B, S, D = x.shape
        X = (lambda x, axes=(-2, -1): jnp.fft.rfft2(x.astype(jnp.float32), axes=axes))(x, axes=(-2, -1))
        W = w_r + 1j * w_i
        X = X * W
        y = (lambda x, s, axes=(-2, -1): jnp.fft.irfft2(x, s=s, axes=axes).astype(jnp.bfloat16))(X, (S, D), axes=(-2, -1))
        return y
    x = A_x
    g = _sigmoid((x * gate_w).sum(-1, keepdims=True))
    a = _A_ref(x, A_mem0, A_Wq, A_Wk, A_Wv, A_Wo, A_seg_len)
    b = _B_ref(x, B_w_r, B_w_i)
    return g * a + (1 - g) * b
```

```python
import functools

import numpy as np
import ml_dtypes

import jax
import jax.numpy as jnp
import jax.experimental.pallas as pl
import jax.experimental.pallas.tpu as pltpu

S_LEN, DM, H, DH, M, SEG = 2048, 1024, 32, 128, 8, 32
L = M + SEG
NSEG = S_LEN // SEG
DF = DM // 2 + 1
f32 = jnp.float32
bf16 = jnp.bfloat16
u32 = jnp.uint32


def _bf16_np(a):
    return np.asarray(a, np.float32).astype(ml_dtypes.bfloat16)


def _pack_rows_u32(a):
    b = _bf16_np(a).view(np.uint16).astype(np.uint32)
    return b[0::2] | (b[1::2] << 16)


def _real_block(mc):
    mr, mi = mc.real, mc.imag
    return np.block([[mr, -mi], [mi, mr]])


def _make_consts():
    d = np.arange(DM)[:, None].astype(np.float64)
    k = np.arange(DM // 2)[None, :].astype(np.float64)
    ang = 2.0 * np.pi * ((d * k) % DM) / DM
    fr = np.cos(ang)
    fi = -np.sin(ang)
    fi[:, 0] = np.cos(np.pi * d[:, 0])
    fmat = np.concatenate([fr, fi], axis=1)
    gmat = fmat.T.copy()

    i16 = np.arange(16)
    w16 = np.exp(-2j * np.pi * np.outer(i16, i16) / 16.0)
    eye8 = np.eye(8)
    a_fwd = _real_block(np.kron(w16, eye8))
    a_inv = _real_block(np.kron(np.conj(w16), eye8))
    s1 = np.arange(128)
    k1 = np.arange(128)
    b_fwd, b_inv = [], []
    for k2 in range(16):
        ph = (s1[None, :] * (k2 + 16 * k1[:, None])) % 2048
        mk = np.exp(-2j * np.pi * ph / 2048.0)
        b_fwd.append(_real_block(mk))
        b_inv.append(_real_block(np.conj(mk).T))
    return (_pack_rows_u32(fmat), _pack_rows_u32(gmat),
            _bf16_np(a_fwd), _bf16_np(a_inv),
            _bf16_np(np.stack(b_fwd)), _bf16_np(np.stack(b_inv)))


_FMAT, _GMAT, _AFWD, _AINV, _BFWD, _BINV = _make_consts()

NCH = 8
CH_ROWS = DM * H // NCH


def _kernel(x_hbm, mem_ref, wq_hbm, wk_hbm, wv_hbm, wo_hbm, wr_hbm, wi_hbm, gw_ref,
            f_hbm, g_hbm, afwd_ref, ainv_ref, bfwd_hbm, binv_hbm,
            out_hbm,
            x_v, f_v, g_v, bfwd_v, binv_v, wr_v, wi_v, wrn_v, win_v, stage, wqkv, wo_v, z1, z2, o_scr, out_v,
            sem_in, sem_wf, sem_w, sem_wo, sem_out):
    w_hbm = (wq_hbm, wk_hbm, wv_hbm)

    cp_x = pltpu.make_async_copy(x_hbm, x_v, sem_in.at[0])
    cp_f = pltpu.make_async_copy(f_hbm, f_v, sem_in.at[1])
    cp_bf = pltpu.make_async_copy(bfwd_hbm, bfwd_v, sem_in.at[2])
    cp_bi = pltpu.make_async_copy(binv_hbm, binv_v, sem_in.at[3])
    cp_g = pltpu.make_async_copy(g_hbm, g_v, sem_in.at[4])
    cp_wf = []
    for i, (src, dst, dstn) in enumerate(((wr_hbm, wr_v, wrn_v), (wi_hbm, wi_v, win_v))):
        for n in range(4):
            cp_wf.append(pltpu.make_async_copy(src.at[:, pl.ds(n * 128, 128)], dst.at[n], sem_wf.at[i * 5 + n]))
        cp_wf.append(pltpu.make_async_copy(src.at[:, pl.ds(512, 1)], dstn, sem_wf.at[i * 5 + 4]))

    def cp_w(which, c):
        return pltpu.make_async_copy(
            w_hbm[which].at[pl.ds(c * CH_ROWS, CH_ROWS)],
            stage.at[which, c],
            sem_w.at[which * NCH + c])

    def cp_wo(n):
        return pltpu.make_async_copy(wo_hbm.at[:, pl.ds(n * 128, 128)], wo_v.at[n], sem_wo.at[n])

    cp_x.start()
    cp_f.start()
    for c in range(NCH):
        for which in range(3):
            cp_w(which, c).start()
        if c == 3:
            cp_bf.start()
            for cp in cp_wf:
                cp.start()
            cp_bi.start()
    for n in range(8):
        cp_wo(n).start()
    cp_g.start()

    cp_x.wait()
    cp_f.wait()
    stage32 = stage.bitcast(u32)
    lane0 = jax.lax.broadcasted_iota(jnp.int32, (256, 128), 1) == 0

    def pro1(c, carry):
        xb = x_v[pl.ds(pl.multiple_of(c * 256, 256), 256), :]
        y = jnp.dot(xb, pltpu.bitcast(f_v[...], bf16), preferred_element_type=f32)
        yi0 = y[:, 512:640]
        zr = jnp.concatenate([y[:, :512], jnp.where(lane0, yi0, 0.0)], axis=1)
        zi = jnp.concatenate([jnp.where(lane0, 0.0, yi0), y[:, 640:], jnp.zeros((256, 128), f32)], axis=1)
        z1[0, pl.ds(2 * c, 2)] = zr.reshape(2, 16, 8, 640)
        z1[1, pl.ds(2 * c, 2)] = zi.reshape(2, 16, 8, 640)
        for which in range(3):
            cp_w(which, c).wait()
        for which in range(3):
            for m in range(8):
                for p in range(16):
                    base = m * 256 + p
                    a = stage32[which, c, pl.ds(base, 8, stride=32), :]
                    b = stage32[which, c, pl.ds(base + 16, 8, stride=32), :]
                    lo = (a & jnp.uint32(0xFFFF)) | (b << 16)
                    hi = (a >> 16) | (b & jnp.uint32(0xFFFF0000))
                    r0 = pl.multiple_of(c * 64 + m * 8, 8)
                    wqkv[(2 * p) * 3 + which, pl.ds(r0, 8), :] = lo
                    wqkv[(2 * p + 1) * 3 + which, pl.ds(r0, 8), :] = hi
        return carry

    jax.lax.fori_loop(0, NCH, pro1, 0)

    def stage_a(hi, carry):
        z = z1[:, :, hi].reshape(256, 640).astype(bf16)
        o = jnp.dot(afwd_ref[...], z, preferred_element_type=f32)
        z2[:, :, hi] = o.reshape(2, 16, 8, 640)
        return carry

    jax.lax.fori_loop(0, 16, stage_a, 0)

    cp_bf.wait()
    cp_bi.wait()
    for cp in cp_wf:
        cp.wait()
    wr_v[4] = jnp.broadcast_to(wrn_v[...], (S_LEN, 128))
    wi_v[4] = jnp.broadcast_to(win_v[...], (S_LEN, 128))
    wr32 = wr_v.bitcast(u32)
    wi32 = wi_v.bitcast(u32)
    lane = jax.lax.broadcasted_iota(jnp.int32, (128, 640), 1)
    cscale = jnp.where((lane == 0) | (lane >= 512), 1.0, 2.0).astype(f32) * (1.0 / (S_LEN * DM))

    def unpack(w32, odd):
        if odd:
            return pltpu.bitcast(w32 & jnp.uint32(0xFFFF0000), f32)
        return pltpu.bitcast(w32 << 16, f32)

    def stage_b(q):
        wr_a = jnp.concatenate([wr32[n, pl.ds(q, 128, stride=8), :] for n in range(5)], axis=1)
        wi_a = jnp.concatenate([wi32[n, pl.ds(q, 128, stride=8), :] for n in range(5)], axis=1)
        for odd in range(2):
            k2 = 2 * q + odd
            z = z2[:, k2].reshape(256, 640).astype(bf16)
            xf = jnp.dot(bfwd_v[k2], z, preferred_element_type=f32)
            xr, xi = xf[:128], xf[128:]
            wr = unpack(wr_a, odd) * cscale
            wi = unpack(wi_a, odd) * cscale
            pr = xr * wr - xi * wi
            pi = xr * wi + xi * wr
            pc = jnp.concatenate([pr, pi], axis=0).astype(bf16)
            gk = jnp.dot(binv_v[k2], pc, preferred_element_type=f32)
            z1[:, k2] = gk.reshape(2, 16, 8, 640)

    for q in range(8):
        stage_b(q)

    lane0a = jax.lax.broadcasted_iota(jnp.int32, (128, 128), 1) == 0

    def stage_a_inv(hi, carry):
        z = z1[:, :, hi].reshape(256, 640).astype(bf16)
        o = jnp.dot(ainv_ref[...], z, preferred_element_type=f32)
        ur = o[:128, :512]
        ui = jnp.concatenate([jnp.where(lane0a, o[:128, 512:640], o[128:, 0:128]), o[128:, 128:512]], axis=1)
        z2[0, :, hi, :, 0:512] = ur.reshape(16, 8, 512)
        z2[1, :, hi, :, 0:512] = ui.reshape(16, 8, 512)
        return carry

    jax.lax.fori_loop(0, 16, stage_a_inv, 0)

    for n in range(8):
        cp_wo(n).wait()
    cp_g.wait()

    scale = DH ** -0.5
    rows = jax.lax.broadcasted_iota(jnp.int32, (L, L), 0)
    cols = jax.lax.broadcasted_iota(jnp.int32, (L, L), 1)
    mask = (rows < M) | (rows >= cols)
    wo32 = wo_v.bitcast(u32)

    def qkv_head(h, hd):
        return tuple(jnp.dot(h, pltpu.bitcast(wqkv[3 * hd + j], bf16), preferred_element_type=f32)
                     for j in range(3))

    def scores(qkv):
        return jax.lax.dot_general(qkv[0], qkv[1].astype(bf16), (((1,), (1,)), ((), ())),
                                   preferred_element_type=f32)

    def softmax(s):
        s = jnp.where(mask, s * scale, -1e9)
        m = jnp.max(s, axis=-1, keepdims=True)
        p = jnp.exp(s - m)
        l = jnp.sum(p, axis=-1, keepdims=True)
        return p / l

    def pv(p, qkv):
        return jnp.dot(p, qkv[2].astype(bf16), preferred_element_type=f32)

    def cp_out(s):
        r0 = pl.multiple_of(s * SEG, SEG)
        return pltpu.make_async_copy(out_v.at[pl.ds(r0, SEG)], out_hbm.at[pl.ds(r0, SEG)], sem_out)

    def step(s, mem):
        r0 = pl.multiple_of(s * SEG, SEG)
        xs = x_v[pl.ds(r0, SEG), :].astype(f32)
        h = jnp.concatenate([mem, xs], axis=0)
        qkvs, sc, ps = {}, {}, {}
        for i in range(3):
            qkvs[i] = qkv_head(h, i)
        sc[0] = scores(qkvs[0])
        sc[1] = scores(qkvs[1])
        ps[0] = softmax(sc.pop(0))
        for hd in range(H):
            if hd + 3 < H:
                qkvs[hd + 3] = qkv_head(h, hd + 3)
            if hd + 2 < H:
                sc[hd + 2] = scores(qkvs[hd + 2])
            if hd + 1 < H:
                ps[hd + 1] = softmax(sc.pop(hd + 1))
            o_scr[:, hd * DH:(hd + 1) * DH] = pv(ps.pop(hd), qkvs.pop(hd))
        s2 = s // 4
        hi0 = (s % 4) * 4
        ur = z2[0, s2, pl.ds(hi0, 4), :, 0:512].reshape(SEG, 512)
        ui = z2[1, s2, pl.ds(hi0, 4), :, 0:512].reshape(SEG, 512)
        u = jnp.concatenate([ur, ui], axis=1)
        b = jnp.dot(u, pltpu.bitcast(g_v[...], bf16), preferred_element_type=f32)
        gate = jax.nn.sigmoid(jnp.sum(xs * gw_ref[...].astype(f32), axis=-1, keepdims=True))
        oall = o_scr[...]
        out = jnp.concatenate(
            [jnp.dot(oall, pltpu.bitcast(wo32[n], bf16), preferred_element_type=f32) for n in range(8)], axis=1)
        res = gate * out[M:] + (1.0 - gate) * b
        out_v[pl.ds(r0, SEG), :] = res.astype(out_v.dtype)
        cp_out(s).start()
        return out[:M].astype(bf16).astype(f32)

    jax.lax.fori_loop(0, NSEG, step, mem_ref[...].astype(f32))
    pltpu.make_async_copy(out_v, out_hbm, sem_out).wait()


@jax.jit
def _run(A_x, A_mem0, A_Wq, A_Wk, A_Wv, A_Wo, B_w_r, B_w_i, gate_w):
    any_spec = pl.BlockSpec(memory_space=pl.ANY)
    vm = lambda shape: pl.BlockSpec(shape, lambda: (0,) * len(shape))
    out = pl.pallas_call(
        _kernel,
        out_shape=jax.ShapeDtypeStruct((S_LEN, DM), A_x.dtype),
        in_specs=[any_spec, vm((M, DM)), any_spec, any_spec, any_spec, any_spec, any_spec, any_spec,
                  vm((1, DM)), any_spec, any_spec, vm((256, 256)), vm((256, 256)), any_spec, any_spec],
        out_specs=any_spec,
        scratch_shapes=[
            pltpu.VMEM((S_LEN, DM), bf16),
            pltpu.VMEM((DM // 2, DM), u32),
            pltpu.VMEM((DM // 2, DM), u32),
            pltpu.VMEM((16, 256, 256), bf16),
            pltpu.VMEM((16, 256, 256), bf16),
            pltpu.VMEM((5, S_LEN, 128), bf16),
            pltpu.VMEM((5, S_LEN, 128), bf16),
            pltpu.VMEM((S_LEN, 1), bf16),
            pltpu.VMEM((S_LEN, 1), bf16),
            pltpu.VMEM((3, NCH, CH_ROWS, DH), bf16),
            pltpu.VMEM((3 * H, DM // 2, DH), u32),
            pltpu.VMEM((8, H * DH, 128), bf16),
            pltpu.VMEM((2, 16, 16, 8, 640), f32),
            pltpu.VMEM((2, 16, 16, 8, 640), f32),
            pltpu.VMEM((L, H * DH), f32),
            pltpu.VMEM((S_LEN, DM), bf16),
            pltpu.SemaphoreType.DMA((5,)),
            pltpu.SemaphoreType.DMA((10,)),
            pltpu.SemaphoreType.DMA((3 * NCH,)),
            pltpu.SemaphoreType.DMA((8,)),
            pltpu.SemaphoreType.DMA(()),
        ],
        compiler_params=pltpu.CompilerParams(vmem_limit_bytes=124 * 1024 * 1024),
    )(A_x.reshape(S_LEN, DM), A_mem0.reshape(M, DM),
      A_Wq.reshape(DM * H, DH), A_Wk.reshape(DM * H, DH), A_Wv.reshape(DM * H, DH),
      A_Wo.reshape(H * DH, DM), B_w_r, B_w_i, gate_w.reshape(1, DM),
      _FMAT, _GMAT, _AFWD, _AINV, _BFWD, _BINV)
    return out.reshape(A_x.shape)


def pallas_gated_mix__memory_aug_recurrent_mem_tr__spectral_gfnet__prompt_kernel(
    A_x: jax.Array,
    A_mem0: jax.Array,
    A_Wq: jax.Array,
    A_Wk: jax.Array,
    A_Wv: jax.Array,
    A_Wo: jax.Array,
    A_seg_len: int,
    B_x: jax.Array,
    B_w_r: jax.Array,
    B_w_i: jax.Array,
    gate_w: jax.Array,
):
    del B_x
    assert int(A_seg_len) == SEG and A_x.shape == (1, S_LEN, DM)
    return _run(A_x, A_mem0, A_Wq, A_Wk, A_Wv, A_Wo, B_w_r, B_w_i, gate_w)
```

```python
import functools
import contextlib
import numpy as np
import ml_dtypes

import jax
import jax.numpy as jnp
import jax.experimental.pallas as pl
import jax.experimental.pallas.tpu as pltpu

S_LEN, DM, H, DH, M, SEG = 2048, 1024, 32, 128, 8, 32
L = M + SEG
NSEG = S_LEN // SEG
DF = DM // 2 + 1
f32 = jnp.float32
bf16 = jnp.bfloat16
u32 = jnp.uint32
NSTEP = 64
SCOPES = 0
UNROLL = 2
FENCE = 0


def scope(n):
    return jax.named_scope(n) if SCOPES else contextlib.nullcontext()


def _bf16_np(a):
    return np.asarray(a, np.float32).astype(ml_dtypes.bfloat16)


def _pack_rows_u32(a):
    b = _bf16_np(a).view(np.uint16).astype(np.uint32)
    return b[0::2] | (b[1::2] << 16)


def _make_consts():
    half = DM // 2
    i = np.arange(half)
    ang = 2.0 * np.pi * ((np.outer(i, i)) % DM) / DM
    ce = np.cos(ang)
    so = -np.sin(ang)
    cs = np.stack([_pack_rows_u32(ce), _pack_rows_u32(so)])
    cs = np.ascontiguousarray(cs.reshape(2, 256, 4, 128).transpose(0, 2, 1, 3)).reshape(8, 256, 128)

    i16 = np.arange(16)
    i128 = np.arange(128)
    d128 = np.exp(-2j * np.pi * ((np.outer(i128, i128)) % 128) / 128.0)
    dc = np.conj(d128)
    small = np.stack([d128.real, d128.imag, dc.real + dc.imag, dc.imag - dc.real]).astype(np.float32)
    tw_f = np.exp(-2j * np.pi * np.outer(i16, i128) / 2048.0)
    tw = np.concatenate([tw_f.real, tw_f.imag]).astype(np.float32)
    twb = np.exp(2j * np.pi * np.outer(i16, np.arange(8)) / 2048.0)
    twb = np.stack([twb.real, twb.imag]).astype(np.float32)
    twb = np.ascontiguousarray(np.broadcast_to(twb[..., None], twb.shape + (128,)))
    tws = np.exp(2j * np.pi * 8 * np.outer(i16, i16) / 2048.0)
    tws = np.concatenate([tws.real.reshape(-1), tws.imag.reshape(-1)]).astype(np.float32)
    perm = np.zeros((128, 128), np.float32)
    for k2 in range(16):
        for lo in range(8):
            perm[k2 * 8 + lo, k2 + 16 * lo] = 1.0
    rev = np.zeros((128, 128), np.float32)
    for p in range(1, 128):
        rev[128 - p, p] = 1.0
    return cs, twb, tws, small, tw, np.stack([perm, rev])


_CS, _TWB, _TWS, _SMALL, _TW, _PERM = _make_consts()
NU = 16


def _cmul_const(x, c):
    re, im = x
    cr, ci = float(np.real(c)), float(np.imag(c))
    if abs(ci) < 1e-9:
        return (re, im) if cr > 0 else (-re, -im)
    if abs(cr) < 1e-9:
        return (-im, re) if ci > 0 else (im, -re)
    if abs(abs(cr) - abs(ci)) < 1e-9:
        a = abs(cr)
        sr, si = (1.0 if cr > 0 else -1.0), (1.0 if ci > 0 else -1.0)
        nr = (re if sr > 0 else -re) - (im if si > 0 else -im)
        ni = (re if si > 0 else -re) + (im if sr > 0 else -im)
        return (nr * a, ni * a)
    return (re * cr - im * ci, re * ci + im * cr)


def _dft4(x, sign):
    (ar, ai), (br, bi), (cr, ci), (dr, di) = x
    s0r, s0i = ar + cr, ai + ci
    s1r, s1i = ar - cr, ai - ci
    s2r, s2i = br + dr, bi + di
    s3r, s3i = br - dr, bi - di
    if sign < 0:
        return [(s0r + s2r, s0i + s2i), (s1r + s3i, s1i - s3r), (s0r - s2r, s0i - s2i), (s1r - s3i, s1i + s3r)]
    return [(s0r + s2r, s0i + s2i), (s1r - s3i, s1i + s3r), (s0r - s2r, s0i - s2i), (s1r + s3i, s1i - s3r)]


def _dft16(x, sign):
    w = np.exp(sign * 2j * np.pi / 16.0)
    t = [[None] * 4 for _ in range(4)]
    for b in range(4):
        col = _dft4([x[4 * a + b] for a in range(4)], sign)
        for c in range(4):
            t[b][c] = col[c] if b * c == 0 else _cmul_const(col[c], w ** (b * c))
    out = [None] * 16
    for c in range(4):
        row = _dft4([t[b][c] for b in range(4)], sign)
        for d in range(4):
            out[c + 4 * d] = row[d]
    return out


def _kernel(x_hbm, mem_ref, wq_hbm, wk_hbm, wv_hbm, wo_hbm, wr_hbm, wi_hbm, gw_ref,
            cs_hbm, twb_ref, tws_ref, small_ref, tw_ref, perm_ref,
            out_hbm,
            x_v, cs_v, wrt_v, wit_v, wp_v, wqkv, wo_v, z1, z2, u0, u1, n_scr, up_scr, wa_scr, a_scr, out_v,
            sem_x, sem_c, sem_in, sem_w, sem_wo, sem_out, sem_fence):
    w32_hbm = tuple(w.bitcast(u32) for w in (wq_hbm, wk_hbm, wv_hbm))
    nt_dims = (((1,), (1,)), ((), ()))

    def cp_x(i):
        r0 = pl.multiple_of(i * 256, 256)
        return pltpu.make_async_copy(x_hbm.at[pl.ds(r0, 256)], x_v.at[pl.ds(r0, 256)], sem_x.at[i])

    cp_cs = pltpu.make_async_copy(cs_hbm, cs_v, sem_c)
    cp_wr = pltpu.make_async_copy(wr_hbm, wrt_v, sem_in.at[0])
    cp_wi = pltpu.make_async_copy(wi_hbm, wit_v, sem_in.at[1])

    def cp_wo(n):
        return pltpu.make_async_copy(wo_hbm.at[:, pl.ds(n * 128, 128)], wo_v.at[n], sem_wo.at[n])

    def cp_w(p, par, which):
        t = 2 * p + par
        return pltpu.make_async_copy(w32_hbm[which].at[:, par * 16 + p], wqkv.at[3 * t + which],
                                     sem_w.at[3 * t + which])

    def unit_start(p):
        for par in range(2):
            for which in range(3):
                cp_w(p, par, which).start()

    def unit_repack(p, rr=range(0, 512, 64), wait=True):
        if wait:
            for par in range(2):
                for which in range(3):
                    cp_w(p, par, which).wait()
        for which in range(3):
            ta = 6 * p + which
            tb = 6 * p + 3 + which
            for r in rr:
                a = wqkv[ta, r:r + 64, :]
                b = wqkv[tb, r:r + 64, :]
                wqkv[ta, r:r + 64, :] = (a & jnp.uint32(0xFFFF)) | (b << 16)
                wqkv[tb, r:r + 64, :] = (a >> 16) | (b & jnp.uint32(0xFFFF0000))

    def half_dft(e, o):
        pe = [jnp.dot(e, pltpu.bitcast(cs_v[nt], bf16), preferred_element_type=f32) for nt in range(4)]
        po = [jnp.dot(o, pltpu.bitcast(cs_v[4 + nt], bf16), preferred_element_type=f32) for nt in range(4)]
        return pe, po

    def reverse_tiles(t, lane0, first):
        return [jnp.where(lane0, first[T], jnp.dot(t[3 - T], perm_ref[1], preferred_element_type=f32))
                for T in range(4)]

    cp_cs.start()
    cp_x(0).start()
    cp_x(1).start()

    lane_i = jax.lax.broadcasted_iota(jnp.int32, (1, 128), 1)
    lane0 = lane_i == 0
    sgn = (1 - 2 * (lane_i & 1)).astype(f32)

    def pro1(c, first):
        @pl.when(c + 2 < 8)
        def _():
            cp_x(c + 2).start()

        @pl.when(c == 2)
        def _():
            cp_wr.start()
            cp_wi.start()

        @pl.when(c >= 5)
        def _():
            unit_start(c - 5)

        cp_x(c).wait()
        if first:
            cp_cs.wait()
        r0 = pl.multiple_of(c * 256, 256)
        xt = [x_v[pl.ds(r0, 256), j * 128:(j + 1) * 128].astype(f32) for j in range(8)]
        zero = jnp.zeros((256, 128), f32)
        rev = reverse_tiles(xt[4:], lane0, [zero, xt[7], xt[6], xt[5]])
        e = jnp.concatenate([xt[T] + rev[T] for T in range(4)], axis=1)
        o = jnp.concatenate([xt[T] - rev[T] for T in range(4)], axis=1)
        mid = jnp.broadcast_to(xt[4][:, 0:1], (256, 128)) * sgn
        pe, po = half_dft(e, o)
        alt = (((xt[0] + xt[1]) + (xt[2] + xt[3])) + ((xt[4] + xt[5]) + (xt[6] + xt[7]))) * sgn
        nyq = jnp.sum(alt, axis=1, keepdims=True)
        for t in range(4):
            sl = slice(t * 128, (t + 1) * 128)
            z1[0, pl.ds(2 * c, 2), :, :, sl] = (pe[t] + mid).reshape(2, 16, 8, 128)
            z1[1, pl.ds(2 * c, 2), :, :, sl] = po[t].reshape(2, 16, 8, 128)
        z1[0, pl.ds(2 * c, 2), :, :, 512:640] = jnp.where(lane0, nyq, 0.0).reshape(2, 16, 8, 128)
        z1[1, pl.ds(2 * c, 2), :, :, 512:640] = jnp.zeros((2, 16, 8, 128), f32)

    with scope("s_pro1"):
        pro1(0, True)
        jax.lax.fori_loop(1, 8, lambda c, carry: (pro1(c, False), carry)[1], 0)

    def stage_a(hi):
        for t in range(5):
            sl = slice(t * 128, (t + 1) * 128)
            xin = [(z1[0, s2, hi, :, sl], z1[1, s2, hi, :, sl]) for s2 in range(16)]
            xo = _dft16(xin, -1)
            for k2 in range(16):
                z2[0, k2, hi, :, sl] = xo[k2][0]
                z2[1, k2, hi, :, sl] = xo[k2][1]

    norm = 1.0 / (S_LEN * DM)
    cscale = [jnp.where(lane0, norm, 2.0 * norm).astype(f32)] + [2.0 * norm] * 3 + [norm]

    def wperm(c, carry):
        @pl.when(c % 2 == 0)
        def _():
            unit_start(3 + c // 2)

        for bb in range(2):
            blk_i = 2 * c + bb
            l0 = pl.multiple_of(blk_i * 128, 128)
            for i, wt in enumerate((wrt_v, wit_v)):
                for t in range(5):
                    if t < 4:
                        blk = wt[t * 128:(t + 1) * 128, pl.ds(l0, 128)]
                    else:
                        blk = jnp.broadcast_to(wt[512:513, pl.ds(l0, 128)], (128, 128))
                    o = jax.lax.dot_general(perm_ref[0], blk, nt_dims, preferred_element_type=f32)
                    wp_v[i, :, blk_i, :, t * 128:(t + 1) * 128] = (o * cscale[t]).reshape(16, 8, 128)
            stage_a(blk_i)
        return carry

    with scope("s_wperm"):
        cp_wr.wait()
        cp_wi.wait()
        jax.lax.fori_loop(0, 8, wperm, 0)

    def cdot3(m1, m2, m3, zr, zi):
        k1 = jnp.dot(m1, (zr + zi).astype(bf16), preferred_element_type=f32)
        k2 = jnp.dot(m2, zi.astype(bf16), preferred_element_type=f32)
        k3 = jnp.dot(m3, zr.astype(bf16), preferred_element_type=f32)
        return k1 - k2, k1 + k3

    def b_fwd(k2):
        tr, ti = tw_ref[pl.ds(k2, 1), :], tw_ref[pl.ds(16 + k2, 1), :]
        mr = small_ref[0] * tr - small_ref[1] * ti
        mi = small_ref[0] * ti + small_ref[1] * tr
        return cdot3(mr, mr + mi, mi - mr, z2[0, k2].reshape(128, 640), z2[1, k2].reshape(128, 640))

    def b_inv(k2, x):
        xr, xi = x
        wr = wp_v[0, k2].reshape(128, 640)
        wi = wp_v[1, k2].reshape(128, 640)
        pr = xr * wr - xi * wi
        pi = xr * wi + xi * wr
        gr, gi = cdot3(small_ref[0], small_ref[2], small_ref[3], pr, pi)
        z1[0, k2] = gr.reshape(16, 8, 640)
        z1[1, k2] = gi.reshape(16, 8, 640)

    def stage_b2(j, carry):
        @pl.when(j < 6)
        def _():
            unit_start(7 + j)

        xa = b_fwd(2 * j)
        xb = b_fwd(2 * j + 1)
        b_inv(2 * j, xa)
        b_inv(2 * j + 1, xb)
        return carry

    with scope('s_stage_b'):
        jax.lax.fori_loop(0, 8, stage_b2, 0)

    lane0a = jax.lax.broadcasted_iota(jnp.int32, (8, 128), 1) == 0

    def fence():
        if FENCE:
            pl.semaphore_signal(sem_fence, 1)
            pl.semaphore_wait(sem_fence, 1)

    def inv_twiddles(hi):
        tw_inv = [None]
        for k2 in range(1, 16):
            cr, ci = tws_ref[hi * 16 + k2], tws_ref[256 + hi * 16 + k2]
            br, bi = twb_ref[0, k2], twb_ref[1, k2]
            tw_inv.append((br * cr - bi * ci, br * ci + bi * cr))
        return tw_inv

    def a_inv_tile(hi, t, tw_inv, u_dst):
        sl = slice(t * 128, (t + 1) * 128)
        xin = []
        for k2 in range(16):
            gr, gi = z1[0, k2, hi, :, sl], z1[1, k2, hi, :, sl]
            if k2 > 0:
                tr, ti = tw_inv[k2]
                gr, gi = gr * tr - gi * ti, gr * ti + gi * tr
            xin.append((gr, gi))
        xo = _dft16(xin, +1)
        for s2 in range(16):
            u_dst[s2, :, sl] = xo[s2][0]
            if t < 4:
                u_dst[s2, :, 640 + t * 128:640 + (t + 1) * 128] = xo[s2][1]

    def stage_c2(m, carry):
        @pl.when(m < 3)
        def _():
            unit_start(13 + m)

        @pl.when(m >= 4)
        def _():
            cp_wo(2 * m - 8).start()
            cp_wo(2 * m - 7).start()

        stage_c(2 * m, 2 * m + 1, u0, u1)
        stage_c(2 * m + 1, jnp.minimum(2 * m + 2, 15), u1, u0)
        return carry

    def stage_c(hi, nxt, u_src, u_dst):
        tw_inv = inv_twiddles(nxt)
        nyq = u_src[:, :, 512:513].reshape(128, 1)
        n_scr[...] = jnp.broadcast_to(nyq, (128, 128)) * sgn
        for nt in range(4):
            sl = slice(nt * 128, (nt + 1) * 128)
            pe = jnp.dot(u_src[:, :, 0:512].reshape(128, 512), pltpu.bitcast(cs_v[nt], bf16),
                         preferred_element_type=f32)
            a_inv_tile(nxt, nt, tw_inv, u_dst)
            po = jnp.dot(u_src[:, :, 640:1152].reshape(128, 512), pltpu.bitcast(cs_v[4 + nt], bf16),
                         preferred_element_type=f32)
            pe = pe + n_scr[...]
            z2[0, :, hi, :, sl] = (pe + po).reshape(16, 8, 128)
            up_scr[nt] = pe - po
            fence()
            if nt == 0:
                a_inv_tile(nxt, 4, tw_inv, u_dst)
            if nt in (1, 2):
                unit_repack(hi, range(0, 256, 64) if nt == 1 else range(256, 512, 64), wait=(nt == 1))
        ur = [u_src[:, :, t * 128:(t + 1) * 128].reshape(128, 128) for t in range(4)]
        y512 = jnp.sum(((ur[0] + ur[1]) + (ur[2] + ur[3])) * sgn, axis=1, keepdims=True) + nyq
        for t in range(4):
            first = y512 if t == 0 else up_scr[4 - t]
            r = jnp.dot(up_scr[3 - t], perm_ref[1], preferred_element_type=f32)
            z2[1, :, hi, :, t * 128:(t + 1) * 128] = jnp.where(lane0, first, r).reshape(16, 8, 128)

    with scope("s_stage_c"):
        tw0 = inv_twiddles(0)
        for t in range(5):
            a_inv_tile(0, t, tw0, u0)
        jax.lax.fori_loop(0, 8, stage_c2, 0)

    scale = DH ** -0.5
    rows = jax.lax.broadcasted_iota(jnp.int32, (L, L), 0)
    cols = jax.lax.broadcasted_iota(jnp.int32, (L, L), 1)
    mask = (rows < M) | (rows >= cols)
    wo32 = wo_v.bitcast(u32)

    def qkv_head(h, hd):
        return tuple(jnp.dot(h, pltpu.bitcast(wqkv[3 * hd + j], bf16), preferred_element_type=f32)
                     for j in range(3))

    def scores(qkv):
        return jax.lax.dot_general(qkv[0], qkv[1].astype(bf16), nt_dims, preferred_element_type=f32)

    def softmax(s):
        s = jnp.where(mask, s * scale, -1e9)
        m = jnp.max(s, axis=-1, keepdims=True)
        p = jnp.exp(s - m)
        l = jnp.sum(p, axis=-1, keepdims=True)
        return p / l

    def pv(p, qkv):
        return jnp.dot(p, qkv[2].astype(bf16), preferred_element_type=f32)

    def cp_out(seg0, nseg):
        r0 = pl.multiple_of(seg0 * SEG, SEG)
        return pltpu.make_async_copy(out_v.at[pl.ds(r0, nseg * SEG)], out_hbm.at[pl.ds(r0, nseg * SEG)], sem_out)

    def mix(seg):
        r0 = pl.multiple_of(seg * SEG, SEG)
        xs = x_v[pl.ds(r0, SEG), :].astype(f32)
        gate = jax.nn.sigmoid(jnp.sum(xs * gw_ref[...].astype(f32), axis=-1, keepdims=True))
        s2 = seg // 4
        hi0 = (seg % 4) * 4
        b = jnp.concatenate([z2[0, s2, pl.ds(hi0, 4), :, 0:512].reshape(SEG, 512),
                             z2[1, s2, pl.ds(hi0, 4), :, 0:512].reshape(SEG, 512)], axis=1)
        res = gate * a_scr[...] + (1.0 - gate) * b
        out_v[pl.ds(r0, SEG), :] = res.astype(out_v.dtype)

    HA = 28

    def wo_part(h0, h1, n, lhs):
        w = pltpu.bitcast(wo32[n, h0 * (DH // 2):h1 * (DH // 2), :], bf16)
        return jnp.dot(lhs, w, preferred_element_type=f32)

    def step(s, mem, first=False):
        r0 = s * SEG if first else pl.multiple_of(s * SEG, SEG)
        xs = x_v[pl.ds(r0, SEG), :].astype(f32)
        h = jnp.concatenate([mem, xs], axis=0)
        qkvs, sc, ps, oh = {}, {}, {}, {}

        def wo_a(n):
            if first:
                cp_wo(n).wait()
            wa_scr[:, n * 128:(n + 1) * 128] = wo_part(0, HA, n, oa)

        for i in range(3):
            qkvs[i] = qkv_head(h, i)
        sc[0] = scores(qkvs[0])
        sc[1] = scores(qkvs[1])
        ps[0] = softmax(sc.pop(0))
        if not first:
            mix(s - 1)
        for hd in range(H):
            if hd + 3 < H:
                qkvs[hd + 3] = qkv_head(h, hd + 3)
            if hd == HA + 1:
                wo_a(0)
            if hd + 2 < H:
                sc[hd + 2] = scores(qkvs[hd + 2])
            if hd + 1 < H:
                ps[hd + 1] = softmax(sc.pop(hd + 1))
            oh[hd] = pv(ps.pop(hd), qkvs.pop(hd))
            if hd == HA - 1:
                oa = jnp.concatenate([oh.pop(i) for i in range(HA)], axis=1)
            if hd == HA + 1:
                for n in (1, 2, 3):
                    wo_a(n)
            if hd == HA + 2:
                for n in (4, 5):
                    wo_a(n)
        for n in (6, 7):
            wo_a(n)
        ob = jnp.concatenate([oh.pop(i) for i in range(HA, H)], axis=1)
        out = wa_scr[...] + jnp.concatenate([wo_part(HA, H, n, ob) for n in range(8)], axis=1)
        a_scr[...] = out[M:]
        if not first:
            @pl.when(s % 4 == 0)
            def _():
                cp_out(s - 4, 4).start()

        return out[:M].astype(bf16).astype(f32)

    with scope('s_main'):
        mem1 = step(0, mem_ref[...].astype(f32), first=True)
        jax.lax.fori_loop(1, NSTEP, step, mem1, unroll=UNROLL)
    mix(NSTEP - 1)
    last = ((NSTEP - 1) // 4) * 4
    cp_out(last, NSTEP - last).start()
    pltpu.make_async_copy(out_v.at[pl.ds(0, NSTEP * SEG)], out_hbm.at[pl.ds(0, NSTEP * SEG)], sem_out).wait()


@jax.jit
def _run(A_x, A_mem0, A_Wq, A_Wk, A_Wv, A_Wo, B_w_r, B_w_i, gate_w):
    any_spec = pl.BlockSpec(memory_space=pl.ANY)
    vm = lambda shape: pl.BlockSpec(shape, lambda: (0,) * len(shape))
    out = pl.pallas_call(
        _kernel,
        out_shape=jax.ShapeDtypeStruct((S_LEN, DM), A_x.dtype),
        in_specs=[any_spec, vm((M, DM)), any_spec, any_spec, any_spec, any_spec, any_spec, any_spec,
                  vm((1, DM)), any_spec, vm((2, 16, 8, 128)), pl.BlockSpec(memory_space=pltpu.SMEM),
                  vm((4, 128, 128)), vm((32, 128)), vm((2, 128, 128))],
        out_specs=any_spec,
        scratch_shapes=[
            pltpu.VMEM((S_LEN, DM), bf16),
            pltpu.VMEM((8, DM // 4, 128), u32),
            pltpu.VMEM((DF, S_LEN), bf16),
            pltpu.VMEM((DF, S_LEN), bf16),
            pltpu.VMEM((2, 16, 16, 8, 640), f32),
            pltpu.VMEM((3 * H, DM // 2, DH), u32),
            pltpu.VMEM((8, H * DH, 128), bf16),
            pltpu.VMEM((2, 16, 16, 8, 640), f32),
            pltpu.VMEM((2, 16, 16, 8, 640), f32),
            pltpu.VMEM((16, 8, 1152), f32),
            pltpu.VMEM((16, 8, 1152), f32),
            pltpu.VMEM((128, 128), f32),
            pltpu.VMEM((4, 128, 128), f32),
            pltpu.VMEM((L, DM), f32),
            pltpu.VMEM((SEG, DM), f32),
            pltpu.VMEM((S_LEN, DM), bf16),
            pltpu.SemaphoreType.DMA((8,)),
            pltpu.SemaphoreType.DMA(()),
            pltpu.SemaphoreType.DMA((2,)),
            pltpu.SemaphoreType.DMA((3 * H,)),
            pltpu.SemaphoreType.DMA((8,)),
            pltpu.SemaphoreType.DMA(()),
            pltpu.SemaphoreType.REGULAR,
        ],
        compiler_params=pltpu.CompilerParams(vmem_limit_bytes=124 * 1024 * 1024),
    )(A_x.reshape(S_LEN, DM), A_mem0.reshape(M, DM),
      A_Wq.reshape(512, 64, DH), A_Wk.reshape(512, 64, DH), A_Wv.reshape(512, 64, DH),
      A_Wo.reshape(H * DH, DM), B_w_r.T, B_w_i.T, gate_w.reshape(1, DM),
      _CS, _TWB, _TWS, _SMALL, _TW, _PERM)
    return out.reshape(A_x.shape)


def pallas_gated_mix__memory_aug_recurrent_mem_tr__spectral_gfnet__prompt_kernel(
    A_x, A_mem0, A_Wq, A_Wk, A_Wv, A_Wo, A_seg_len, B_x, B_w_r, B_w_i, gate_w,
):
    del B_x
    assert int(A_seg_len) == SEG and A_x.shape == (1, S_LEN, DM)
    return _run(A_x, A_mem0, A_Wq, A_Wk, A_Wv, A_Wo, B_w_r, B_w_i, gate_w)
```

```python
import functools
import contextlib
import numpy as np
import ml_dtypes

import jax
import jax.numpy as jnp
import jax.experimental.pallas as pl
import jax.experimental.pallas.tpu as pltpu

S_LEN, DM, H, DH, M, SEG = 2048, 1024, 32, 128, 8, 32
L = M + SEG
NSEG = S_LEN // SEG
DF = DM // 2 + 1
f32 = jnp.float32
bf16 = jnp.bfloat16
u32 = jnp.uint32
NSTEP = 64
SCOPES = 0
UNROLL = 2
FENCE = 0
WO0 = 2


def scope(n):
    return jax.named_scope(n) if SCOPES else contextlib.nullcontext()


def _bf16_np(a):
    return np.asarray(a, np.float32).astype(ml_dtypes.bfloat16)


def _pack_rows_u32(a):
    b = _bf16_np(a).view(np.uint16).astype(np.uint32)
    return b[0::2] | (b[1::2] << 16)


def _make_consts():
    q = np.arange(DM // 4)
    th = 2.0 * np.pi / DM
    a0 = th * ((2 * np.outer(q, q)) % DM)
    a1 = th * ((np.outer(q, 2 * q + 1)) % DM)
    s1f = -np.sin(a1)
    s1f[0, :] = -np.cos(np.pi * q)
    mperm = 16 * (q // 16) + ((q % 16) >> 1) + 8 * (q & 1)
    fwd = [np.cos(a0), np.cos(a1), -np.sin(a0), s1f]
    inv = [np.cos(a0).T, np.cos(a1).T, -np.sin(a0).T, -np.sin(a1).T]
    mats = [m[:, mperm] for m in fwd] + [m[mperm, :] for m in inv]
    cs = np.stack([_pack_rows_u32(m) for m in mats])
    cs = np.ascontiguousarray(cs.reshape(8, 128, 2, 128).transpose(0, 2, 1, 3)).reshape(16, 128, 128)

    i16 = np.arange(16)
    i128 = np.arange(128)
    d128 = np.exp(-2j * np.pi * ((np.outer(i128, i128)) % 128) / 128.0)
    dc = np.conj(d128)
    small = np.stack([d128.real, d128.imag, dc.real + dc.imag, dc.imag - dc.real]).astype(np.float32)
    tw_f = np.exp(-2j * np.pi * np.outer(i16, i128) / 2048.0)
    tw = np.concatenate([tw_f.real, tw_f.imag]).astype(np.float32)
    twb = np.exp(2j * np.pi * np.outer(i16, np.arange(8)) / 2048.0)
    twb = np.stack([twb.real, twb.imag]).astype(np.float32)
    twb = np.ascontiguousarray(np.broadcast_to(twb[..., None], twb.shape + (128,)))
    tws = np.exp(2j * np.pi * 8 * np.outer(i16, i16) / 2048.0)
    tws = np.concatenate([tws.real.reshape(-1), tws.imag.reshape(-1)]).astype(np.float32)
    perm = np.zeros((128, 128), np.float32)
    for k2 in range(16):
        for lo in range(8):
            perm[k2 * 8 + lo, k2 + 16 * lo] = 1.0
    rev = np.zeros((128, 128), np.float32)
    for p in range(1, 128):
        rev[128 - p, p] = 1.0
    return cs, twb, tws, small, tw, np.stack([perm, rev])


_CS, _TWB, _TWS, _SMALL, _TW, _PERM = _make_consts()
NU = 16


def _cmul_const(x, c):
    re, im = x
    cr, ci = float(np.real(c)), float(np.imag(c))
    if abs(ci) < 1e-9:
        return (re, im) if cr > 0 else (-re, -im)
    if abs(cr) < 1e-9:
        return (-im, re) if ci > 0 else (im, -re)
    if abs(abs(cr) - abs(ci)) < 1e-9:
        a = abs(cr)
        sr, si = (1.0 if cr > 0 else -1.0), (1.0 if ci > 0 else -1.0)
        nr = (re if sr > 0 else -re) - (im if si > 0 else -im)
        ni = (re if si > 0 else -re) + (im if sr > 0 else -im)
        return (nr * a, ni * a)
    return (re * cr - im * ci, re * ci + im * cr)


def _dft4(x, sign):
    (ar, ai), (br, bi), (cr, ci), (dr, di) = x
    s0r, s0i = ar + cr, ai + ci
    s1r, s1i = ar - cr, ai - ci
    s2r, s2i = br + dr, bi + di
    s3r, s3i = br - dr, bi - di
    if sign < 0:
        return [(s0r + s2r, s0i + s2i), (s1r + s3i, s1i - s3r), (s0r - s2r, s0i - s2i), (s1r - s3i, s1i + s3r)]
    return [(s0r + s2r, s0i + s2i), (s1r - s3i, s1i + s3r), (s0r - s2r, s0i - s2i), (s1r + s3i, s1i - s3r)]


def _dft16(x, sign):
    w = np.exp(sign * 2j * np.pi / 16.0)
    t = [[None] * 4 for _ in range(4)]
    for b in range(4):
        col = _dft4([x[4 * a + b] for a in range(4)], sign)
        for c in range(4):
            t[b][c] = col[c] if b * c == 0 else _cmul_const(col[c], w ** (b * c))
    out = [None] * 16
    for c in range(4):
        row = _dft4([t[b][c] for b in range(4)], sign)
        for d in range(4):
            out[c + 4 * d] = row[d]
    return out


def _kernel(x_hbm, mem_ref, wq_hbm, wk_hbm, wv_hbm, wo_hbm, wr_hbm, wi_hbm, gw_ref,
            cs_hbm, twb_ref, tws_ref, small_ref, tw_ref, perm_ref,
            out_hbm,
            x_v, cs_v, wrt_v, wit_v, wrn_v, win_v, wp_v, wqkv, wo_v, z1, z2, u0, u1, bt_scr, up_scr, wa_scr, a_scr, out_v,
            sem_x, sem_c, sem_in, sem_w, sem_wo, sem_out, sem_fence):
    w32_hbm = tuple(w.bitcast(u32) for w in (wq_hbm, wk_hbm, wv_hbm))
    nt_dims = (((1,), (1,)), ((), ()))

    def cp_x(i):
        r0 = pl.multiple_of(i * 256, 256)
        return pltpu.make_async_copy(x_hbm.at[pl.ds(r0, 256)], x_v.at[pl.ds(r0, 256)], sem_x.at[i])

    cp_cs = pltpu.make_async_copy(cs_hbm, cs_v, sem_c)
    cp_wt = []
    for i, (src, dst, dstn) in enumerate(((wr_hbm, wrt_v, wrn_v), (wi_hbm, wit_v, win_v))):
        cp_wt.append(pltpu.make_async_copy(src.at[pl.ds(0, 512)], dst, sem_in.at[2 * i]))
        cp_wt.append(pltpu.make_async_copy(src.at[pl.ds(512, 1)], dstn, sem_in.at[2 * i + 1]))

    def cp_wo(n):
        return pltpu.make_async_copy(wo_hbm.at[:, pl.ds(n * 128, 128)], wo_v.at[n], sem_wo.at[n])

    def cp_w(p, par, which):
        t = 2 * p + par
        return pltpu.make_async_copy(w32_hbm[which].at[:, par * 16 + p], wqkv.at[3 * t + which],
                                     sem_w.at[3 * t + which])

    def unit_start(p):
        for par in range(2):
            for which in range(3):
                cp_w(p, par, which).start()

    def unit_repack(p, rr=range(0, 512, 64), wait=True):
        if wait:
            for par in range(2):
                for which in range(3):
                    cp_w(p, par, which).wait()
        for which in range(3):
            ta = 6 * p + which
            tb = 6 * p + 3 + which
            for r in rr:
                a = wqkv[ta, r:r + 64, :]
                b = wqkv[tb, r:r + 64, :]
                wqkv[ta, r:r + 64, :] = pltpu.bitcast(pltpu.pack_elementwise([a, b], packed_dtype=jnp.uint16), u32)
                wqkv[tb, r:r + 64, :] = pltpu.bitcast(pltpu.pack_elementwise([a >> 16, b >> 16], packed_dtype=jnp.uint16), u32)

    C0, C1, S0, S1F, C0T, C1T, S0T, S1T = range(8)

    def qdot(lhs, mat, nt):
        return jnp.dot(lhs, pltpu.bitcast(cs_v[2 * mat + nt], bf16), preferred_element_type=f32)

    def rev(t, first):
        return jnp.where(lane0, first, jnp.dot(t, perm_ref[1], preferred_element_type=f32))

    cp_cs.start()
    cp_x(0).start()
    cp_x(1).start()

    lane_i = jax.lax.broadcasted_iota(jnp.int32, (1, 128), 1)
    lane0 = lane_i == 0
    sgn = (1 - 2 * (lane_i & 1)).astype(f32)
    sgn_m = (1 - 2 * ((lane_i >> 1) & 1)).astype(f32)

    def pro1(c, first):
        @pl.when(c < 3)
        def _():
            cp_x(2 * c + 2).start()
            cp_x(2 * c + 3).start()

        @pl.when(c == 3)
        def _():
            for cp in cp_wt:
                cp.start()

        @pl.when(c >= 4)
        def _():
            unit_start(c - 4)

        cp_x(c).wait()
        if first:
            cp_cs.wait()
        r0 = pl.multiple_of(c * 256, 256)
        xt = [x_v[pl.ds(r0, 256), j * 128:(j + 1) * 128].astype(f32) for j in range(8)]
        zero = jnp.zeros((256, 128), f32)
        r1 = [rev(xt[7], zero), rev(xt[6], xt[7])]
        r2 = [rev(xt[3], zero), rev(xt[2], xt[3])]
        ee, eo, oe, oo = [], [], [], []
        for T in range(2):
            e1, o1 = xt[T] + r1[T], xt[T] - r1[T]
            e2, o2 = r2[T] + xt[4 + T], r2[T] - xt[4 + T]
            ee.append(e1 + e2)
            eo.append(e1 - e2)
            oe.append(o1 - o2)
            oo.append(o1 + o2)
        oo[0] = jnp.where(lane0, xt[2] - xt[6], oo[0])
        e256 = (xt[2] + xt[6])[:, 0:1]
        mid = jnp.broadcast_to(e256, (256, 128)) * sgn_m
        nyq = jnp.sum((ee[0] + ee[1]) * sgn, axis=1, keepdims=True) + e256
        ee, eo, oe, oo = (jnp.concatenate(v, axis=1) for v in (ee, eo, oe, oo))
        rr = pl.ds(2 * c, 2)
        for t in range(2):
            z1[0, rr, :, :, t * 128:(t + 1) * 128] = (qdot(ee, C0, t) + mid).reshape(2, 16, 8, 128)
            z1[0, rr, :, :, (2 + t) * 128:(3 + t) * 128] = qdot(eo, C1, t).reshape(2, 16, 8, 128)
            z1[1, rr, :, :, t * 128:(t + 1) * 128] = qdot(oe, S0, t).reshape(2, 16, 8, 128)
            z1[1, rr, :, :, (2 + t) * 128:(3 + t) * 128] = qdot(oo, S1F, t).reshape(2, 16, 8, 128)
        z1[0, rr, :, :, 512:640] = jnp.where(lane0, nyq, 0.0).reshape(2, 16, 8, 128)
        z1[1, rr, :, :, 512:640] = jnp.zeros((2, 16, 8, 128), f32)

    with scope("s_pro1"):
        pro1(0, True)
        jax.lax.fori_loop(1, 8, lambda c, carry: (pro1(c, False), carry)[1], 0)

    def stage_a(hi):
        for t in range(5):
            sl = slice(t * 128, (t + 1) * 128)
            xin = [(z1[0, s2, hi, :, sl], z1[1, s2, hi, :, sl]) for s2 in range(16)]
            xo = _dft16(xin, -1)
            for k2 in range(16):
                z2[0, k2, hi, :, sl] = xo[k2][0]
                z2[1, k2, hi, :, sl] = xo[k2][1]

    norm = 1.0 / (S_LEN * DM)
    cscale = [jnp.where(lane0, norm, 2.0 * norm).astype(f32)] + [2.0 * norm] * 3 + [norm]

    def wperm(c, carry):
        @pl.when(c % 3 == 0)
        def _():
            unit_start(6 + c // 3)

        for bb in range(2):
            blk_i = 2 * c + bb
            l0 = pl.multiple_of(blk_i * 128, 128)
            for i, (wt, wn) in enumerate(((wrt_v.bitcast(u32), wrn_v), (wit_v.bitcast(u32), win_v))):
                for t in range(5):
                    if t < 4:
                        w = wt[(t % 2) * 128:(t % 2 + 1) * 128, pl.ds(l0, 128)].reshape(8, 16, 128)
                        if t >= 2:
                            w = w >> 16
                        pk = pltpu.pack_elementwise([w[:, :8, :], w[:, 8:, :]], packed_dtype=jnp.uint16)
                        blk = pltpu.bitcast(pltpu.bitcast(pk, u32).reshape(64, 128), bf16)
                    else:
                        blk = jnp.broadcast_to(wn[:, pl.ds(l0, 128)], (128, 128))
                    o = jax.lax.dot_general(perm_ref[0], blk, nt_dims, preferred_element_type=f32)
                    wp_v[i, :, blk_i, :, t * 128:(t + 1) * 128] = (o * cscale[t]).reshape(16, 8, 128)
        return carry

    def stage_a_loop(hi, carry):
        @pl.when(hi % 8 == 0)
        def _():
            unit_start(4 + hi // 8)

        stage_a(hi)
        return carry

    with scope("s_stage_a"):
        jax.lax.fori_loop(0, 16, stage_a_loop, 0)

    with scope("s_wperm"):
        for cp in cp_wt:
            cp.wait()
        jax.lax.fori_loop(0, 8, wperm, 0)

    def cdot3(m1, m2, m3, zr, zi):
        k1 = jnp.dot(m1, (zr + zi).astype(bf16), preferred_element_type=f32)
        k2 = jnp.dot(m2, zi.astype(bf16), preferred_element_type=f32)
        k3 = jnp.dot(m3, zr.astype(bf16), preferred_element_type=f32)
        return k1 - k2, k1 + k3

    def b_fwd(k2):
        tr, ti = tw_ref[pl.ds(k2, 1), :], tw_ref[pl.ds(16 + k2, 1), :]
        mr = small_ref[0] * tr - small_ref[1] * ti
        mi = small_ref[0] * ti + small_ref[1] * tr
        return cdot3(mr, mr + mi, mi - mr, z2[0, k2].reshape(128, 640), z2[1, k2].reshape(128, 640))

    def b_inv(k2, x):
        xr, xi = x
        wr = wp_v[0, k2].reshape(128, 640)
        wi = wp_v[1, k2].reshape(128, 640)
        pr = xr * wr - xi * wi
        pi = xr * wi + xi * wr
        gr, gi = cdot3(small_ref[0], small_ref[2], small_ref[3], pr, pi)
        z1[0, k2] = gr.reshape(16, 8, 640)
        z1[1, k2] = gi.reshape(16, 8, 640)

    def stage_b2(j, carry):
        @pl.when(j < 7)
        def _():
            unit_start(9 + j)

        xa = b_fwd(2 * j)
        xb = b_fwd(2 * j + 1)
        b_inv(2 * j, xa)
        b_inv(2 * j + 1, xb)
        return carry

    with scope('s_stage_b'):
        jax.lax.fori_loop(0, 8, stage_b2, 0)

    lane0a = jax.lax.broadcasted_iota(jnp.int32, (8, 128), 1) == 0

    def fence():
        if FENCE:
            pl.semaphore_signal(sem_fence, 1)
            pl.semaphore_wait(sem_fence, 1)

    def inv_twiddles(hi):
        tw_inv = [None]
        for k2 in range(1, 16):
            cr, ci = tws_ref[hi * 16 + k2], tws_ref[256 + hi * 16 + k2]
            br, bi = twb_ref[0, k2], twb_ref[1, k2]
            tw_inv.append((br * cr - bi * ci, br * ci + bi * cr))
        return tw_inv

    def a_inv_tile(hi, t, tw_inv, u_dst):
        sl = slice(t * 128, (t + 1) * 128)
        w = np.exp(2j * np.pi / 16.0)
        tmp = bt_scr.at[t % 2]
        for b in range(4):
            xin = []
            for a in range(4):
                k2 = 4 * a + b
                gr, gi = z1[0, k2, hi, :, sl], z1[1, k2, hi, :, sl]
                if k2 > 0:
                    tr, ti = tw_inv[k2]
                    gr, gi = gr * tr - gi * ti, gr * ti + gi * tr
                xin.append((gr, gi))
            col = _dft4(xin, +1)
            for c in range(4):
                v = col[c] if b * c == 0 else _cmul_const(col[c], w ** (b * c))
                tmp[0, b, c] = v[0]
                tmp[1, b, c] = v[1]
        for c in range(4):
            row = _dft4([(tmp[0, b, c], tmp[1, b, c]) for b in range(4)], +1)
            for d in range(4):
                s2 = c + 4 * d
                u_dst[s2, :, sl] = row[d][0]
                if t < 4:
                    u_dst[s2, :, 640 + t * 128:640 + (t + 1) * 128] = row[d][1]

    def stage_c2(m, carry):
        @pl.when(jnp.logical_and(m >= WO0, m < WO0 + 4))
        def _():
            cp_wo(2 * (m - WO0)).start()
            cp_wo(2 * (m - WO0) + 1).start()

        stage_c(2 * m, 2 * m + 1, u0, u1)
        stage_c(2 * m + 1, jnp.minimum(2 * m + 2, 15), u1, u0)
        return carry

    def stage_c(hi, nxt, u_src, u_dst):
        tw_inv = inv_twiddles(nxt)
        unit_repack(hi)
        for t in range(5):
            a_inv_tile(nxt, t, tw_inv, u_dst)
        nyq = u_src[:, :, 512:513].reshape(128, 1)
        n = jnp.broadcast_to(nyq, (128, 128)) * sgn
        ue_r = u_src[:, :, 0:256].reshape(128, 256)
        uo_r = u_src[:, :, 256:512].reshape(128, 256)
        ue_i = u_src[:, :, 640:896].reshape(128, 256)
        uo_i = u_src[:, :, 896:1152].reshape(128, 256)
        for T in range(2):
            a0 = qdot(ue_r, C0T, T) + n
            a1 = qdot(uo_r, C1T, T)
            b0 = qdot(ue_i, S0T, T)
            b1 = qdot(uo_i, S1T, T)
            p, q, pm, qm = a0 + a1, b0 + b1, a0 - a1, b0 - b1
            z2[0, :, hi, :, T * 128:(T + 1) * 128] = (p + q).reshape(16, 8, 128)
            z2[1, :, hi, :, T * 128:(T + 1) * 128] = (pm + qm).reshape(16, 8, 128)
            up_scr[T] = p - q
            up_scr[2 + T] = pm - qm
        s_e = jnp.sum((ue_r[:, :128] + ue_r[:, 128:]) * sgn_m, axis=1, keepdims=True) + nyq
        s_o = jnp.sum((uo_i[:, :128] + uo_i[:, 128:]) * sgn_m, axis=1, keepdims=True)
        z2[1, :, hi, :, 384:512] = rev(up_scr[0], up_scr[1]).reshape(16, 8, 128)
        z2[1, :, hi, :, 256:384] = rev(up_scr[1], s_e + s_o).reshape(16, 8, 128)
        z2[0, :, hi, :, 384:512] = rev(up_scr[2], up_scr[3]).reshape(16, 8, 128)
        z2[0, :, hi, :, 256:384] = rev(up_scr[3], s_e - s_o).reshape(16, 8, 128)

    with scope("s_stage_c"):
        tw0 = inv_twiddles(0)
        for t in range(5):
            a_inv_tile(0, t, tw0, u0)
        jax.lax.fori_loop(0, 8, stage_c2, 0)

    scale = DH ** -0.5
    rows = jax.lax.broadcasted_iota(jnp.int32, (L, L), 0)
    cols = jax.lax.broadcasted_iota(jnp.int32, (L, L), 1)
    mask = (rows < M) | (rows >= cols)
    wo32 = wo_v.bitcast(u32)

    def qkv_head(h, hd):
        return tuple(jnp.dot(h, pltpu.bitcast(wqkv[3 * hd + j], bf16), preferred_element_type=f32)
                     for j in range(3))

    def scores(qkv):
        return jax.lax.dot_general(qkv[0], qkv[1].astype(bf16), nt_dims, preferred_element_type=f32)

    def softmax(s):
        s = jnp.where(mask, s * scale, -1e9)
        m = jnp.max(s, axis=-1, keepdims=True)
        p = jnp.exp(s - m)
        l = jnp.sum(p, axis=-1, keepdims=True)
        return p / l

    def pv(p, qkv):
        return jnp.dot(p, qkv[2].astype(bf16), preferred_element_type=f32)

    def cp_out(seg0, nseg):
        r0 = pl.multiple_of(seg0 * SEG, SEG)
        return pltpu.make_async_copy(out_v.at[pl.ds(r0, nseg * SEG)], out_hbm.at[pl.ds(r0, nseg * SEG)], sem_out)

    def mix(seg):
        r0 = pl.multiple_of(seg * SEG, SEG)
        xs = x_v[pl.ds(r0, SEG), :].astype(f32)
        gate = jax.nn.sigmoid(jnp.sum(xs * gw_ref[...].astype(f32), axis=-1, keepdims=True))
        s2 = seg // 4
        hi0 = (seg % 4) * 4
        b = jnp.concatenate([z2[0, s2, pl.ds(hi0, 4), :, 0:512].reshape(SEG, 512),
                             z2[1, s2, pl.ds(hi0, 4), :, 0:512].reshape(SEG, 512)], axis=1)
        res = gate * a_scr[...] + (1.0 - gate) * b
        out_v[pl.ds(r0, SEG), :] = res.astype(out_v.dtype)

    HA = 28

    def wo_part(h0, h1, n, lhs):
        w = pltpu.bitcast(wo32[n, h0 * (DH // 2):h1 * (DH // 2), :], bf16)
        return jnp.dot(lhs, w, preferred_element_type=f32)

    def step(s, mem, first=False):
        r0 = s * SEG if first else pl.multiple_of(s * SEG, SEG)
        xs = x_v[pl.ds(r0, SEG), :].astype(f32)
        h = jnp.concatenate([mem, xs], axis=0)
        qkvs, sc, ps, oh = {}, {}, {}, {}

        def wo_a(n):
            if first:
                cp_wo(n).wait()
            wa_scr[:, n * 128:(n + 1) * 128] = wo_part(0, HA, n, oa)

        for i in range(3):
            qkvs[i] = qkv_head(h, i)
        sc[0] = scores(qkvs[0])
        sc[1] = scores(qkvs[1])
        ps[0] = softmax(sc.pop(0))
        if not first:
            mix(s - 1)
        for hd in range(H):
            if hd + 3 < H:
                qkvs[hd + 3] = qkv_head(h, hd + 3)
            if hd == HA + 1:
                wo_a(0)
            if hd + 2 < H:
                sc[hd + 2] = scores(qkvs[hd + 2])
            if hd + 1 < H:
                ps[hd + 1] = softmax(sc.pop(hd + 1))
            oh[hd] = pv(ps.pop(hd), qkvs.pop(hd))
            if hd == HA - 1:
                oa = jnp.concatenate([oh.pop(i) for i in range(HA)], axis=1)
            if hd == HA + 1:
                for n in (1, 2, 3):
                    wo_a(n)
            if hd == HA + 2:
                for n in (4, 5):
                    wo_a(n)
        for n in (6, 7):
            wo_a(n)
        ob = jnp.concatenate([oh.pop(i) for i in range(HA, H)], axis=1)
        out = wa_scr[...] + jnp.concatenate([wo_part(HA, H, n, ob) for n in range(8)], axis=1)
        a_scr[...] = out[M:]
        if not first:
            @pl.when(s % 4 == 0)
            def _():
                cp_out(s - 4, 4).start()

        return out[:M].astype(bf16).astype(f32)

    with scope('s_main'):
        mem1 = step(0, mem_ref[...].astype(f32), first=True)
        jax.lax.fori_loop(1, NSTEP, step, mem1, unroll=UNROLL)
    mix(NSTEP - 1)
    last = ((NSTEP - 1) // 4) * 4
    cp_out(last, NSTEP - last).start()
    pltpu.make_async_copy(out_v.at[pl.ds(0, NSTEP * SEG)], out_hbm.at[pl.ds(0, NSTEP * SEG)], sem_out).wait()


@jax.jit
def _run(A_x, A_mem0, A_Wq, A_Wk, A_Wv, A_Wo, B_w_r, B_w_i, gate_w):
    any_spec = pl.BlockSpec(memory_space=pl.ANY)
    vm = lambda shape: pl.BlockSpec(shape, lambda: (0,) * len(shape))
    out = pl.pallas_call(
        _kernel,
        out_shape=jax.ShapeDtypeStruct((S_LEN, DM), A_x.dtype),
        in_specs=[any_spec, vm((M, DM)), any_spec, any_spec, any_spec, any_spec, any_spec, any_spec,
                  vm((1, DM)), any_spec, vm((2, 16, 8, 128)), pl.BlockSpec(memory_space=pltpu.SMEM),
                  vm((4, 128, 128)), vm((32, 128)), vm((2, 128, 128))],
        out_specs=any_spec,
        scratch_shapes=[
            pltpu.VMEM((S_LEN, DM), bf16),
            pltpu.VMEM((16, 128, 128), u32),
            pltpu.VMEM((DM // 2, S_LEN), bf16),
            pltpu.VMEM((DM // 2, S_LEN), bf16),
            pltpu.VMEM((1, S_LEN), bf16),
            pltpu.VMEM((1, S_LEN), bf16),
            pltpu.VMEM((2, 16, 16, 8, 640), f32),
            pltpu.VMEM((3 * H, DM // 2, DH), u32),
            pltpu.VMEM((8, H * DH, 128), bf16),
            pltpu.VMEM((2, 16, 16, 8, 640), f32),
            pltpu.VMEM((2, 16, 16, 8, 640), f32),
            pltpu.VMEM((16, 8, 1152), f32),
            pltpu.VMEM((16, 8, 1152), f32),
            pltpu.VMEM((2, 2, 4, 4, 8, 128), f32),
            pltpu.VMEM((4, 128, 128), f32),
            pltpu.VMEM((L, DM), f32),
            pltpu.VMEM((SEG, DM), f32),
            pltpu.VMEM((S_LEN, DM), bf16),
            pltpu.SemaphoreType.DMA((8,)),
            pltpu.SemaphoreType.DMA(()),
            pltpu.SemaphoreType.DMA((4,)),
            pltpu.SemaphoreType.DMA((3 * H,)),
            pltpu.SemaphoreType.DMA((8,)),
            pltpu.SemaphoreType.DMA(()),
            pltpu.SemaphoreType.REGULAR,
        ],
        compiler_params=pltpu.CompilerParams(vmem_limit_bytes=124 * 1024 * 1024),
    )(A_x.reshape(S_LEN, DM), A_mem0.reshape(M, DM),
      A_Wq.reshape(512, 64, DH), A_Wk.reshape(512, 64, DH), A_Wv.reshape(512, 64, DH),
      A_Wo.reshape(H * DH, DM), B_w_r.T, B_w_i.T, gate_w.reshape(1, DM),
      _CS, _TWB, _TWS, _SMALL, _TW, _PERM)
    return out.reshape(A_x.shape)


def pallas_gated_mix__memory_aug_recurrent_mem_tr__spectral_gfnet__prompt_kernel(
    A_x, A_mem0, A_Wq, A_Wk, A_Wv, A_Wo, A_seg_len, B_x, B_w_r, B_w_i, gate_w,
):
    del B_x
    assert int(A_seg_len) == SEG and A_x.shape == (1, S_LEN, DM)
    return _run(A_x, A_mem0, A_Wq, A_Wk, A_Wv, A_Wo, B_w_r, B_w_i, gate_w)
```

```python
import functools
import contextlib
import numpy as np
import ml_dtypes

import jax
import jax.numpy as jnp
import jax.experimental.pallas as pl
import jax.experimental.pallas.tpu as pltpu

S_LEN, DM, H, DH, M, SEG = 2048, 1024, 32, 128, 8, 32
L = M + SEG
NSEG = S_LEN // SEG
DF = DM // 2 + 1
f32 = jnp.float32
bf16 = jnp.bfloat16
u32 = jnp.uint32
NSTEP = 64
SCOPES = 0
UNROLL = 3
WO0 = 2


def scope(n):
    return jax.named_scope(n) if SCOPES else contextlib.nullcontext()


def _bf16_np(a):
    return np.asarray(a, np.float32).astype(ml_dtypes.bfloat16)


def _pack_rows_u32(a):
    b = _bf16_np(a).view(np.uint16).astype(np.uint32)
    return b[0::2] | (b[1::2] << 16)


def _make_consts():
    q = np.arange(DM // 4)
    th = 2.0 * np.pi / DM
    a0 = th * ((2 * np.outer(q, q)) % DM)
    a1 = th * ((np.outer(q, 2 * q + 1)) % DM)
    s1f = -np.sin(a1)
    s1f[0, :] = -np.cos(np.pi * q)
    mperm = 16 * (q // 16) + ((q % 16) >> 1) + 8 * (q & 1)
    fwd = [np.cos(a0), np.cos(a1), -np.sin(a0), s1f]
    cs = np.stack([_pack_rows_u32(m[:, mperm]) for m in fwd])
    cs = np.ascontiguousarray(cs.reshape(4, 128, 2, 128).transpose(0, 2, 1, 3)).reshape(8, 128, 128)

    i16 = np.arange(16)
    i128 = np.arange(128)
    d128 = np.exp(-2j * np.pi * ((np.outer(i128, i128)) % 128) / 128.0)
    dc = np.conj(d128)
    small = np.stack([d128.real, d128.imag, dc.real + dc.imag, dc.imag - dc.real]).astype(np.float32)
    tw_f = np.exp(-2j * np.pi * np.outer(i16, i128) / 2048.0)
    tw = np.concatenate([tw_f.real, tw_f.imag]).astype(np.float32)
    twb = np.exp(2j * np.pi * np.outer(i16, np.arange(8)) / 2048.0)
    twb = np.stack([twb.real, twb.imag]).astype(np.float32)
    twb = np.ascontiguousarray(np.broadcast_to(twb[..., None], twb.shape + (128,)))
    tws = np.exp(2j * np.pi * 8 * np.outer(i16, i16) / 2048.0)
    tws = np.concatenate([tws.real.reshape(-1), tws.imag.reshape(-1)]).astype(np.float32)
    perm = np.zeros((128, 128), np.float32)
    for k2 in range(16):
        for lo in range(8):
            perm[k2 * 8 + lo, k2 + 16 * lo] = 1.0
    rev = np.zeros((128, 128), np.float32)
    for p in range(1, 128):
        rev[128 - p, p] = 1.0
    return cs, twb, tws, small, tw, np.stack([perm, rev])


_CS, _TWB, _TWS, _SMALL, _TW, _PERM = _make_consts()
NU = 16


def _cmul_const(x, c):
    re, im = x
    cr, ci = float(np.real(c)), float(np.imag(c))
    if abs(ci) < 1e-9:
        return (re, im) if cr > 0 else (-re, -im)
    if abs(cr) < 1e-9:
        return (-im, re) if ci > 0 else (im, -re)
    if abs(abs(cr) - abs(ci)) < 1e-9:
        a = abs(cr)
        sr, si = (1.0 if cr > 0 else -1.0), (1.0 if ci > 0 else -1.0)
        nr = (re if sr > 0 else -re) - (im if si > 0 else -im)
        ni = (re if si > 0 else -re) + (im if sr > 0 else -im)
        return (nr * a, ni * a)
    return (re * cr - im * ci, re * ci + im * cr)


def _dft4(x, sign):
    (ar, ai), (br, bi), (cr, ci), (dr, di) = x
    s0r, s0i = ar + cr, ai + ci
    s1r, s1i = ar - cr, ai - ci
    s2r, s2i = br + dr, bi + di
    s3r, s3i = br - dr, bi - di
    if sign < 0:
        return [(s0r + s2r, s0i + s2i), (s1r + s3i, s1i - s3r), (s0r - s2r, s0i - s2i), (s1r - s3i, s1i + s3r)]
    return [(s0r + s2r, s0i + s2i), (s1r - s3i, s1i + s3r), (s0r - s2r, s0i - s2i), (s1r + s3i, s1i - s3r)]


def _dft16(x, sign):
    w = np.exp(sign * 2j * np.pi / 16.0)
    t = [[None] * 4 for _ in range(4)]
    for b in range(4):
        col = _dft4([x[4 * a + b] for a in range(4)], sign)
        for c in range(4):
            t[b][c] = col[c] if b * c == 0 else _cmul_const(col[c], w ** (b * c))
    out = [None] * 16
    for c in range(4):
        row = _dft4([t[b][c] for b in range(4)], sign)
        for d in range(4):
            out[c + 4 * d] = row[d]
    return out


def _kernel(x_hbm, mem_hbm, wq_hbm, wk_hbm, wv_hbm, wo_hbm, wr_hbm, wi_hbm, gw_hbm,
            cs_hbm, twb_hbm, tws_hbm, small_hbm, tw_hbm, perm_hbm,
            out_hbm,
            mem_ref, gw_ref, twb_ref, tws_ref, small_ref, tw_ref, perm_ref,
            x_v, cs_v, wrt_v, wit_v, wrn_v, win_v, wp_v, wqkv, wo_v, z1, z2, u0, u1, bt_scr, up_scr, wa_scr, a_scr, out_v,
            sem_x, sem_c, sem_s, sem_in, sem_w, sem_wo, sem_out):
    w32_hbm = tuple(w.bitcast(u32) for w in (wq_hbm, wk_hbm, wv_hbm))
    nt_dims = (((1,), (1,)), ((), ()))

    def cp_x(i):
        r0 = pl.multiple_of(i * 256, 256)
        return pltpu.make_async_copy(x_hbm.at[pl.ds(r0, 256)], x_v.at[pl.ds(r0, 256)], sem_x.at[i])

    cp_cs = pltpu.make_async_copy(cs_hbm, cs_v, sem_c)
    cp_wt = []
    for i, (src, dst, dstn) in enumerate(((wr_hbm, wrt_v, wrn_v), (wi_hbm, wit_v, win_v))):
        cp_wt.append(pltpu.make_async_copy(src.at[pl.ds(0, 512)], dst, sem_in.at[2 * i]))
        cp_wt.append(pltpu.make_async_copy(src.at[pl.ds(512, 1)], dstn, sem_in.at[2 * i + 1]))

    def cp_wo(n):
        return pltpu.make_async_copy(wo_hbm.at[:, pl.ds(n * 128, 128)], wo_v.at[n], sem_wo.at[n])

    def cp_w(p, par, which):
        t = 2 * p + par
        return pltpu.make_async_copy(w32_hbm[which].at[:, par * 16 + p], wqkv.at[3 * t + which],
                                     sem_w.at[3 * t + which])

    def unit_start(p):
        for par in range(2):
            for which in range(3):
                cp_w(p, par, which).start()

    def unit_repack(p, rr=range(0, 512, 64), wait=True):
        if wait:
            for par in range(2):
                for which in range(3):
                    cp_w(p, par, which).wait()
        for which in range(3):
            ta = 6 * p + which
            tb = 6 * p + 3 + which
            for r in rr:
                a = wqkv[ta, r:r + 64, :]
                b = wqkv[tb, r:r + 64, :]
                wqkv[ta, r:r + 64, :] = pltpu.bitcast(pltpu.pack_elementwise([a, b], packed_dtype=jnp.uint16), u32)
                wqkv[tb, r:r + 64, :] = pltpu.bitcast(pltpu.pack_elementwise([a >> 16, b >> 16], packed_dtype=jnp.uint16), u32)

    C0, C1, S0, S1F = range(4)

    def qdot(lhs, mat, nt):
        return jnp.dot(lhs, pltpu.bitcast(cs_v[2 * mat + nt], bf16), preferred_element_type=f32)

    def qdot_t(lhs, mat, dt):
        rows = jnp.concatenate([cs_v[2 * mat + kt, dt * 64:(dt + 1) * 64, :] for kt in range(2)], axis=1)
        return jax.lax.dot_general(lhs, pltpu.bitcast(rows, bf16), nt_dims, preferred_element_type=f32)

    def rev(t, first):
        return jnp.where(lane0, first, jnp.dot(t, perm_ref[1], preferred_element_type=f32))

    cp_small = [pltpu.make_async_copy(src, dst, sem_s.at[i]) for i, (src, dst) in enumerate((
        (perm_hbm, perm_ref), (twb_hbm, twb_ref), (tws_hbm, tws_ref), (small_hbm, small_ref), (tw_hbm, tw_ref),
        (mem_hbm, mem_ref), (gw_hbm, gw_ref)))]
    cp_cs.start()
    cp_small[0].start()
    cp_x(0).start()
    cp_x(1).start()
    for cp in cp_small[1:]:
        cp.start()

    lane_i = jax.lax.broadcasted_iota(jnp.int32, (1, 128), 1)
    lane0 = lane_i == 0
    sgn = (1 - 2 * (lane_i & 1)).astype(f32)
    sgn_m = (1 - 2 * ((lane_i >> 1) & 1)).astype(f32)

    def pro1(c, first):
        @pl.when(c < 3)
        def _():
            cp_x(2 * c + 2).start()
            cp_x(2 * c + 3).start()

        @pl.when(c == 3)
        def _():
            for cp in cp_wt:
                cp.start()

        @pl.when(c >= 4)
        def _():
            unit_start(c - 4)

        cp_x(c).wait()
        if first:
            cp_cs.wait()
            cp_small[0].wait()
        r0 = pl.multiple_of(c * 256, 256)
        xt = [x_v[pl.ds(r0, 256), j * 128:(j + 1) * 128].astype(f32) for j in range(8)]
        zero = jnp.zeros((256, 128), f32)
        r1 = [rev(xt[7], zero), rev(xt[6], xt[7])]
        r2 = [rev(xt[3], zero), rev(xt[2], xt[3])]
        ee, eo, oe, oo = [], [], [], []
        for T in range(2):
            e1, o1 = xt[T] + r1[T], xt[T] - r1[T]
            e2, o2 = r2[T] + xt[4 + T], r2[T] - xt[4 + T]
            ee.append(e1 + e2)
            eo.append(e1 - e2)
            oe.append(o1 - o2)
            oo.append(o1 + o2)
        oo[0] = jnp.where(lane0, xt[2] - xt[6], oo[0])
        e256 = (xt[2] + xt[6])[:, 0:1]
        mid = jnp.broadcast_to(e256, (256, 128)) * sgn_m
        nyq = jnp.sum((ee[0] + ee[1]) * sgn, axis=1, keepdims=True) + e256
        ee, eo, oe, oo = (jnp.concatenate(v, axis=1) for v in (ee, eo, oe, oo))
        rr = pl.ds(2 * c, 2)
        for t in range(2):
            z1[0, rr, :, :, t * 128:(t + 1) * 128] = (qdot(ee, C0, t) + mid).reshape(2, 16, 8, 128)
            z1[0, rr, :, :, (2 + t) * 128:(3 + t) * 128] = qdot(eo, C1, t).reshape(2, 16, 8, 128)
            z1[1, rr, :, :, t * 128:(t + 1) * 128] = qdot(oe, S0, t).reshape(2, 16, 8, 128)
            z1[1, rr, :, :, (2 + t) * 128:(3 + t) * 128] = qdot(oo, S1F, t).reshape(2, 16, 8, 128)
        z1[0, rr, :, :, 512:640] = jnp.where(lane0, nyq, 0.0).reshape(2, 16, 8, 128)
        z1[1, rr, :, :, 512:640] = jnp.zeros((2, 16, 8, 128), f32)

    with scope("s_pro1"):
        pro1(0, True)
        jax.lax.fori_loop(1, 8, lambda c, carry: (pro1(c, False), carry)[1], 0)

    def stage_a(hi):
        for t in range(5):
            sl = slice(t * 128, (t + 1) * 128)
            xin = [(z1[0, s2, hi, :, sl], z1[1, s2, hi, :, sl]) for s2 in range(16)]
            xo = _dft16(xin, -1)
            for k2 in range(16):
                z2[0, k2, hi, :, sl] = xo[k2][0]
                z2[1, k2, hi, :, sl] = xo[k2][1]

    norm = 1.0 / (S_LEN * DM)
    cscale = [jnp.where(lane0, norm, 2.0 * norm).astype(f32)] + [2.0 * norm] * 3 + [norm]

    def wperm(c, carry):
        @pl.when(c % 3 == 0)
        def _():
            unit_start(6 + c // 3)

        for bb in range(2):
            blk_i = 2 * c + bb
            l0 = pl.multiple_of(blk_i * 128, 128)
            for i, (wt, wn) in enumerate(((wrt_v.bitcast(u32), wrn_v), (wit_v.bitcast(u32), win_v))):
                for t in range(5):
                    if t < 4:
                        w = wt[(t % 2) * 128:(t % 2 + 1) * 128, pl.ds(l0, 128)].reshape(8, 16, 128)
                        if t >= 2:
                            w = w >> 16
                        pk = pltpu.pack_elementwise([w[:, :8, :], w[:, 8:, :]], packed_dtype=jnp.uint16)
                        blk = pltpu.bitcast(pltpu.bitcast(pk, u32).reshape(64, 128), bf16)
                    else:
                        blk = jnp.broadcast_to(wn[:, pl.ds(l0, 128)], (128, 128))
                    o = jax.lax.dot_general(perm_ref[0], blk, nt_dims, preferred_element_type=f32)
                    wp_v[i, :, blk_i, :, t * 128:(t + 1) * 128] = (o * cscale[t]).reshape(16, 8, 128)
        return carry

    def stage_a_loop(hi, carry):
        @pl.when(hi % 8 == 0)
        def _():
            unit_start(4 + hi // 8)

        stage_a(hi)
        return carry

    with scope("s_stage_a"):
        for cp in cp_small[1:]:
            cp.wait()
        jax.lax.fori_loop(0, 16, stage_a_loop, 0)

    with scope("s_wperm"):
        for cp in cp_wt:
            cp.wait()
        jax.lax.fori_loop(0, 8, wperm, 0)

    def cdot3(m1, m2, m3, zr, zi):
        k1 = jnp.dot(m1, (zr + zi).astype(bf16), preferred_element_type=f32)
        k2 = jnp.dot(m2, zi.astype(bf16), preferred_element_type=f32)
        k3 = jnp.dot(m3, zr.astype(bf16), preferred_element_type=f32)
        return k1 - k2, k1 + k3

    def b_fwd(k2):
        tr, ti = tw_ref[pl.ds(k2, 1), :], tw_ref[pl.ds(16 + k2, 1), :]
        mr = small_ref[0] * tr - small_ref[1] * ti
        mi = small_ref[0] * ti + small_ref[1] * tr
        return cdot3(mr, mr + mi, mi - mr, z2[0, k2].reshape(128, 640), z2[1, k2].reshape(128, 640))

    def b_inv(k2, x):
        xr, xi = x
        wr = wp_v[0, k2].reshape(128, 640)
        wi = wp_v[1, k2].reshape(128, 640)
        pr = xr * wr - xi * wi
        pi = xr * wi + xi * wr
        gr, gi = cdot3(small_ref[0], small_ref[2], small_ref[3], pr, pi)
        z1[0, k2] = gr.reshape(16, 8, 640)
        z1[1, k2] = gi.reshape(16, 8, 640)

    def stage_b2(j, carry):
        @pl.when(j < 7)
        def _():
            unit_start(9 + j)

        xa = b_fwd(2 * j)
        xb = b_fwd(2 * j + 1)
        b_inv(2 * j, xa)
        b_inv(2 * j + 1, xb)
        return carry

    with scope('s_stage_b'):
        jax.lax.fori_loop(0, 8, stage_b2, 0)

    lane0a = jax.lax.broadcasted_iota(jnp.int32, (8, 128), 1) == 0

    def inv_twiddles(hi):
        tw_inv = [None]
        for k2 in range(1, 16):
            cr, ci = tws_ref[hi * 16 + k2], tws_ref[256 + hi * 16 + k2]
            br, bi = twb_ref[0, k2], twb_ref[1, k2]
            tw_inv.append((br * cr - bi * ci, br * ci + bi * cr))
        return tw_inv

    def a_inv_tile(hi, t, tw_inv, u_dst):
        sl = slice(t * 128, (t + 1) * 128)
        w = np.exp(2j * np.pi / 16.0)
        tmp = bt_scr.at[t % 2]
        for b in range(4):
            xin = []
            for a in range(4):
                k2 = 4 * a + b
                gr, gi = z1[0, k2, hi, :, sl], z1[1, k2, hi, :, sl]
                if k2 > 0:
                    tr, ti = tw_inv[k2]
                    gr, gi = gr * tr - gi * ti, gr * ti + gi * tr
                xin.append((gr, gi))
            col = _dft4(xin, +1)
            for c in range(4):
                v = col[c] if b * c == 0 else _cmul_const(col[c], w ** (b * c))
                tmp[0, b, c] = v[0]
                tmp[1, b, c] = v[1]
        for c in range(4):
            row = _dft4([(tmp[0, b, c], tmp[1, b, c]) for b in range(4)], +1)
            for d in range(4):
                s2 = c + 4 * d
                u_dst[s2, :, sl] = row[d][0]
                if t < 4:
                    u_dst[s2, :, 640 + t * 128:640 + (t + 1) * 128] = row[d][1]

    def stage_c2(m, carry):
        @pl.when(jnp.logical_and(m >= WO0, m < WO0 + 4))
        def _():
            cp_wo(2 * (m - WO0)).start()
            cp_wo(2 * (m - WO0) + 1).start()

        stage_c(2 * m, 2 * m + 1, u0, u1)
        stage_c(2 * m + 1, jnp.minimum(2 * m + 2, 15), u1, u0)
        return carry

    def stage_c(hi, nxt, u_src, u_dst):
        tw_inv = inv_twiddles(nxt)
        unit_repack(hi)
        for t in range(5):
            a_inv_tile(nxt, t, tw_inv, u_dst)
        nyq = u_src[:, :, 512:513].reshape(128, 1)
        n = jnp.broadcast_to(nyq, (128, 128)) * sgn
        ue_r = u_src[:, :, 0:256].reshape(128, 256)
        uo_r = u_src[:, :, 256:512].reshape(128, 256)
        ue_i = u_src[:, :, 640:896].reshape(128, 256)
        uo_i = u_src[:, :, 896:1152].reshape(128, 256)
        for T in range(2):
            a0 = qdot_t(ue_r, C0, T) + n
            a1 = qdot_t(uo_r, C1, T)
            b0 = qdot_t(ue_i, S0, T)
            b1 = qdot_t(uo_i, S1F, T)
            if T == 0:
                b1 = jnp.where(lane0, 0.0, b1)
            p, q, pm, qm = a0 + a1, b0 + b1, a0 - a1, b0 - b1
            z2[0, :, hi, :, T * 128:(T + 1) * 128] = (p + q).reshape(16, 8, 128)
            z2[1, :, hi, :, T * 128:(T + 1) * 128] = (pm + qm).reshape(16, 8, 128)
            up_scr[T] = p - q
            up_scr[2 + T] = pm - qm
        s_e = jnp.sum((ue_r[:, :128] + ue_r[:, 128:]) * sgn_m, axis=1, keepdims=True) + nyq
        s_o = jnp.sum((uo_i[:, :128] + uo_i[:, 128:]) * sgn_m, axis=1, keepdims=True)
        z2[1, :, hi, :, 384:512] = rev(up_scr[0], up_scr[1]).reshape(16, 8, 128)
        z2[1, :, hi, :, 256:384] = rev(up_scr[1], s_e + s_o).reshape(16, 8, 128)
        z2[0, :, hi, :, 384:512] = rev(up_scr[2], up_scr[3]).reshape(16, 8, 128)
        z2[0, :, hi, :, 256:384] = rev(up_scr[3], s_e - s_o).reshape(16, 8, 128)

    with scope("s_stage_c"):
        tw0 = inv_twiddles(0)
        for t in range(5):
            a_inv_tile(0, t, tw0, u0)
        jax.lax.fori_loop(0, 8, stage_c2, 0)

    scale = DH ** -0.5
    rows = jax.lax.broadcasted_iota(jnp.int32, (L, L), 0)
    cols = jax.lax.broadcasted_iota(jnp.int32, (L, L), 1)
    mask = (rows < M) | (rows >= cols)
    wo32 = wo_v.bitcast(u32)

    def qkv_head(h, hd):
        return tuple(jnp.dot(h, pltpu.bitcast(wqkv[3 * hd + j], bf16), preferred_element_type=f32)
                     for j in range(3))

    def scores(qkv):
        return jax.lax.dot_general(qkv[0], qkv[1].astype(bf16), nt_dims, preferred_element_type=f32)

    def softmax(s):
        s = jnp.where(mask, s * scale, -1e9)
        m = jnp.max(s, axis=-1, keepdims=True)
        p = jnp.exp(s - m)
        l = jnp.sum(p, axis=-1, keepdims=True)
        return p / l

    def pv(p, qkv):
        return jnp.dot(p, qkv[2].astype(bf16), preferred_element_type=f32)

    def cp_out(seg0, nseg):
        r0 = pl.multiple_of(seg0 * SEG, SEG)
        return pltpu.make_async_copy(out_v.at[pl.ds(r0, nseg * SEG)], out_hbm.at[pl.ds(r0, nseg * SEG)], sem_out)

    def mix(seg):
        r0 = pl.multiple_of(seg * SEG, SEG)
        xs = x_v[pl.ds(r0, SEG), :].astype(f32)
        gw = gw_ref[...].astype(f32)
        gwr = jnp.concatenate([gw[r:r + 1, :] for r in range(8)], axis=1)
        gate = jax.nn.sigmoid(jnp.sum(xs * gwr, axis=-1, keepdims=True))
        s2 = seg // 4
        hi0 = (seg % 4) * 4
        b = jnp.concatenate([z2[0, s2, pl.ds(hi0, 4), :, 0:512].reshape(SEG, 512),
                             z2[1, s2, pl.ds(hi0, 4), :, 0:512].reshape(SEG, 512)], axis=1)
        res = gate * a_scr[...] + (1.0 - gate) * b
        out_v[pl.ds(r0, SEG), :] = res.astype(out_v.dtype)

    HA = 28

    def wo_part(h0, h1, n, lhs):
        w = pltpu.bitcast(wo32[n, h0 * (DH // 2):h1 * (DH // 2), :], bf16)
        return jnp.dot(lhs, w, preferred_element_type=f32)

    def step(s, mem, first=False):
        r0 = s * SEG if first else pl.multiple_of(s * SEG, SEG)
        xs = x_v[pl.ds(r0, SEG), :].astype(f32)
        h = jnp.concatenate([mem, xs], axis=0)
        qkvs, sc, ps, oh = {}, {}, {}, {}

        def wo_a(n):
            if first:
                cp_wo(n).wait()
            wa_scr[:, n * 128:(n + 1) * 128] = wo_part(0, HA, n, oa)

        for i in range(3):
            qkvs[i] = qkv_head(h, i)
        sc[0] = scores(qkvs[0])
        sc[1] = scores(qkvs[1])
        ps[0] = softmax(sc.pop(0))
        if not first:
            mix(s - 1)
        for hd in range(H):
            if hd + 3 < H:
                qkvs[hd + 3] = qkv_head(h, hd + 3)
            if hd == HA + 1:
                wo_a(0)
            if hd + 2 < H:
                sc[hd + 2] = scores(qkvs[hd + 2])
            if hd + 1 < H:
                ps[hd + 1] = softmax(sc.pop(hd + 1))
            oh[hd] = pv(ps.pop(hd), qkvs.pop(hd))
            if hd == HA - 1:
                oa = jnp.concatenate([oh.pop(i) for i in range(HA)], axis=1)
            if hd == HA + 1:
                for n in (1, 2, 3):
                    wo_a(n)
            if hd == HA + 2:
                for n in (4, 5):
                    wo_a(n)
        for n in (6, 7):
            wo_a(n)
        ob = jnp.concatenate([oh.pop(i) for i in range(HA, H)], axis=1)
        out = wa_scr[...] + jnp.concatenate([wo_part(HA, H, n, ob) for n in range(8)], axis=1)
        a_scr[...] = out[M:]
        if not first:
            @pl.when(s % 3 == 0)
            def _():
                cp_out(s - 3, 3).start()

        return out[:M].astype(bf16).astype(f32)

    with scope('s_main'):
        mem1 = step(0, mem_ref[...].astype(f32), first=True)
        jax.lax.fori_loop(1, NSTEP, step, mem1, unroll=UNROLL)
    mix(NSTEP - 1)
    last = ((NSTEP - 1) // 3) * 3
    cp_out(last, NSTEP - last).start()
    pltpu.make_async_copy(out_v.at[pl.ds(0, NSTEP * SEG)], out_hbm.at[pl.ds(0, NSTEP * SEG)], sem_out).wait()


@jax.jit
def _run(A_x, A_mem0, A_Wq, A_Wk, A_Wv, A_Wo, B_w_r, B_w_i, gate_w):
    any_spec = pl.BlockSpec(memory_space=pl.ANY)
    out = pl.pallas_call(
        _kernel,
        out_shape=jax.ShapeDtypeStruct((S_LEN, DM), A_x.dtype),
        in_specs=[any_spec] * 15,
        out_specs=any_spec,
        scratch_shapes=[
            pltpu.VMEM((M, DM), bf16),
            pltpu.VMEM((8, 128), bf16),
            pltpu.VMEM((2, 16, 8, 128), f32),
            pltpu.SMEM((512,), f32),
            pltpu.VMEM((4, 128, 128), f32),
            pltpu.VMEM((32, 128), f32),
            pltpu.VMEM((2, 128, 128), f32),
            pltpu.VMEM((S_LEN, DM), bf16),
            pltpu.VMEM((8, 128, 128), u32),
            pltpu.VMEM((DM // 2, S_LEN), bf16),
            pltpu.VMEM((DM // 2, S_LEN), bf16),
            pltpu.VMEM((1, S_LEN), bf16),
            pltpu.VMEM((1, S_LEN), bf16),
            pltpu.VMEM((2, 16, 16, 8, 640), f32),
            pltpu.VMEM((3 * H, DM // 2, DH), u32),
            pltpu.VMEM((8, H * DH, 128), bf16),
            pltpu.VMEM((2, 16, 16, 8, 640), f32),
            pltpu.VMEM((2, 16, 16, 8, 640), f32),
            pltpu.VMEM((16, 8, 1152), f32),
            pltpu.VMEM((16, 8, 1152), f32),
            pltpu.VMEM((2, 2, 4, 4, 8, 128), f32),
            pltpu.VMEM((4, 128, 128), f32),
            pltpu.VMEM((L, DM), f32),
            pltpu.VMEM((SEG, DM), f32),
            pltpu.VMEM((S_LEN, DM), bf16),
            pltpu.SemaphoreType.DMA((8,)),
            pltpu.SemaphoreType.DMA(()),
            pltpu.SemaphoreType.DMA((7,)),
            pltpu.SemaphoreType.DMA((4,)),
            pltpu.SemaphoreType.DMA((3 * H,)),
            pltpu.SemaphoreType.DMA((8,)),
            pltpu.SemaphoreType.DMA(()),
        ],
        compiler_params=pltpu.CompilerParams(vmem_limit_bytes=124 * 1024 * 1024),
    )(A_x.reshape(S_LEN, DM), A_mem0.reshape(M, DM),
      A_Wq.reshape(512, 64, DH), A_Wk.reshape(512, 64, DH), A_Wv.reshape(512, 64, DH),
      A_Wo.reshape(H * DH, DM), B_w_r.T, B_w_i.T, gate_w.reshape(8, 128),
      _CS, _TWB, _TWS, _SMALL, _TW, _PERM)
    return out.reshape(A_x.shape)


def pallas_gated_mix__memory_aug_recurrent_mem_tr__spectral_gfnet__prompt_kernel(
    A_x, A_mem0, A_Wq, A_Wk, A_Wv, A_Wo, A_seg_len, B_x, B_w_r, B_w_i, gate_w,
):
    del B_x
    assert int(A_seg_len) == SEG and A_x.shape == (1, S_LEN, DM)
    return _run(A_x, A_mem0, A_Wq, A_Wk, A_Wv, A_Wo, B_w_r, B_w_i, gate_w)
```

```python
import functools
import contextlib
import numpy as np
import ml_dtypes

import jax
import jax.numpy as jnp
import jax.experimental.pallas as pl
import jax.experimental.pallas.tpu as pltpu

S_LEN, DM, H, DH, M, SEG = 2048, 1024, 32, 128, 8, 32
L = M + SEG
NSEG = S_LEN // SEG
DF = DM // 2 + 1
f32 = jnp.float32
bf16 = jnp.bfloat16
u32 = jnp.uint32
NSTEP = 64
SCOPES = 0
UNROLL = 3
WO0 = 2
HA_K = 27
SCHED_ID = 4
_SCHEDS = [
    {(28, 0): (0,), (28, 1): (1, 2, 3), (29, 1): (4, 5), (31, 1): (6, 7)},
    {(28, 0): (0,), (28, 1): (1, 2), (29, 1): (3, 4), (30, 1): (5, 6), (31, 1): (7,)},
    {(28, 1): (0, 1), (29, 1): (2, 3), (30, 1): (4, 5), (31, 1): (6, 7)},
    {(28, 0): (0,), (29, 0): (1, 2), (30, 0): (3, 4), (31, 0): (5, 6), (31, 1): (7,)},
    {(28, 1): (0,), (29, 0): (1,), (29, 1): (2, 3), (30, 1): (4, 5, 6), (31, 1): (7,)},
    {(29, 0): (0, 1), (29, 1): (2, 3), (30, 1): (4, 5), (31, 1): (6, 7)},
]
SCHED = _SCHEDS[SCHED_ID]


def scope(n):
    return jax.named_scope(n) if SCOPES else contextlib.nullcontext()


def _bf16_np(a):
    return np.asarray(a, np.float32).astype(ml_dtypes.bfloat16)


def _pack_rows_u32(a):
    b = _bf16_np(a).view(np.uint16).astype(np.uint32)
    return b[0::2] | (b[1::2] << 16)


def _make_consts():
    q = np.arange(DM // 4)
    th = 2.0 * np.pi / DM
    a0 = th * ((2 * np.outer(q, q)) % DM)
    a1 = th * ((np.outer(q, 2 * q + 1)) % DM)
    s1f = -np.sin(a1)
    s1f[0, :] = -np.cos(np.pi * q)
    mperm = 16 * (q // 16) + ((q % 16) >> 1) + 8 * (q & 1)
    fwd = [np.cos(a0), np.cos(a1), -np.sin(a0), s1f]
    cs = np.stack([_pack_rows_u32(m[:, mperm]) for m in fwd])
    cs = np.ascontiguousarray(cs.reshape(4, 128, 2, 128).transpose(0, 2, 1, 3)).reshape(8, 128, 128)

    i16 = np.arange(16)
    i128 = np.arange(128)
    d128 = np.exp(-2j * np.pi * ((np.outer(i128, i128)) % 128) / 128.0)
    dc = np.conj(d128)
    small = np.stack([d128.real, d128.imag, dc.real + dc.imag, dc.imag - dc.real]).astype(np.float32)
    tw_f = np.exp(-2j * np.pi * np.outer(i16, i128) / 2048.0)
    tw = np.concatenate([tw_f.real, tw_f.imag]).astype(np.float32)
    twb = np.exp(2j * np.pi * np.outer(i16, np.arange(8)) / 2048.0)
    twb = np.stack([twb.real, twb.imag]).astype(np.float32)
    twb = np.ascontiguousarray(np.broadcast_to(twb[..., None], twb.shape + (128,)))
    tws = np.exp(2j * np.pi * 8 * np.outer(i16, i16) / 2048.0)
    tws = np.concatenate([tws.real.reshape(-1), tws.imag.reshape(-1)]).astype(np.float32)
    perm = np.zeros((128, 128), np.float32)
    for k2 in range(16):
        for lo in range(8):
            perm[k2 * 8 + lo, k2 + 16 * lo] = 1.0
    rev = np.zeros((128, 128), np.float32)
    for p in range(1, 128):
        rev[128 - p, p] = 1.0
    return cs, twb, tws, small, tw, np.stack([perm, rev])


_CS, _TWB, _TWS, _SMALL, _TW, _PERM = _make_consts()
NU = 16


def _lo_pair(a, b):
    return (a & np.uint32(0xFFFF)) | (b << 16)


def _hi_pair(a, b):
    return (a >> 16) | (b & np.uint32(0xFFFF0000))


def _cmul_const(x, c):
    re, im = x
    cr, ci = float(np.real(c)), float(np.imag(c))
    if abs(ci) < 1e-9:
        return (re, im) if cr > 0 else (-re, -im)
    if abs(cr) < 1e-9:
        return (-im, re) if ci > 0 else (im, -re)
    if abs(abs(cr) - abs(ci)) < 1e-9:
        a = abs(cr)
        sr, si = (1.0 if cr > 0 else -1.0), (1.0 if ci > 0 else -1.0)
        nr = (re if sr > 0 else -re) - (im if si > 0 else -im)
        ni = (re if si > 0 else -re) + (im if sr > 0 else -im)
        return (nr * a, ni * a)
    return (re * cr - im * ci, re * ci + im * cr)


def _dft4(x, sign):
    (ar, ai), (br, bi), (cr, ci), (dr, di) = x
    s0r, s0i = ar + cr, ai + ci
    s1r, s1i = ar - cr, ai - ci
    s2r, s2i = br + dr, bi + di
    s3r, s3i = br - dr, bi - di
    if sign < 0:
        return [(s0r + s2r, s0i + s2i), (s1r + s3i, s1i - s3r), (s0r - s2r, s0i - s2i), (s1r - s3i, s1i + s3r)]
    return [(s0r + s2r, s0i + s2i), (s1r - s3i, s1i + s3r), (s0r - s2r, s0i - s2i), (s1r + s3i, s1i - s3r)]


def _dft16(x, sign):
    w = np.exp(sign * 2j * np.pi / 16.0)
    t = [[None] * 4 for _ in range(4)]
    for b in range(4):
        col = _dft4([x[4 * a + b] for a in range(4)], sign)
        for c in range(4):
            t[b][c] = col[c] if b * c == 0 else _cmul_const(col[c], w ** (b * c))
    out = [None] * 16
    for c in range(4):
        row = _dft4([t[b][c] for b in range(4)], sign)
        for d in range(4):
            out[c + 4 * d] = row[d]
    return out


def _kernel(x_hbm, mem_hbm, wq_hbm, wk_hbm, wv_hbm, wo_hbm, wr_hbm, wi_hbm, gw_hbm,
            cs_hbm, twb_hbm, tws_hbm, small_hbm, tw_hbm, perm_hbm,
            out_hbm,
            mem_ref, gw_ref, gw_row, twb_ref, tws_ref, small_ref, tw_ref, perm_ref,
            x_v, cs_v, wrt_v, wit_v, wrn_v, win_v, wp_v, wqkv, wo_v, z1, z2, u0, u1, bt_scr, up_scr, wa_scr, a_scr, out_v,
            sem_x, sem_c, sem_s, sem_in, sem_w, sem_wo, sem_out):
    w32_hbm = tuple(w.bitcast(u32) for w in (wq_hbm, wk_hbm, wv_hbm))
    nt_dims = (((1,), (1,)), ((), ()))

    def cp_x(i):
        r0 = pl.multiple_of(i * 256, 256)
        return pltpu.make_async_copy(x_hbm.at[pl.ds(r0, 256)], x_v.at[pl.ds(r0, 256)], sem_x.at[i])

    cp_cs = pltpu.make_async_copy(cs_hbm, cs_v, sem_c)
    cp_wt = []
    for i, (src, dst, dstn) in enumerate(((wr_hbm, wrt_v, wrn_v), (wi_hbm, wit_v, win_v))):
        cp_wt.append(pltpu.make_async_copy(src.at[pl.ds(0, 512)], dst, sem_in.at[2 * i]))
        cp_wt.append(pltpu.make_async_copy(src.at[pl.ds(512, 1)], dstn, sem_in.at[2 * i + 1]))

    def cp_wo(n):
        return pltpu.make_async_copy(wo_hbm.at[:, pl.ds(n * 128, 128)], wo_v.at[n], sem_wo.at[n])

    def cp_w(p, par, which):
        t = 2 * p + par
        return pltpu.make_async_copy(w32_hbm[which].at[:, par * 16 + p], wqkv.at[3 * t + which],
                                     sem_w.at[3 * t + which])

    def unit_start(p):
        for par in range(2):
            for which in range(3):
                cp_w(p, par, which).start()

    def unit_repack(p, rr=range(0, 512, 64), wait=True):
        if wait:
            for par in range(2):
                for which in range(3):
                    cp_w(p, par, which).wait()
        for which in range(3):
            ta = 6 * p + which
            tb = 6 * p + 3 + which
            for r in rr:
                a = wqkv[ta, r:r + 64, :]
                b = wqkv[tb, r:r + 64, :]
                wqkv[ta, r:r + 64, :] = _lo_pair(a, b)
                wqkv[tb, r:r + 64, :] = _hi_pair(a, b)

    C0, C1, S0, S1F = range(4)

    def qdot(lhs, mat, nt):
        return jnp.dot(lhs, pltpu.bitcast(cs_v[2 * mat + nt], bf16), preferred_element_type=f32)

    def qdot_t(lhs, mat, dt):
        rows = jnp.concatenate([cs_v[2 * mat + kt, dt * 64:(dt + 1) * 64, :] for kt in range(2)], axis=1)
        return jax.lax.dot_general(lhs, pltpu.bitcast(rows, bf16), nt_dims, preferred_element_type=f32)

    def rev(t, first):
        return jnp.where(lane0, first, jnp.dot(t, perm_ref[1], preferred_element_type=f32))

    cp_small = [pltpu.make_async_copy(src, dst, sem_s.at[i]) for i, (src, dst) in enumerate((
        (perm_hbm, perm_ref), (twb_hbm, twb_ref), (tws_hbm, tws_ref), (small_hbm, small_ref), (tw_hbm, tw_ref),
        (mem_hbm, mem_ref), (gw_hbm, gw_ref)))]
    cp_cs.start()
    cp_small[0].start()
    cp_x(0).start()
    cp_x(1).start()
    for cp in cp_small[1:]:
        cp.start()

    lane_i = jax.lax.broadcasted_iota(jnp.int32, (1, 128), 1)
    lane0 = lane_i == 0
    sgn = (1 - 2 * (lane_i & 1)).astype(f32)
    sgn_m = (1 - 2 * ((lane_i >> 1) & 1)).astype(f32)

    def pro1(c, first):
        @pl.when(c < 3)
        def _():
            cp_x(2 * c + 2).start()
            cp_x(2 * c + 3).start()

        @pl.when(c == 3)
        def _():
            for cp in cp_wt:
                cp.start()

        @pl.when(c >= 4)
        def _():
            unit_start(c - 4)

        cp_x(c).wait()
        if first:
            cp_cs.wait()
            cp_small[0].wait()
        r0 = pl.multiple_of(c * 256, 256)
        xt = [x_v[pl.ds(r0, 256), j * 128:(j + 1) * 128].astype(f32) for j in range(8)]
        zero = jnp.zeros((256, 128), f32)
        r1 = [rev(xt[7], zero), rev(xt[6], xt[7])]
        r2 = [rev(xt[3], zero), rev(xt[2], xt[3])]
        ee, eo, oe, oo = [], [], [], []
        for T in range(2):
            e1, o1 = xt[T] + r1[T], xt[T] - r1[T]
            e2, o2 = r2[T] + xt[4 + T], r2[T] - xt[4 + T]
            ee.append(e1 + e2)
            eo.append(e1 - e2)
            oe.append(o1 - o2)
            oo.append(o1 + o2)
        oo[0] = jnp.where(lane0, xt[2] - xt[6], oo[0])
        e256 = (xt[2] + xt[6])[:, 0:1]
        mid = jnp.broadcast_to(e256, (256, 128)) * sgn_m
        nyq = jnp.sum((ee[0] + ee[1]) * sgn, axis=1, keepdims=True) + e256
        ee, eo, oe, oo = (jnp.concatenate(v, axis=1) for v in (ee, eo, oe, oo))
        rr = pl.ds(2 * c, 2)
        for t in range(2):
            z1[0, rr, :, :, t * 128:(t + 1) * 128] = (qdot(ee, C0, t) + mid).reshape(2, 16, 8, 128)
            z1[0, rr, :, :, (2 + t) * 128:(3 + t) * 128] = qdot(eo, C1, t).reshape(2, 16, 8, 128)
            z1[1, rr, :, :, t * 128:(t + 1) * 128] = qdot(oe, S0, t).reshape(2, 16, 8, 128)
            z1[1, rr, :, :, (2 + t) * 128:(3 + t) * 128] = qdot(oo, S1F, t).reshape(2, 16, 8, 128)
        z1[0, rr, :, :, 512:640] = jnp.where(lane0, nyq, 0.0).reshape(2, 16, 8, 128)
        z1[1, rr, :, :, 512:640] = jnp.zeros((2, 16, 8, 128), f32)

    with scope("s_pro1"):
        pro1(0, True)
        jax.lax.fori_loop(1, 8, lambda c, carry: (pro1(c, False), carry)[1], 0)

    def stage_a(hi):
        for t in range(5):
            sl = slice(t * 128, (t + 1) * 128)
            xin = [(z1[0, s2, hi, :, sl], z1[1, s2, hi, :, sl]) for s2 in range(16)]
            xo = _dft16(xin, -1)
            for k2 in range(16):
                z2[0, k2, hi, :, sl] = xo[k2][0]
                z2[1, k2, hi, :, sl] = xo[k2][1]

    norm = 1.0 / (S_LEN * DM)
    cscale = [jnp.where(lane0, norm, 2.0 * norm).astype(f32)] + [2.0 * norm] * 3 + [norm]

    def wperm(c, carry):
        @pl.when(c % 3 == 0)
        def _():
            unit_start(6 + c // 3)

        for bb in range(2):
            blk_i = 2 * c + bb
            l0 = pl.multiple_of(blk_i * 128, 128)
            for i, (wt, wn) in enumerate(((wrt_v.bitcast(u32), wrn_v), (wit_v.bitcast(u32), win_v))):
                for t in range(5):
                    if t < 4:
                        w = wt[(t % 2) * 128:(t % 2 + 1) * 128, pl.ds(l0, 128)].reshape(8, 16, 128)
                        pk = (_lo_pair if t < 2 else _hi_pair)(w[:, :8, :], w[:, 8:, :])
                        blk = pltpu.bitcast(pk.reshape(64, 128), bf16)
                    else:
                        blk = jnp.broadcast_to(wn[:, pl.ds(l0, 128)], (128, 128))
                    o = jax.lax.dot_general(perm_ref[0], blk, nt_dims, preferred_element_type=f32)
                    wp_v[i, :, blk_i, :, t * 128:(t + 1) * 128] = (o * cscale[t]).reshape(16, 8, 128)
        return carry

    def stage_a_loop(hi, carry):
        @pl.when(hi % 8 == 0)
        def _():
            unit_start(4 + hi // 8)

        stage_a(hi)
        return carry

    with scope("s_stage_a"):
        for cp in cp_small[1:]:
            cp.wait()
        gw_row[...] = gw_ref[...].astype(f32)
        jax.lax.fori_loop(0, 16, stage_a_loop, 0)

    with scope("s_wperm"):
        for cp in cp_wt:
            cp.wait()
        jax.lax.fori_loop(0, 8, wperm, 0)

    def cdot3(m1, m2, m3, zr, zi):
        k1 = jnp.dot(m1, (zr + zi).astype(bf16), preferred_element_type=f32)
        k2 = jnp.dot(m2, zi.astype(bf16), preferred_element_type=f32)
        k3 = jnp.dot(m3, zr.astype(bf16), preferred_element_type=f32)
        return k1 - k2, k1 + k3

    def b_fwd(k2):
        tr, ti = tw_ref[pl.ds(k2, 1), :], tw_ref[pl.ds(16 + k2, 1), :]
        mr = small_ref[0] * tr - small_ref[1] * ti
        mi = small_ref[0] * ti + small_ref[1] * tr
        return cdot3(mr, mr + mi, mi - mr, z2[0, k2].reshape(128, 640), z2[1, k2].reshape(128, 640))

    def b_inv(k2, x):
        xr, xi = x
        wr = wp_v[0, k2].reshape(128, 640)
        wi = wp_v[1, k2].reshape(128, 640)
        pr = xr * wr - xi * wi
        pi = xr * wi + xi * wr
        gr, gi = cdot3(small_ref[0], small_ref[2], small_ref[3], pr, pi)
        z1[0, k2] = gr.reshape(16, 8, 640)
        z1[1, k2] = gi.reshape(16, 8, 640)

    def stage_b2(j, carry):
        @pl.when(j < 7)
        def _():
            unit_start(9 + j)

        xa = b_fwd(2 * j)
        xb = b_fwd(2 * j + 1)
        b_inv(2 * j, xa)
        b_inv(2 * j + 1, xb)
        return carry

    with scope('s_stage_b'):
        jax.lax.fori_loop(0, 8, stage_b2, 0)

    lane0a = jax.lax.broadcasted_iota(jnp.int32, (8, 128), 1) == 0

    def inv_twiddles(hi):
        tw_inv = [None]
        for k2 in range(1, 16):
            cr, ci = tws_ref[hi * 16 + k2], tws_ref[256 + hi * 16 + k2]
            br, bi = twb_ref[0, k2], twb_ref[1, k2]
            tw_inv.append((br * cr - bi * ci, br * ci + bi * cr))
        return tw_inv

    def a_inv_tile(hi, t, tw_inv, u_dst):
        sl = slice(t * 128, (t + 1) * 128)
        w = np.exp(2j * np.pi / 16.0)
        tmp = bt_scr.at[t % 2]
        for b in range(4):
            xin = []
            for a in range(4):
                k2 = 4 * a + b
                gr, gi = z1[0, k2, hi, :, sl], z1[1, k2, hi, :, sl]
                if k2 > 0:
                    tr, ti = tw_inv[k2]
                    gr, gi = gr * tr - gi * ti, gr * ti + gi * tr
                xin.append((gr, gi))
            col = _dft4(xin, +1)
            for c in range(4):
                v = col[c] if b * c == 0 else _cmul_const(col[c], w ** (b * c))
                tmp[0, b, c] = v[0]
                tmp[1, b, c] = v[1]
        for c in range(4):
            row = _dft4([(tmp[0, b, c], tmp[1, b, c]) for b in range(4)], +1)
            for d in range(4):
                s2 = c + 4 * d
                u_dst[s2, :, sl] = row[d][0]
                if t < 4:
                    u_dst[s2, :, 640 + t * 128:640 + (t + 1) * 128] = row[d][1]

    def stage_c2(m, carry):
        @pl.when(jnp.logical_and(m >= WO0, m < WO0 + 4))
        def _():
            cp_wo(2 * (m - WO0)).start()
            cp_wo(2 * (m - WO0) + 1).start()

        stage_c(2 * m, 2 * m + 1, u0, u1)
        stage_c(2 * m + 1, jnp.minimum(2 * m + 2, 15), u1, u0)
        return carry

    def stage_c(hi, nxt, u_src, u_dst):
        tw_inv = inv_twiddles(nxt)
        unit_repack(hi)
        for t in range(5):
            a_inv_tile(nxt, t, tw_inv, u_dst)
        nyq = u_src[:, :, 512:513].reshape(128, 1)
        n = jnp.broadcast_to(nyq, (128, 128)) * sgn
        ue_r = u_src[:, :, 0:256].reshape(128, 256)
        uo_r = u_src[:, :, 256:512].reshape(128, 256)
        ue_i = u_src[:, :, 640:896].reshape(128, 256)
        uo_i = u_src[:, :, 896:1152].reshape(128, 256)
        for T in range(2):
            a0 = qdot_t(ue_r, C0, T) + n
            a1 = qdot_t(uo_r, C1, T)
            b0 = qdot_t(ue_i, S0, T)
            b1 = qdot_t(uo_i, S1F, T)
            if T == 0:
                b1 = jnp.where(lane0, 0.0, b1)
            p, q, pm, qm = a0 + a1, b0 + b1, a0 - a1, b0 - b1
            z2[0, :, hi, :, T * 128:(T + 1) * 128] = (p + q).reshape(16, 8, 128)
            z2[1, :, hi, :, T * 128:(T + 1) * 128] = (pm + qm).reshape(16, 8, 128)
            up_scr[T] = p - q
            up_scr[2 + T] = pm - qm
        s_e = jnp.sum((ue_r[:, :128] + ue_r[:, 128:]) * sgn_m, axis=1, keepdims=True) + nyq
        s_o = jnp.sum((uo_i[:, :128] + uo_i[:, 128:]) * sgn_m, axis=1, keepdims=True)
        z2[1, :, hi, :, 384:512] = rev(up_scr[0], up_scr[1]).reshape(16, 8, 128)
        z2[1, :, hi, :, 256:384] = rev(up_scr[1], s_e + s_o).reshape(16, 8, 128)
        z2[0, :, hi, :, 384:512] = rev(up_scr[2], up_scr[3]).reshape(16, 8, 128)
        z2[0, :, hi, :, 256:384] = rev(up_scr[3], s_e - s_o).reshape(16, 8, 128)

    with scope("s_stage_c"):
        tw0 = inv_twiddles(0)
        for t in range(5):
            a_inv_tile(0, t, tw0, u0)
        jax.lax.fori_loop(0, 8, stage_c2, 0)

    scale = DH ** -0.5
    rows = jax.lax.broadcasted_iota(jnp.int32, (L, L), 0)
    cols = jax.lax.broadcasted_iota(jnp.int32, (L, L), 1)
    mask = (rows < M) | (rows >= cols)
    wo32 = wo_v.bitcast(u32)

    def qkv_head(h, hd):
        return tuple(jnp.dot(h, pltpu.bitcast(wqkv[3 * hd + j], bf16), preferred_element_type=f32)
                     for j in range(3))

    def scores(qkv):
        return jax.lax.dot_general(qkv[0], qkv[1].astype(bf16), nt_dims, preferred_element_type=f32)

    def softmax(s):
        s = jnp.where(mask, s * scale, -1e9)
        m = jnp.max(s, axis=-1, keepdims=True)
        p = jnp.exp(s - m)
        l = jnp.sum(p, axis=-1, keepdims=True)
        return p / l

    def pv(p, qkv):
        return jnp.dot(p, qkv[2].astype(bf16), preferred_element_type=f32)

    def cp_out(seg0, nseg):
        r0 = pl.multiple_of(seg0 * SEG, SEG)
        return pltpu.make_async_copy(out_v.at[pl.ds(r0, nseg * SEG)], out_hbm.at[pl.ds(r0, nseg * SEG)], sem_out)

    def mix(seg):
        r0 = pl.multiple_of(seg * SEG, SEG)
        xs = x_v[pl.ds(r0, SEG), :].astype(f32)
        gate = jax.nn.sigmoid(jnp.sum(xs * gw_row[...], axis=-1, keepdims=True))
        s2 = seg // 4
        hi0 = (seg % 4) * 4
        b = jnp.concatenate([z2[0, s2, pl.ds(hi0, 4), :, 0:512].reshape(SEG, 512),
                             z2[1, s2, pl.ds(hi0, 4), :, 0:512].reshape(SEG, 512)], axis=1)
        res = gate * a_scr[...] + (1.0 - gate) * b
        out_v[pl.ds(r0, SEG), :] = res.astype(out_v.dtype)

    HA = HA_K

    def wo_part(h0, h1, n, lhs):
        w = pltpu.bitcast(wo32[n, h0 * (DH // 2):h1 * (DH // 2), :], bf16)
        return jnp.dot(lhs, w, preferred_element_type=f32)

    def step(s, mem, first=False):
        r0 = s * SEG if first else pl.multiple_of(s * SEG, SEG)
        xs = x_v[pl.ds(r0, SEG), :].astype(f32)
        h = jnp.concatenate([mem, xs], axis=0)
        qkvs, sc, ps, oh = {}, {}, {}, {}

        def wo_a(n):
            if first:
                cp_wo(n).wait()
            wa_scr[:, n * 128:(n + 1) * 128] = wo_part(0, HA, n, oa)

        for i in range(3):
            qkvs[i] = qkv_head(h, i)
        sc[0] = scores(qkvs[0])
        sc[1] = scores(qkvs[1])
        ps[0] = softmax(sc.pop(0))
        if not first:
            mix(s - 1)
        for hd in range(H):
            if hd + 3 < H:
                qkvs[hd + 3] = qkv_head(h, hd + 3)
            for n in SCHED.get((hd, 0), ()):
                wo_a(n)
            if hd + 2 < H:
                sc[hd + 2] = scores(qkvs[hd + 2])
            if hd + 1 < H:
                ps[hd + 1] = softmax(sc.pop(hd + 1))
            oh[hd] = pv(ps.pop(hd), qkvs.pop(hd))
            if hd == HA - 1:
                oa = jnp.concatenate([oh.pop(i) for i in range(HA)], axis=1)
            for n in SCHED.get((hd, 1), ()):
                wo_a(n)
        ob = jnp.concatenate([oh.pop(i) for i in range(HA, H)], axis=1)
        out = wa_scr[...] + jnp.concatenate([wo_part(HA, H, n, ob) for n in range(8)], axis=1)
        a_scr[...] = out[M:]
        if not first:
            @pl.when(s % 3 == 0)
            def _():
                cp_out(s - 3, 3).start()

        return out[:M].astype(bf16).astype(f32)

    with scope('s_main'):
        mem1 = step(0, mem_ref[...].astype(f32), first=True)
        jax.lax.fori_loop(1, NSTEP, step, mem1, unroll=UNROLL)
    mix(NSTEP - 1)
    last = ((NSTEP - 1) // 3) * 3
    cp_out(last, NSTEP - last).start()
    pltpu.make_async_copy(out_v.at[pl.ds(0, NSTEP * SEG)], out_hbm.at[pl.ds(0, NSTEP * SEG)], sem_out).wait()


@jax.jit
def _run(A_x, A_mem0, A_Wq, A_Wk, A_Wv, A_Wo, B_w_r, B_w_i, gate_w):
    any_spec = pl.BlockSpec(memory_space=pl.ANY)
    out = pl.pallas_call(
        _kernel,
        out_shape=jax.ShapeDtypeStruct((S_LEN, DM), A_x.dtype),
        in_specs=[any_spec] * 15,
        out_specs=any_spec,
        scratch_shapes=[
            pltpu.VMEM((M, DM), bf16),
            pltpu.VMEM((1, DM), bf16),
            pltpu.VMEM((1, DM), f32),
            pltpu.VMEM((2, 16, 8, 128), f32),
            pltpu.SMEM((512,), f32),
            pltpu.VMEM((4, 128, 128), f32),
            pltpu.VMEM((32, 128), f32),
            pltpu.VMEM((2, 128, 128), f32),
            pltpu.VMEM((S_LEN, DM), bf16),
            pltpu.VMEM((8, 128, 128), u32),
            pltpu.VMEM((DM // 2, S_LEN), bf16),
            pltpu.VMEM((DM // 2, S_LEN), bf16),
            pltpu.VMEM((1, S_LEN), bf16),
            pltpu.VMEM((1, S_LEN), bf16),
            pltpu.VMEM((2, 16, 16, 8, 640), f32),
            pltpu.VMEM((3 * H, DM // 2, DH), u32),
            pltpu.VMEM((8, H * DH, 128), bf16),
            pltpu.VMEM((2, 16, 16, 8, 640), f32),
            pltpu.VMEM((2, 16, 16, 8, 640), f32),
            pltpu.VMEM((16, 8, 1152), f32),
            pltpu.VMEM((16, 8, 1152), f32),
            pltpu.VMEM((2, 2, 4, 4, 8, 128), f32),
            pltpu.VMEM((4, 128, 128), f32),
            pltpu.VMEM((L, DM), f32),
            pltpu.VMEM((SEG, DM), f32),
            pltpu.VMEM((S_LEN, DM), bf16),
            pltpu.SemaphoreType.DMA((8,)),
            pltpu.SemaphoreType.DMA(()),
            pltpu.SemaphoreType.DMA((7,)),
            pltpu.SemaphoreType.DMA((4,)),
            pltpu.SemaphoreType.DMA((3 * H,)),
            pltpu.SemaphoreType.DMA((8,)),
            pltpu.SemaphoreType.DMA(()),
        ],
        compiler_params=pltpu.CompilerParams(vmem_limit_bytes=124 * 1024 * 1024),
    )(A_x.reshape(S_LEN, DM), A_mem0.reshape(M, DM),
      A_Wq.reshape(512, 64, DH), A_Wk.reshape(512, 64, DH), A_Wv.reshape(512, 64, DH),
      A_Wo.reshape(H * DH, DM), B_w_r.T, B_w_i.T, gate_w.reshape(1, DM),
      _CS, _TWB, _TWS, _SMALL, _TW, _PERM)
    return out.reshape(A_x.shape)


def pallas_gated_mix__memory_aug_recurrent_mem_tr__spectral_gfnet__prompt_kernel(
    A_x, A_mem0, A_Wq, A_Wk, A_Wv, A_Wo, A_seg_len, B_x, B_w_r, B_w_i, gate_w,
):
    del B_x
    assert int(A_seg_len) == SEG and A_x.shape == (1, S_LEN, DM)
    return _run(A_x, A_mem0, A_Wq, A_Wk, A_Wv, A_Wo, B_w_r, B_w_i, gate_w)
```

```python
import functools
import contextlib
import numpy as np
import ml_dtypes

import jax
import jax.numpy as jnp
import jax.experimental.pallas as pl
import jax.experimental.pallas.tpu as pltpu

S_LEN, DM, H, DH, M, SEG = 2048, 1024, 32, 128, 8, 32
L = M + SEG
NSEG = S_LEN // SEG
DF = DM // 2 + 1
f32 = jnp.float32
bf16 = jnp.bfloat16
u32 = jnp.uint32
NSTEP = 64
SCOPES = 0
UNROLL = 3
WO0 = 2
HA_K = 27
SCHED_ID = 4
_SCHEDS = [
    {(28, 0): (0,), (28, 1): (1, 2, 3), (29, 1): (4, 5), (31, 1): (6, 7)},
    {(28, 0): (0,), (28, 1): (1, 2), (29, 1): (3, 4), (30, 1): (5, 6), (31, 1): (7,)},
    {(28, 1): (0, 1), (29, 1): (2, 3), (30, 1): (4, 5), (31, 1): (6, 7)},
    {(28, 0): (0,), (29, 0): (1, 2), (30, 0): (3, 4), (31, 0): (5, 6), (31, 1): (7,)},
    {(28, 1): (0,), (29, 0): (1,), (29, 1): (2, 3), (30, 1): (4, 5, 6), (31, 1): (7,)},
    {(29, 0): (0, 1), (29, 1): (2, 3), (30, 1): (4, 5), (31, 1): (6, 7)},
]
SCHED = _SCHEDS[SCHED_ID]


def scope(n):
    return jax.named_scope(n) if SCOPES else contextlib.nullcontext()


def _bf16_np(a):
    return np.asarray(a, np.float32).astype(ml_dtypes.bfloat16)


def _pack_rows_u32(a):
    b = _bf16_np(a).view(np.uint16).astype(np.uint32)
    return b[0::2] | (b[1::2] << 16)


def _make_consts():
    q = np.arange(DM // 4)
    th = 2.0 * np.pi / DM
    a0 = th * ((2 * np.outer(q, q)) % DM)
    a1 = th * ((np.outer(q, 2 * q + 1)) % DM)
    s1f = -np.sin(a1)
    s1f[0, :] = -np.cos(np.pi * q)
    mperm = 16 * (q // 16) + ((q % 16) >> 1) + 8 * (q & 1)
    fwd = [np.cos(a0), np.cos(a1), -np.sin(a0), s1f]
    cs = np.stack([_pack_rows_u32(m[:, mperm]) for m in fwd])
    cs = np.ascontiguousarray(cs.reshape(4, 128, 2, 128).transpose(0, 2, 1, 3)).reshape(8, 128, 128)

    i16 = np.arange(16)
    i128 = np.arange(128)
    d128 = np.exp(-2j * np.pi * ((np.outer(i128, i128)) % 128) / 128.0)
    dc = np.conj(d128)
    small = np.stack([d128.real, d128.imag]).astype(np.float32)
    tw_f = np.exp(-2j * np.pi * np.outer(i16, i128) / 2048.0)
    tw = np.concatenate([tw_f.real, tw_f.imag]).astype(np.float32)
    twb = np.exp(2j * np.pi * np.outer(i16, np.arange(8)) / 2048.0)
    tws = np.exp(2j * np.pi * 8 * np.outer(i16, i16) / 2048.0)
    tws = np.concatenate([tws.real.reshape(-1), tws.imag.reshape(-1),
                          twb.real.reshape(-1), twb.imag.reshape(-1)]).astype(np.float32)
    return cs, tws, small, tw


_CS, _TWS, _SMALL, _TW = _make_consts()
NU = 16


def _lo_pair(a, b):
    return (a & np.uint32(0xFFFF)) | (b << 16)


def _hi_pair(a, b):
    return (a >> 16) | (b & np.uint32(0xFFFF0000))


def _cmul_const(x, c):
    re, im = x
    cr, ci = float(np.real(c)), float(np.imag(c))
    if abs(ci) < 1e-9:
        return (re, im) if cr > 0 else (-re, -im)
    if abs(cr) < 1e-9:
        return (-im, re) if ci > 0 else (im, -re)
    if abs(abs(cr) - abs(ci)) < 1e-9:
        a = abs(cr)
        sr, si = (1.0 if cr > 0 else -1.0), (1.0 if ci > 0 else -1.0)
        nr = (re if sr > 0 else -re) - (im if si > 0 else -im)
        ni = (re if si > 0 else -re) + (im if sr > 0 else -im)
        return (nr * a, ni * a)
    return (re * cr - im * ci, re * ci + im * cr)


def _dft4(x, sign):
    (ar, ai), (br, bi), (cr, ci), (dr, di) = x
    s0r, s0i = ar + cr, ai + ci
    s1r, s1i = ar - cr, ai - ci
    s2r, s2i = br + dr, bi + di
    s3r, s3i = br - dr, bi - di
    if sign < 0:
        return [(s0r + s2r, s0i + s2i), (s1r + s3i, s1i - s3r), (s0r - s2r, s0i - s2i), (s1r - s3i, s1i + s3r)]
    return [(s0r + s2r, s0i + s2i), (s1r - s3i, s1i + s3r), (s0r - s2r, s0i - s2i), (s1r + s3i, s1i - s3r)]


def _dft16(x, sign):
    w = np.exp(sign * 2j * np.pi / 16.0)
    t = [[None] * 4 for _ in range(4)]
    for b in range(4):
        col = _dft4([x[4 * a + b] for a in range(4)], sign)
        for c in range(4):
            t[b][c] = col[c] if b * c == 0 else _cmul_const(col[c], w ** (b * c))
    out = [None] * 16
    for c in range(4):
        row = _dft4([t[b][c] for b in range(4)], sign)
        for d in range(4):
            out[c + 4 * d] = row[d]
    return out


def _kernel(x_hbm, mem_hbm, wq_hbm, wk_hbm, wv_hbm, wo_hbm, wr_hbm, wi_hbm, gw_hbm,
            cs_hbm, tws_hbm, small_hbm, tw_hbm,
            out_hbm,
            mem_ref, gw_ref, gw_row, twb_ref, tws_ref, small_ref, tw_ref, perm_ref,
            x_v, cs_v, wrt_v, wit_v, wrn_v, win_v, wp_v, wqkv, wo_v, z1, z2, u0, u1, bt_scr, up_scr, wa_scr, a_scr, out_v,
            sem_x, sem_c, sem_s, sem_in, sem_w, sem_wo, sem_out):
    w32_hbm = tuple(w.bitcast(u32) for w in (wq_hbm, wk_hbm, wv_hbm))
    nt_dims = (((1,), (1,)), ((), ()))

    def cp_x(i):
        r0 = pl.multiple_of(i * 256, 256)
        return pltpu.make_async_copy(x_hbm.at[pl.ds(r0, 256)], x_v.at[pl.ds(r0, 256)], sem_x.at[i])

    cp_cs = pltpu.make_async_copy(cs_hbm, cs_v, sem_c)
    cp_wt = []
    for i, (src, dst, dstn) in enumerate(((wr_hbm, wrt_v, wrn_v), (wi_hbm, wit_v, win_v))):
        cp_wt.append(pltpu.make_async_copy(src.at[pl.ds(0, 512)], dst, sem_in.at[2 * i]))
        cp_wt.append(pltpu.make_async_copy(src.at[pl.ds(512, 1)], dstn, sem_in.at[2 * i + 1]))

    def cp_wo(n):
        return pltpu.make_async_copy(wo_hbm.at[:, pl.ds(n * 128, 128)], wo_v.at[n], sem_wo.at[n])

    def cp_w(p, par, which):
        t = 2 * p + par
        return pltpu.make_async_copy(w32_hbm[which].at[:, par * 16 + p], wqkv.at[3 * t + which],
                                     sem_w.at[3 * t + which])

    def unit_start(p):
        for par in range(2):
            for which in range(3):
                cp_w(p, par, which).start()

    def unit_repack(p, rr=range(0, 512, 64), wait=True):
        if wait:
            for par in range(2):
                for which in range(3):
                    cp_w(p, par, which).wait()
        for which in range(3):
            ta = 6 * p + which
            tb = 6 * p + 3 + which
            for r in rr:
                a = wqkv[ta, r:r + 64, :]
                b = wqkv[tb, r:r + 64, :]
                wqkv[ta, r:r + 64, :] = _lo_pair(a, b)
                wqkv[tb, r:r + 64, :] = _hi_pair(a, b)

    C0, C1, S0, S1F = range(4)

    def qdot(lhs, mat, nt):
        return jnp.dot(lhs, pltpu.bitcast(cs_v[2 * mat + nt], bf16), preferred_element_type=f32)

    def qdot_t(lhs, mat, dt):
        rows = jnp.concatenate([cs_v[2 * mat + kt, dt * 64:(dt + 1) * 64, :] for kt in range(2)], axis=1)
        return jax.lax.dot_general(lhs, pltpu.bitcast(rows, bf16), nt_dims, preferred_element_type=f32)

    def rev(t, first):
        return jnp.where(lane0, first, jnp.dot(t, perm_ref[1], preferred_element_type=f32))

    cp_small = [pltpu.make_async_copy(src, dst, sem_s.at[i]) for i, (src, dst) in enumerate((
        (tws_hbm, tws_ref), (small_hbm, small_ref.at[pl.ds(0, 2)]), (tw_hbm, tw_ref),
        (mem_hbm, mem_ref), (gw_hbm, gw_ref)))]
    cp_cs.start()
    cp_x(0).start()
    cp_x(1).start()
    for cp in cp_small:
        cp.start()
    ri = jax.lax.broadcasted_iota(jnp.int32, (128, 128), 0)
    ci = jax.lax.broadcasted_iota(jnp.int32, (128, 128), 1)
    perm_ref[0] = (ci == (ri >> 3) + 16 * (ri & 7)).astype(f32)
    perm_ref[1] = ((ri + ci == 128) & (ci >= 1)).astype(f32)

    lane_i = jax.lax.broadcasted_iota(jnp.int32, (1, 128), 1)
    lane0 = lane_i == 0
    sgn = (1 - 2 * (lane_i & 1)).astype(f32)
    sgn_m = (1 - 2 * ((lane_i >> 1) & 1)).astype(f32)

    def pro1(c, first):
        @pl.when(c < 3)
        def _():
            cp_x(2 * c + 2).start()
            cp_x(2 * c + 3).start()

        @pl.when(c == 3)
        def _():
            for cp in cp_wt:
                cp.start()

        @pl.when(c >= 4)
        def _():
            unit_start(c - 4)

        cp_x(c).wait()
        if first:
            cp_cs.wait()
        r0 = pl.multiple_of(c * 256, 256)
        xt = [x_v[pl.ds(r0, 256), j * 128:(j + 1) * 128].astype(f32) for j in range(8)]
        zero = jnp.zeros((256, 128), f32)
        r1 = [rev(xt[7], zero), rev(xt[6], xt[7])]
        r2 = [rev(xt[3], zero), rev(xt[2], xt[3])]
        ee, eo, oe, oo = [], [], [], []
        for T in range(2):
            e1, o1 = xt[T] + r1[T], xt[T] - r1[T]
            e2, o2 = r2[T] + xt[4 + T], r2[T] - xt[4 + T]
            ee.append(e1 + e2)
            eo.append(e1 - e2)
            oe.append(o1 - o2)
            oo.append(o1 + o2)
        oo[0] = jnp.where(lane0, xt[2] - xt[6], oo[0])
        e256 = (xt[2] + xt[6])[:, 0:1]
        mid = jnp.broadcast_to(e256, (256, 128)) * sgn_m
        nyq = jnp.sum((ee[0] + ee[1]) * sgn, axis=1, keepdims=True) + e256
        ee, eo, oe, oo = (jnp.concatenate(v, axis=1) for v in (ee, eo, oe, oo))
        rr = pl.ds(2 * c, 2)
        for t in range(2):
            z1[0, rr, :, :, t * 128:(t + 1) * 128] = (qdot(ee, C0, t) + mid).reshape(2, 16, 8, 128)
            z1[0, rr, :, :, (2 + t) * 128:(3 + t) * 128] = qdot(eo, C1, t).reshape(2, 16, 8, 128)
            z1[1, rr, :, :, t * 128:(t + 1) * 128] = qdot(oe, S0, t).reshape(2, 16, 8, 128)
            z1[1, rr, :, :, (2 + t) * 128:(3 + t) * 128] = qdot(oo, S1F, t).reshape(2, 16, 8, 128)
        z1[0, rr, :, :, 512:640] = jnp.where(lane0, nyq, 0.0).reshape(2, 16, 8, 128)
        z1[1, rr, :, :, 512:640] = jnp.zeros((2, 16, 8, 128), f32)

    with scope("s_pro1"):
        pro1(0, True)
        jax.lax.fori_loop(1, 8, lambda c, carry: (pro1(c, False), carry)[1], 0)

    def stage_a(hi):
        for t in range(5):
            sl = slice(t * 128, (t + 1) * 128)
            xin = [(z1[0, s2, hi, :, sl], z1[1, s2, hi, :, sl]) for s2 in range(16)]
            xo = _dft16(xin, -1)
            for k2 in range(16):
                z2[0, k2, hi, :, sl] = xo[k2][0]
                z2[1, k2, hi, :, sl] = xo[k2][1]

    norm = 1.0 / (S_LEN * DM)
    cscale = [jnp.where(lane0, norm, 2.0 * norm).astype(f32)] + [2.0 * norm] * 3 + [norm]

    def wperm(c, carry):
        @pl.when(c % 3 == 0)
        def _():
            unit_start(6 + c // 3)

        for bb in range(2):
            blk_i = 2 * c + bb
            l0 = pl.multiple_of(blk_i * 128, 128)
            for i, (wt, wn) in enumerate(((wrt_v.bitcast(u32), wrn_v), (wit_v.bitcast(u32), win_v))):
                for t in range(5):
                    if t < 4:
                        w = wt[(t % 2) * 128:(t % 2 + 1) * 128, pl.ds(l0, 128)].reshape(8, 16, 128)
                        pk = (_lo_pair if t < 2 else _hi_pair)(w[:, :8, :], w[:, 8:, :])
                        blk = pltpu.bitcast(pk.reshape(64, 128), bf16)
                    else:
                        blk = jnp.broadcast_to(wn[:, pl.ds(l0, 128)], (128, 128))
                    o = jax.lax.dot_general(perm_ref[0], blk, nt_dims, preferred_element_type=f32)
                    wp_v[i, :, blk_i, :, t * 128:(t + 1) * 128] = (o * cscale[t]).reshape(16, 8, 128)
        return carry

    def stage_a_loop(hi, carry):
        @pl.when(hi % 8 == 0)
        def _():
            unit_start(4 + hi // 8)

        stage_a(hi)
        return carry

    with scope("s_stage_a"):
        for cp in cp_small:
            cp.wait()
        small_ref[2] = small_ref[0] - small_ref[1]
        small_ref[3] = -small_ref[1] - small_ref[0]
        sub = jax.lax.broadcasted_iota(jnp.int32, (8, 128), 0)
        for part in range(2):
            for k2 in range(1, 16):
                v = jnp.zeros((8, 128), f32)
                for j in range(8):
                    v = jnp.where(sub == j, tws_ref[512 + part * 128 + k2 * 8 + j], v)
                twb_ref[part, k2] = v
        gw_row[...] = gw_ref[...].astype(f32)
        jax.lax.fori_loop(0, 16, stage_a_loop, 0)

    with scope("s_wperm"):
        for cp in cp_wt:
            cp.wait()
        jax.lax.fori_loop(0, 8, wperm, 0)

    def cdot3(m1, m2, m3, zr, zi):
        k1 = jnp.dot(m1, (zr + zi).astype(bf16), preferred_element_type=f32)
        k2 = jnp.dot(m2, zi.astype(bf16), preferred_element_type=f32)
        k3 = jnp.dot(m3, zr.astype(bf16), preferred_element_type=f32)
        return k1 - k2, k1 + k3

    def b_fwd(k2):
        tr, ti = tw_ref[pl.ds(k2, 1), :], tw_ref[pl.ds(16 + k2, 1), :]
        mr = small_ref[0] * tr - small_ref[1] * ti
        mi = small_ref[0] * ti + small_ref[1] * tr
        return cdot3(mr, mr + mi, mi - mr, z2[0, k2].reshape(128, 640), z2[1, k2].reshape(128, 640))

    def b_inv(k2, x):
        xr, xi = x
        wr = wp_v[0, k2].reshape(128, 640)
        wi = wp_v[1, k2].reshape(128, 640)
        pr = xr * wr - xi * wi
        pi = xr * wi + xi * wr
        gr, gi = cdot3(small_ref[0], small_ref[2], small_ref[3], pr, pi)
        z1[0, k2] = gr.reshape(16, 8, 640)
        z1[1, k2] = gi.reshape(16, 8, 640)

    def stage_b2(j, carry):
        @pl.when(j < 7)
        def _():
            unit_start(9 + j)

        xa = b_fwd(2 * j)
        xb = b_fwd(2 * j + 1)
        b_inv(2 * j, xa)
        b_inv(2 * j + 1, xb)
        return carry

    with scope('s_stage_b'):
        jax.lax.fori_loop(0, 8, stage_b2, 0)

    lane0a = jax.lax.broadcasted_iota(jnp.int32, (8, 128), 1) == 0

    def inv_twiddles(hi):
        tw_inv = [None]
        for k2 in range(1, 16):
            cr, ci = tws_ref[hi * 16 + k2], tws_ref[256 + hi * 16 + k2]
            br, bi = twb_ref[0, k2], twb_ref[1, k2]
            tw_inv.append((br * cr - bi * ci, br * ci + bi * cr))
        return tw_inv

    def a_inv_tile(hi, t, tw_inv, u_dst):
        sl = slice(t * 128, (t + 1) * 128)
        w = np.exp(2j * np.pi / 16.0)
        tmp = bt_scr.at[t % 2]
        for b in range(4):
            xin = []
            for a in range(4):
                k2 = 4 * a + b
                gr, gi = z1[0, k2, hi, :, sl], z1[1, k2, hi, :, sl]
                if k2 > 0:
                    tr, ti = tw_inv[k2]
                    gr, gi = gr * tr - gi * ti, gr * ti + gi * tr
                xin.append((gr, gi))
            col = _dft4(xin, +1)
            for c in range(4):
                v = col[c] if b * c == 0 else _cmul_const(col[c], w ** (b * c))
                tmp[0, b, c] = v[0]
                tmp[1, b, c] = v[1]
        for c in range(4):
            row = _dft4([(tmp[0, b, c], tmp[1, b, c]) for b in range(4)], +1)
            for d in range(4):
                s2 = c + 4 * d
                u_dst[s2, :, sl] = row[d][0]
                if t < 4:
                    u_dst[s2, :, 640 + t * 128:640 + (t + 1) * 128] = row[d][1]

    def stage_c2(m, carry):
        @pl.when(jnp.logical_and(m >= WO0, m < WO0 + 4))
        def _():
            cp_wo(2 * (m - WO0)).start()
            cp_wo(2 * (m - WO0) + 1).start()

        stage_c(2 * m, 2 * m + 1, u0, u1)
        stage_c(2 * m + 1, jnp.minimum(2 * m + 2, 15), u1, u0)
        return carry

    def stage_c(hi, nxt, u_src, u_dst):
        tw_inv = inv_twiddles(nxt)
        unit_repack(hi)
        for t in range(5):
            a_inv_tile(nxt, t, tw_inv, u_dst)
        nyq = u_src[:, :, 512:513].reshape(128, 1)
        n = jnp.broadcast_to(nyq, (128, 128)) * sgn
        ue_r = u_src[:, :, 0:256].reshape(128, 256)
        uo_r = u_src[:, :, 256:512].reshape(128, 256)
        ue_i = u_src[:, :, 640:896].reshape(128, 256)
        uo_i = u_src[:, :, 896:1152].reshape(128, 256)
        for T in range(2):
            a0 = qdot_t(ue_r, C0, T) + n
            a1 = qdot_t(uo_r, C1, T)
            b0 = qdot_t(ue_i, S0, T)
            b1 = qdot_t(uo_i, S1F, T)
            if T == 0:
                b1 = jnp.where(lane0, 0.0, b1)
            p, q, pm, qm = a0 + a1, b0 + b1, a0 - a1, b0 - b1
            z2[0, :, hi, :, T * 128:(T + 1) * 128] = (p + q).reshape(16, 8, 128)
            z2[1, :, hi, :, T * 128:(T + 1) * 128] = (pm + qm).reshape(16, 8, 128)
            up_scr[T] = p - q
            up_scr[2 + T] = pm - qm
        s_e = jnp.sum((ue_r[:, :128] + ue_r[:, 128:]) * sgn_m, axis=1, keepdims=True) + nyq
        s_o = jnp.sum((uo_i[:, :128] + uo_i[:, 128:]) * sgn_m, axis=1, keepdims=True)
        z2[1, :, hi, :, 384:512] = rev(up_scr[0], up_scr[1]).reshape(16, 8, 128)
        z2[1, :, hi, :, 256:384] = rev(up_scr[1], s_e + s_o).reshape(16, 8, 128)
        z2[0, :, hi, :, 384:512] = rev(up_scr[2], up_scr[3]).reshape(16, 8, 128)
        z2[0, :, hi, :, 256:384] = rev(up_scr[3], s_e - s_o).reshape(16, 8, 128)

    with scope("s_stage_c"):
        tw0 = inv_twiddles(0)
        for t in range(5):
            a_inv_tile(0, t, tw0, u0)
        jax.lax.fori_loop(0, 8, stage_c2, 0)

    scale = DH ** -0.5
    rows = jax.lax.broadcasted_iota(jnp.int32, (L, L), 0)
    cols = jax.lax.broadcasted_iota(jnp.int32, (L, L), 1)
    mask = (rows < M) | (rows >= cols)
    wo32 = wo_v.bitcast(u32)

    def qkv_head(h, hd):
        return tuple(jnp.dot(h, pltpu.bitcast(wqkv[3 * hd + j], bf16), preferred_element_type=f32)
                     for j in range(3))

    def scores(qkv):
        return jax.lax.dot_general(qkv[0], qkv[1].astype(bf16), nt_dims, preferred_element_type=f32)

    def softmax(s):
        s = jnp.where(mask, s * scale, -1e9)
        m = jnp.max(s, axis=-1, keepdims=True)
        p = jnp.exp(s - m)
        l = jnp.sum(p, axis=-1, keepdims=True)
        return p / l

    def pv(p, qkv):
        return jnp.dot(p, qkv[2].astype(bf16), preferred_element_type=f32)

    def cp_out(seg0, nseg):
        r0 = pl.multiple_of(seg0 * SEG, SEG)
        return pltpu.make_async_copy(out_v.at[pl.ds(r0, nseg * SEG)], out_hbm.at[pl.ds(r0, nseg * SEG)], sem_out)

    def mix(seg):
        r0 = pl.multiple_of(seg * SEG, SEG)
        xs = x_v[pl.ds(r0, SEG), :].astype(f32)
        gate = jax.nn.sigmoid(jnp.sum(xs * gw_row[...], axis=-1, keepdims=True))
        s2 = seg // 4
        hi0 = (seg % 4) * 4
        b = jnp.concatenate([z2[0, s2, pl.ds(hi0, 4), :, 0:512].reshape(SEG, 512),
                             z2[1, s2, pl.ds(hi0, 4), :, 0:512].reshape(SEG, 512)], axis=1)
        res = gate * a_scr[...] + (1.0 - gate) * b
        out_v[pl.ds(r0, SEG), :] = res.astype(out_v.dtype)

    HA = HA_K

    def wo_part(h0, h1, n, lhs):
        w = pltpu.bitcast(wo32[n, h0 * (DH // 2):h1 * (DH // 2), :], bf16)
        return jnp.dot(lhs, w, preferred_element_type=f32)

    def step(s, mem, first=False):
        r0 = s * SEG if first else pl.multiple_of(s * SEG, SEG)
        xs = x_v[pl.ds(r0, SEG), :].astype(f32)
        h = jnp.concatenate([mem, xs], axis=0)
        qkvs, sc, ps, oh = {}, {}, {}, {}

        def wo_a(n):
            if first:
                cp_wo(n).wait()
            wa_scr[:, n * 128:(n + 1) * 128] = wo_part(0, HA, n, oa)

        for i in range(3):
            qkvs[i] = qkv_head(h, i)
        sc[0] = scores(qkvs[0])
        sc[1] = scores(qkvs[1])
        ps[0] = softmax(sc.pop(0))
        if not first:
            mix(s - 1)
        for hd in range(H):
            if hd + 3 < H:
                qkvs[hd + 3] = qkv_head(h, hd + 3)
            for n in SCHED.get((hd, 0), ()):
                wo_a(n)
            if hd + 2 < H:
                sc[hd + 2] = scores(qkvs[hd + 2])
            if hd + 1 < H:
                ps[hd + 1] = softmax(sc.pop(hd + 1))
            oh[hd] = pv(ps.pop(hd), qkvs.pop(hd))
            if hd == HA - 1:
                oa = jnp.concatenate([oh.pop(i) for i in range(HA)], axis=1)
            for n in SCHED.get((hd, 1), ()):
                wo_a(n)
        ob = jnp.concatenate([oh.pop(i) for i in range(HA, H)], axis=1)
        out = wa_scr[...] + jnp.concatenate([wo_part(HA, H, n, ob) for n in range(8)], axis=1)
        a_scr[...] = out[M:]
        if not first:
            @pl.when(s % 3 == 0)
            def _():
                cp_out(s - 3, 3).start()

        return out[:M].astype(bf16).astype(f32)

    with scope('s_main'):
        mem1 = step(0, mem_ref[...].astype(f32), first=True)
        jax.lax.fori_loop(1, NSTEP, step, mem1, unroll=UNROLL)
    mix(NSTEP - 1)
    last = ((NSTEP - 1) // 3) * 3
    cp_out(last, NSTEP - last).start()
    pltpu.make_async_copy(out_v.at[pl.ds(0, NSTEP * SEG)], out_hbm.at[pl.ds(0, NSTEP * SEG)], sem_out).wait()


@jax.jit
def _run(A_x, A_mem0, A_Wq, A_Wk, A_Wv, A_Wo, B_w_r, B_w_i, gate_w):
    any_spec = pl.BlockSpec(memory_space=pl.ANY)
    out = pl.pallas_call(
        _kernel,
        out_shape=jax.ShapeDtypeStruct((S_LEN, DM), A_x.dtype),
        in_specs=[any_spec] * 13,
        out_specs=any_spec,
        scratch_shapes=[
            pltpu.VMEM((M, DM), bf16),
            pltpu.VMEM((1, DM), bf16),
            pltpu.VMEM((1, DM), f32),
            pltpu.VMEM((2, 16, 8, 128), f32),
            pltpu.SMEM((768,), f32),
            pltpu.VMEM((4, 128, 128), f32),
            pltpu.VMEM((32, 128), f32),
            pltpu.VMEM((2, 128, 128), f32),
            pltpu.VMEM((S_LEN, DM), bf16),
            pltpu.VMEM((8, 128, 128), u32),
            pltpu.VMEM((DM // 2, S_LEN), bf16),
            pltpu.VMEM((DM // 2, S_LEN), bf16),
            pltpu.VMEM((1, S_LEN), bf16),
            pltpu.VMEM((1, S_LEN), bf16),
            pltpu.VMEM((2, 16, 16, 8, 640), f32),
            pltpu.VMEM((3 * H, DM // 2, DH), u32),
            pltpu.VMEM((8, H * DH, 128), bf16),
            pltpu.VMEM((2, 16, 16, 8, 640), f32),
            pltpu.VMEM((2, 16, 16, 8, 640), f32),
            pltpu.VMEM((16, 8, 1152), f32),
            pltpu.VMEM((16, 8, 1152), f32),
            pltpu.VMEM((2, 2, 4, 4, 8, 128), f32),
            pltpu.VMEM((4, 128, 128), f32),
            pltpu.VMEM((L, DM), f32),
            pltpu.VMEM((SEG, DM), f32),
            pltpu.VMEM((S_LEN, DM), bf16),
            pltpu.SemaphoreType.DMA((8,)),
            pltpu.SemaphoreType.DMA(()),
            pltpu.SemaphoreType.DMA((5,)),
            pltpu.SemaphoreType.DMA((4,)),
            pltpu.SemaphoreType.DMA((3 * H,)),
            pltpu.SemaphoreType.DMA((8,)),
            pltpu.SemaphoreType.DMA(()),
        ],
        compiler_params=pltpu.CompilerParams(vmem_limit_bytes=124 * 1024 * 1024),
    )(A_x.reshape(S_LEN, DM), A_mem0.reshape(M, DM),
      A_Wq.reshape(512, 64, DH), A_Wk.reshape(512, 64, DH), A_Wv.reshape(512, 64, DH),
      A_Wo.reshape(H * DH, DM), B_w_r.T, B_w_i.T, gate_w.reshape(1, DM),
      _CS, _TWS, _SMALL, _TW)
    return out.reshape(A_x.shape)


def pallas_gated_mix__memory_aug_recurrent_mem_tr__spectral_gfnet__prompt_kernel(
    A_x, A_mem0, A_Wq, A_Wk, A_Wv, A_Wo, A_seg_len, B_x, B_w_r, B_w_i, gate_w,
):
    del B_x
    assert int(A_seg_len) == SEG and A_x.shape == (1, S_LEN, DM)
    return _run(A_x, A_mem0, A_Wq, A_Wk, A_Wv, A_Wo, B_w_r, B_w_i, gate_w)
```

```python
import numpy as np
import ml_dtypes

import jax
import jax.numpy as jnp
import jax.experimental.pallas as pl
import jax.experimental.pallas.tpu as pltpu

S_LEN, DM, H, DH, M, SEG = 2048, 1024, 32, 128, 8, 32
L = M + SEG
NSEG = S_LEN // SEG
DF = DM // 2 + 1
f32 = jnp.float32
bf16 = jnp.bfloat16
u32 = jnp.uint32
UNROLL = 3
HA = 27
WO_SCHED = {(28, 1): (0,), (29, 0): (1,), (29, 1): (2, 3), (30, 1): (4, 5, 6), (31, 1): (7,)}


def _bf16_np(a):
    return np.asarray(a, np.float32).astype(ml_dtypes.bfloat16)


def _pack_rows_u32(a):
    b = _bf16_np(a).view(np.uint16).astype(np.uint32)
    return b[0::2] | (b[1::2] << 16)


def _make_consts():
    q = np.arange(DM // 4)
    th = 2.0 * np.pi / DM
    a0 = th * ((2 * np.outer(q, q)) % DM)
    a1 = th * ((np.outer(q, 2 * q + 1)) % DM)
    s1f = -np.sin(a1)
    s1f[0, :] = -np.cos(np.pi * q)
    mperm = 16 * (q // 16) + ((q % 16) >> 1) + 8 * (q & 1)
    fwd = [np.cos(a0), np.cos(a1), -np.sin(a0), s1f]
    cs = np.stack([_pack_rows_u32(m[:, mperm]) for m in fwd])
    cs = np.ascontiguousarray(cs.reshape(4, 128, 2, 128).transpose(0, 2, 1, 3)).reshape(8, 128, 128)

    i16 = np.arange(16)
    i128 = np.arange(128)
    d128 = np.exp(-2j * np.pi * ((np.outer(i128, i128)) % 128) / 128.0)
    dc = np.conj(d128)
    small = np.stack([d128.real, d128.imag]).astype(np.float32)
    tw_f = np.exp(-2j * np.pi * np.outer(i16, i128) / 2048.0)
    tw = np.concatenate([tw_f.real, tw_f.imag]).astype(np.float32)
    twb = np.exp(2j * np.pi * np.outer(i16, np.arange(8)) / 2048.0)
    tws = np.exp(2j * np.pi * 8 * np.outer(i16, i16) / 2048.0)
    tws = np.concatenate([tws.real.reshape(-1), tws.imag.reshape(-1),
                          twb.real.reshape(-1), twb.imag.reshape(-1)]).astype(np.float32)
    return cs, tws, small, tw


_CS, _TWS, _SMALL, _TW = _make_consts()
NU = 16


def _lo_pair(a, b):
    return (a & np.uint32(0xFFFF)) | (b << 16)


def _hi_pair(a, b):
    return (a >> 16) | (b & np.uint32(0xFFFF0000))


def _cmul_const(x, c):
    re, im = x
    cr, ci = float(np.real(c)), float(np.imag(c))
    if abs(ci) < 1e-9:
        return (re, im) if cr > 0 else (-re, -im)
    if abs(cr) < 1e-9:
        return (-im, re) if ci > 0 else (im, -re)
    if abs(abs(cr) - abs(ci)) < 1e-9:
        a = abs(cr)
        sr, si = (1.0 if cr > 0 else -1.0), (1.0 if ci > 0 else -1.0)
        nr = (re if sr > 0 else -re) - (im if si > 0 else -im)
        ni = (re if si > 0 else -re) + (im if sr > 0 else -im)
        return (nr * a, ni * a)
    return (re * cr - im * ci, re * ci + im * cr)


def _dft4(x, sign):
    (ar, ai), (br, bi), (cr, ci), (dr, di) = x
    s0r, s0i = ar + cr, ai + ci
    s1r, s1i = ar - cr, ai - ci
    s2r, s2i = br + dr, bi + di
    s3r, s3i = br - dr, bi - di
    if sign < 0:
        return [(s0r + s2r, s0i + s2i), (s1r + s3i, s1i - s3r), (s0r - s2r, s0i - s2i), (s1r - s3i, s1i + s3r)]
    return [(s0r + s2r, s0i + s2i), (s1r - s3i, s1i + s3r), (s0r - s2r, s0i - s2i), (s1r + s3i, s1i - s3r)]


def _dft16(x, sign):
    w = np.exp(sign * 2j * np.pi / 16.0)
    t = [[None] * 4 for _ in range(4)]
    for b in range(4):
        col = _dft4([x[4 * a + b] for a in range(4)], sign)
        for c in range(4):
            t[b][c] = col[c] if b * c == 0 else _cmul_const(col[c], w ** (b * c))
    out = [None] * 16
    for c in range(4):
        row = _dft4([t[b][c] for b in range(4)], sign)
        for d in range(4):
            out[c + 4 * d] = row[d]
    return out


def _kernel(x_hbm, mem_hbm, wq_hbm, wk_hbm, wv_hbm, wo_hbm, wr_hbm, wi_hbm, gw_hbm,
            cs_hbm, tws_hbm, small_hbm, tw_hbm,
            out_hbm,
            mem_ref, gw_ref, gw_row, twb_ref, tws_ref, small_ref, tw_ref, perm_ref,
            x_v, cs_v, wrt_v, wit_v, wrn_v, win_v, wp_v, wqkv, wo_v, z1, z2, u0, u1, bt_scr, up_scr, wa_scr, a_scr, out_v,
            sem_x, sem_c, sem_s, sem_in, sem_w, sem_wo, sem_out):
    w32_hbm = tuple(w.bitcast(u32) for w in (wq_hbm, wk_hbm, wv_hbm))
    nt_dims = (((1,), (1,)), ((), ()))

    def cp_x(i):
        r0 = pl.multiple_of(i * 256, 256)
        return pltpu.make_async_copy(x_hbm.at[pl.ds(r0, 256)], x_v.at[pl.ds(r0, 256)], sem_x.at[i])

    cp_cs = pltpu.make_async_copy(cs_hbm, cs_v, sem_c)
    cp_wt = []
    for i, (src, dst, dstn) in enumerate(((wr_hbm, wrt_v, wrn_v), (wi_hbm, wit_v, win_v))):
        cp_wt.append(pltpu.make_async_copy(src.at[pl.ds(0, 512)], dst, sem_in.at[2 * i]))
        cp_wt.append(pltpu.make_async_copy(src.at[pl.ds(512, 1)], dstn, sem_in.at[2 * i + 1]))

    def cp_wo(n):
        return pltpu.make_async_copy(wo_hbm.at[:, pl.ds(n * 128, 128)], wo_v.at[n], sem_wo.at[n])

    def cp_w(p, par, which):
        t = 2 * p + par
        return pltpu.make_async_copy(w32_hbm[which].at[:, par * 16 + p], wqkv.at[3 * t + which],
                                     sem_w.at[3 * t + which])

    def unit_start(p):
        for par in range(2):
            for which in range(3):
                cp_w(p, par, which).start()

    def unit_repack(p, rr=range(0, 512, 64), wait=True):
        if wait:
            for par in range(2):
                for which in range(3):
                    cp_w(p, par, which).wait()
        for which in range(3):
            ta = 6 * p + which
            tb = 6 * p + 3 + which
            for r in rr:
                a = wqkv[ta, r:r + 64, :]
                b = wqkv[tb, r:r + 64, :]
                wqkv[ta, r:r + 64, :] = _lo_pair(a, b)
                wqkv[tb, r:r + 64, :] = _hi_pair(a, b)

    C0, C1, S0, S1F = range(4)

    def qdot(lhs, mat, nt):
        return jnp.dot(lhs, pltpu.bitcast(cs_v[2 * mat + nt], bf16), preferred_element_type=f32)

    def qdot_t(lhs, mat, dt):
        rows = jnp.concatenate([cs_v[2 * mat + kt, dt * 64:(dt + 1) * 64, :] for kt in range(2)], axis=1)
        return jax.lax.dot_general(lhs, pltpu.bitcast(rows, bf16), nt_dims, preferred_element_type=f32)

    def rev(t, first):
        return jnp.where(lane0, first, jnp.dot(t, perm_ref[1], preferred_element_type=f32))

    cp_small = [pltpu.make_async_copy(src, dst, sem_s.at[i]) for i, (src, dst) in enumerate((
        (tws_hbm, tws_ref), (small_hbm, small_ref.at[pl.ds(0, 2)]), (tw_hbm, tw_ref),
        (mem_hbm, mem_ref), (gw_hbm, gw_ref)))]
    cp_cs.start()
    cp_x(0).start()
    cp_x(1).start()
    for cp in cp_small:
        cp.start()
    ri = jax.lax.broadcasted_iota(jnp.int32, (128, 128), 0)
    ci = jax.lax.broadcasted_iota(jnp.int32, (128, 128), 1)
    perm_ref[0] = (ci == (ri >> 3) + 16 * (ri & 7)).astype(f32)
    perm_ref[1] = ((ri + ci == 128) & (ci >= 1)).astype(f32)

    lane_i = jax.lax.broadcasted_iota(jnp.int32, (1, 128), 1)
    lane0 = lane_i == 0
    sgn = (1 - 2 * (lane_i & 1)).astype(f32)
    sgn_m = (1 - 2 * ((lane_i >> 1) & 1)).astype(f32)

    def pro1(c, carry):
        @pl.when(c < 3)
        def _():
            cp_x(2 * c + 2).start()
            cp_x(2 * c + 3).start()

        @pl.when(c == 3)
        def _():
            for cp in cp_wt:
                cp.start()

        @pl.when(c >= 4)
        def _():
            unit_start(c - 4)

        cp_x(c).wait()
        r0 = pl.multiple_of(c * 256, 256)
        xt = [x_v[pl.ds(r0, 256), j * 128:(j + 1) * 128].astype(f32) for j in range(8)]
        zero = jnp.zeros((256, 128), f32)
        r1 = [rev(xt[7], zero), rev(xt[6], xt[7])]
        r2 = [rev(xt[3], zero), rev(xt[2], xt[3])]
        ee, eo, oe, oo = [], [], [], []
        for T in range(2):
            e1, o1 = xt[T] + r1[T], xt[T] - r1[T]
            e2, o2 = r2[T] + xt[4 + T], r2[T] - xt[4 + T]
            ee.append(e1 + e2)
            eo.append(e1 - e2)
            oe.append(o1 - o2)
            oo.append(o1 + o2)
        oo[0] = jnp.where(lane0, xt[2] - xt[6], oo[0])
        e256 = (xt[2] + xt[6])[:, 0:1]
        mid = jnp.broadcast_to(e256, (256, 128)) * sgn_m
        nyq = jnp.sum((ee[0] + ee[1]) * sgn, axis=1, keepdims=True) + e256
        ee, eo, oe, oo = (jnp.concatenate(v, axis=1) for v in (ee, eo, oe, oo))
        rr = pl.ds(2 * c, 2)
        for t in range(2):
            z1[0, rr, :, :, t * 128:(t + 1) * 128] = (qdot(ee, C0, t) + mid).reshape(2, 16, 8, 128)
            z1[0, rr, :, :, (2 + t) * 128:(3 + t) * 128] = qdot(eo, C1, t).reshape(2, 16, 8, 128)
            z1[1, rr, :, :, t * 128:(t + 1) * 128] = qdot(oe, S0, t).reshape(2, 16, 8, 128)
            z1[1, rr, :, :, (2 + t) * 128:(3 + t) * 128] = qdot(oo, S1F, t).reshape(2, 16, 8, 128)
        z1[0, rr, :, :, 512:640] = jnp.where(lane0, nyq, 0.0).reshape(2, 16, 8, 128)
        z1[1, rr, :, :, 512:640] = jnp.zeros((2, 16, 8, 128), f32)
        return carry

    cp_cs.wait()
    jax.lax.fori_loop(0, 8, pro1, 0)

    def stage_a(hi):
        for t in range(5):
            sl = slice(t * 128, (t + 1) * 128)
            xin = [(z1[0, s2, hi, :, sl], z1[1, s2, hi, :, sl]) for s2 in range(16)]
            xo = _dft16(xin, -1)
            for k2 in range(16):
                z2[0, k2, hi, :, sl] = xo[k2][0]
                z2[1, k2, hi, :, sl] = xo[k2][1]

    norm = 1.0 / (S_LEN * DM)
    cscale = [jnp.where(lane0, norm, 2.0 * norm).astype(f32)] + [2.0 * norm] * 3 + [norm]

    def wperm(c, carry):
        @pl.when(c % 3 == 0)
        def _():
            unit_start(6 + c // 3)

        for bb in range(2):
            blk_i = 2 * c + bb
            l0 = pl.multiple_of(blk_i * 128, 128)
            for i, (wt, wn) in enumerate(((wrt_v.bitcast(u32), wrn_v), (wit_v.bitcast(u32), win_v))):
                for t in range(5):
                    if t < 4:
                        w = wt[(t % 2) * 128:(t % 2 + 1) * 128, pl.ds(l0, 128)].reshape(8, 16, 128)
                        pk = (_lo_pair if t < 2 else _hi_pair)(w[:, :8, :], w[:, 8:, :])
                        blk = pltpu.bitcast(pk.reshape(64, 128), bf16)
                    else:
                        blk = jnp.broadcast_to(wn[:, pl.ds(l0, 128)], (128, 128))
                    o = jax.lax.dot_general(perm_ref[0], blk, nt_dims, preferred_element_type=f32)
                    wp_v[i, :, blk_i, :, t * 128:(t + 1) * 128] = (o * cscale[t]).reshape(16, 8, 128)
        return carry

    def stage_a_loop(hi, carry):
        @pl.when(hi % 8 == 0)
        def _():
            unit_start(4 + hi // 8)

        stage_a(hi)
        return carry

    for cp in cp_small:
        cp.wait()
    small_ref[2] = small_ref[0] - small_ref[1]
    small_ref[3] = -small_ref[1] - small_ref[0]
    sub = jax.lax.broadcasted_iota(jnp.int32, (8, 128), 0)
    for part in range(2):
        for k2 in range(1, 16):
            v = jnp.zeros((8, 128), f32)
            for j in range(8):
                v = jnp.where(sub == j, tws_ref[512 + part * 128 + k2 * 8 + j], v)
            twb_ref[part, k2] = v
    gw_row[...] = gw_ref[...].astype(f32)
    jax.lax.fori_loop(0, 16, stage_a_loop, 0)

    for cp in cp_wt:
        cp.wait()
    jax.lax.fori_loop(0, 8, wperm, 0)

    def cdot3(m1, m2, m3, zr, zi):
        k1 = jnp.dot(m1, (zr + zi).astype(bf16), preferred_element_type=f32)
        k2 = jnp.dot(m2, zi.astype(bf16), preferred_element_type=f32)
        k3 = jnp.dot(m3, zr.astype(bf16), preferred_element_type=f32)
        return k1 - k2, k1 + k3

    def b_fwd(k2):
        tr, ti = tw_ref[pl.ds(k2, 1), :], tw_ref[pl.ds(16 + k2, 1), :]
        mr = small_ref[0] * tr - small_ref[1] * ti
        mi = small_ref[0] * ti + small_ref[1] * tr
        return cdot3(mr, mr + mi, mi - mr, z2[0, k2].reshape(128, 640), z2[1, k2].reshape(128, 640))

    def b_inv(k2, x):
        xr, xi = x
        wr = wp_v[0, k2].reshape(128, 640)
        wi = wp_v[1, k2].reshape(128, 640)
        pr = xr * wr - xi * wi
        pi = xr * wi + xi * wr
        gr, gi = cdot3(small_ref[0], small_ref[2], small_ref[3], pr, pi)
        z1[0, k2] = gr.reshape(16, 8, 640)
        z1[1, k2] = gi.reshape(16, 8, 640)

    def stage_b2(j, carry):
        @pl.when(j < 7)
        def _():
            unit_start(9 + j)

        xa = b_fwd(2 * j)
        xb = b_fwd(2 * j + 1)
        b_inv(2 * j, xa)
        b_inv(2 * j + 1, xb)
        return carry

    jax.lax.fori_loop(0, 8, stage_b2, 0)

    lane0a = jax.lax.broadcasted_iota(jnp.int32, (8, 128), 1) == 0

    def inv_twiddles(hi):
        tw_inv = [None]
        for k2 in range(1, 16):
            cr, ci = tws_ref[hi * 16 + k2], tws_ref[256 + hi * 16 + k2]
            br, bi = twb_ref[0, k2], twb_ref[1, k2]
            tw_inv.append((br * cr - bi * ci, br * ci + bi * cr))
        return tw_inv

    def a_inv_tile(hi, t, tw_inv, u_dst):
        sl = slice(t * 128, (t + 1) * 128)
        w = np.exp(2j * np.pi / 16.0)
        tmp = bt_scr.at[t % 2]
        for b in range(4):
            xin = []
            for a in range(4):
                k2 = 4 * a + b
                gr, gi = z1[0, k2, hi, :, sl], z1[1, k2, hi, :, sl]
                if k2 > 0:
                    tr, ti = tw_inv[k2]
                    gr, gi = gr * tr - gi * ti, gr * ti + gi * tr
                xin.append((gr, gi))
            col = _dft4(xin, +1)
            for c in range(4):
                v = col[c] if b * c == 0 else _cmul_const(col[c], w ** (b * c))
                tmp[0, b, c] = v[0]
                tmp[1, b, c] = v[1]
        for c in range(4):
            row = _dft4([(tmp[0, b, c], tmp[1, b, c]) for b in range(4)], +1)
            for d in range(4):
                s2 = c + 4 * d
                u_dst[s2, :, sl] = row[d][0]
                if t < 4:
                    u_dst[s2, :, 640 + t * 128:640 + (t + 1) * 128] = row[d][1]

    def stage_c2(m, carry):
        @pl.when(jnp.logical_and(m >= 2, m < 6))
        def _():
            cp_wo(2 * (m - 2)).start()
            cp_wo(2 * (m - 2) + 1).start()

        stage_c(2 * m, 2 * m + 1, u0, u1)
        stage_c(2 * m + 1, jnp.minimum(2 * m + 2, 15), u1, u0)
        return carry

    def stage_c(hi, nxt, u_src, u_dst):
        tw_inv = inv_twiddles(nxt)
        unit_repack(hi)
        for t in range(5):
            a_inv_tile(nxt, t, tw_inv, u_dst)
        nyq = u_src[:, :, 512:513].reshape(128, 1)
        n = jnp.broadcast_to(nyq, (128, 128)) * sgn
        ue_r = u_src[:, :, 0:256].reshape(128, 256)
        uo_r = u_src[:, :, 256:512].reshape(128, 256)
        ue_i = u_src[:, :, 640:896].reshape(128, 256)
        uo_i = u_src[:, :, 896:1152].reshape(128, 256)
        for T in range(2):
            a0 = qdot_t(ue_r, C0, T) + n
            a1 = qdot_t(uo_r, C1, T)
            b0 = qdot_t(ue_i, S0, T)
            b1 = qdot_t(uo_i, S1F, T)
            if T == 0:
                b1 = jnp.where(lane0, 0.0, b1)
            p, q, pm, qm = a0 + a1, b0 + b1, a0 - a1, b0 - b1
            z2[0, :, hi, :, T * 128:(T + 1) * 128] = (p + q).reshape(16, 8, 128)
            z2[1, :, hi, :, T * 128:(T + 1) * 128] = (pm + qm).reshape(16, 8, 128)
            up_scr[T] = p - q
            up_scr[2 + T] = pm - qm
        s_e = jnp.sum((ue_r[:, :128] + ue_r[:, 128:]) * sgn_m, axis=1, keepdims=True) + nyq
        s_o = jnp.sum((uo_i[:, :128] + uo_i[:, 128:]) * sgn_m, axis=1, keepdims=True)
        z2[1, :, hi, :, 384:512] = rev(up_scr[0], up_scr[1]).reshape(16, 8, 128)
        z2[1, :, hi, :, 256:384] = rev(up_scr[1], s_e + s_o).reshape(16, 8, 128)
        z2[0, :, hi, :, 384:512] = rev(up_scr[2], up_scr[3]).reshape(16, 8, 128)
        z2[0, :, hi, :, 256:384] = rev(up_scr[3], s_e - s_o).reshape(16, 8, 128)

    tw0 = inv_twiddles(0)
    for t in range(5):
        a_inv_tile(0, t, tw0, u0)
    jax.lax.fori_loop(0, 8, stage_c2, 0)

    scale = DH ** -0.5
    rows = jax.lax.broadcasted_iota(jnp.int32, (L, L), 0)
    cols = jax.lax.broadcasted_iota(jnp.int32, (L, L), 1)
    mask = (rows < M) | (rows >= cols)
    wo32 = wo_v.bitcast(u32)

    def qkv_head(h, hd):
        return tuple(jnp.dot(h, pltpu.bitcast(wqkv[3 * hd + j], bf16), preferred_element_type=f32)
                     for j in range(3))

    def scores(qkv):
        return jax.lax.dot_general(qkv[0], qkv[1].astype(bf16), nt_dims, preferred_element_type=f32)

    def softmax(s):
        s = jnp.where(mask, s * scale, -1e9)
        m = jnp.max(s, axis=-1, keepdims=True)
        p = jnp.exp(s - m)
        l = jnp.sum(p, axis=-1, keepdims=True)
        return p / l

    def pv(p, qkv):
        return jnp.dot(p, qkv[2].astype(bf16), preferred_element_type=f32)

    def cp_out(seg0, nseg):
        r0 = pl.multiple_of(seg0 * SEG, SEG)
        return pltpu.make_async_copy(out_v.at[pl.ds(r0, nseg * SEG)], out_hbm.at[pl.ds(r0, nseg * SEG)], sem_out)

    def mix(seg):
        r0 = pl.multiple_of(seg * SEG, SEG)
        xs = x_v[pl.ds(r0, SEG), :].astype(f32)
        gate = jax.nn.sigmoid(jnp.sum(xs * gw_row[...], axis=-1, keepdims=True))
        s2 = seg // 4
        hi0 = (seg % 4) * 4
        b = jnp.concatenate([z2[0, s2, pl.ds(hi0, 4), :, 0:512].reshape(SEG, 512),
                             z2[1, s2, pl.ds(hi0, 4), :, 0:512].reshape(SEG, 512)], axis=1)
        res = gate * a_scr[...] + (1.0 - gate) * b
        out_v[pl.ds(r0, SEG), :] = res.astype(out_v.dtype)


    def wo_part(h0, h1, n, lhs):
        w = pltpu.bitcast(wo32[n, h0 * (DH // 2):h1 * (DH // 2), :], bf16)
        return jnp.dot(lhs, w, preferred_element_type=f32)

    def step(s, mem, first=False):
        r0 = s * SEG if first else pl.multiple_of(s * SEG, SEG)
        xs = x_v[pl.ds(r0, SEG), :].astype(f32)
        h = jnp.concatenate([mem, xs], axis=0)
        qkvs, sc, ps, oh = {}, {}, {}, {}

        def wo_a(n):
            if first:
                cp_wo(n).wait()
            wa_scr[:, n * 128:(n + 1) * 128] = wo_part(0, HA, n, oa)

        for i in range(3):
            qkvs[i] = qkv_head(h, i)
        sc[0] = scores(qkvs[0])
        sc[1] = scores(qkvs[1])
        ps[0] = softmax(sc.pop(0))
        if not first:
            mix(s - 1)
        for hd in range(H):
            if hd + 3 < H:
                qkvs[hd + 3] = qkv_head(h, hd + 3)
            for n in WO_SCHED.get((hd, 0), ()):
                wo_a(n)
            if hd + 2 < H:
                sc[hd + 2] = scores(qkvs[hd + 2])
            if hd + 1 < H:
                ps[hd + 1] = softmax(sc.pop(hd + 1))
            oh[hd] = pv(ps.pop(hd), qkvs.pop(hd))
            if hd == HA - 1:
                oa = jnp.concatenate([oh.pop(i) for i in range(HA)], axis=1)
            for n in WO_SCHED.get((hd, 1), ()):
                wo_a(n)
        ob = jnp.concatenate([oh.pop(i) for i in range(HA, H)], axis=1)
        out = wa_scr[...] + jnp.concatenate([wo_part(HA, H, n, ob) for n in range(8)], axis=1)
        a_scr[...] = out[M:]
        if not first:
            @pl.when(s % 3 == 0)
            def _():
                cp_out(s - 3, 3).start()

        return out[:M]

    mem1 = step(0, mem_ref[...].astype(f32), first=True)
    jax.lax.fori_loop(1, NSEG, step, mem1, unroll=UNROLL)
    mix(NSEG - 1)
    last = ((NSEG - 1) // 3) * 3
    cp_out(last, NSEG - last).start()
    pltpu.make_async_copy(out_v.at[pl.ds(0, NSEG * SEG)], out_hbm.at[pl.ds(0, NSEG * SEG)], sem_out).wait()


@jax.jit
def _run(A_x, A_mem0, A_Wq, A_Wk, A_Wv, A_Wo, B_w_r, B_w_i, gate_w):
    any_spec = pl.BlockSpec(memory_space=pl.ANY)
    out = pl.pallas_call(
        _kernel,
        out_shape=jax.ShapeDtypeStruct((S_LEN, DM), A_x.dtype),
        in_specs=[any_spec] * 13,
        out_specs=any_spec,
        scratch_shapes=[
            pltpu.VMEM((M, DM), bf16),
            pltpu.VMEM((1, DM), bf16),
            pltpu.VMEM((1, DM), f32),
            pltpu.VMEM((2, 16, 8, 128), f32),
            pltpu.SMEM((768,), f32),
            pltpu.VMEM((4, 128, 128), f32),
            pltpu.VMEM((32, 128), f32),
            pltpu.VMEM((2, 128, 128), f32),
            pltpu.VMEM((S_LEN, DM), bf16),
            pltpu.VMEM((8, 128, 128), u32),
            pltpu.VMEM((DM // 2, S_LEN), bf16),
            pltpu.VMEM((DM // 2, S_LEN), bf16),
            pltpu.VMEM((1, S_LEN), bf16),
            pltpu.VMEM((1, S_LEN), bf16),
            pltpu.VMEM((2, 16, 16, 8, 640), f32),
            pltpu.VMEM((3 * H, DM // 2, DH), u32),
            pltpu.VMEM((8, H * DH, 128), bf16),
            pltpu.VMEM((2, 16, 16, 8, 640), f32),
            pltpu.VMEM((2, 16, 16, 8, 640), f32),
            pltpu.VMEM((16, 8, 1152), f32),
            pltpu.VMEM((16, 8, 1152), f32),
            pltpu.VMEM((2, 2, 4, 4, 8, 128), f32),
            pltpu.VMEM((4, 128, 128), f32),
            pltpu.VMEM((L, DM), f32),
            pltpu.VMEM((SEG, DM), f32),
            pltpu.VMEM((S_LEN, DM), bf16),
            pltpu.SemaphoreType.DMA((8,)),
            pltpu.SemaphoreType.DMA(()),
            pltpu.SemaphoreType.DMA((5,)),
            pltpu.SemaphoreType.DMA((4,)),
            pltpu.SemaphoreType.DMA((3 * H,)),
            pltpu.SemaphoreType.DMA((8,)),
            pltpu.SemaphoreType.DMA(()),
        ],
        compiler_params=pltpu.CompilerParams(vmem_limit_bytes=124 * 1024 * 1024),
    )(A_x.reshape(S_LEN, DM), A_mem0.reshape(M, DM),
      A_Wq.reshape(512, 64, DH), A_Wk.reshape(512, 64, DH), A_Wv.reshape(512, 64, DH),
      A_Wo.reshape(H * DH, DM), B_w_r.T, B_w_i.T, gate_w.reshape(1, DM),
      _CS, _TWS, _SMALL, _TW)
    return out.reshape(A_x.shape)


def pallas_gated_mix__memory_aug_recurrent_mem_tr__spectral_gfnet__prompt_kernel(
    A_x, A_mem0, A_Wq, A_Wk, A_Wv, A_Wo, A_seg_len, B_x, B_w_r, B_w_i, gate_w,
):
    del B_x
    assert int(A_seg_len) == SEG and A_x.shape == (1, S_LEN, DM)
    return _run(A_x, A_mem0, A_Wq, A_Wk, A_Wv, A_Wo, B_w_r, B_w_i, gate_w)
```

```python
import numpy as np
import ml_dtypes

import jax
import jax.numpy as jnp
import jax.experimental.pallas as pl
import jax.experimental.pallas.tpu as pltpu

S_LEN, DM, H, DH, M, SEG = 2048, 1024, 32, 128, 8, 32
L = M + SEG
NSEG = S_LEN // SEG
DF = DM // 2 + 1
f32 = jnp.float32
bf16 = jnp.bfloat16
u32 = jnp.uint32
UNROLL = 3
QL = 4
HA = 27
WO_SCHED = {(27, 1): (0,), (28, 0): (1,), (28, 1): (2,), (29, 0): (3,), (29, 1): (4,), (30, 1): (5, 6), (31, 1): (7,)}


def _bf16_np(a):
    return np.asarray(a, np.float32).astype(ml_dtypes.bfloat16)


def _pack_rows_u32(a):
    b = _bf16_np(a).view(np.uint16).astype(np.uint32)
    return b[0::2] | (b[1::2] << 16)


def _make_consts():
    q = np.arange(DM // 4)
    th = 2.0 * np.pi / DM
    a0 = th * ((2 * np.outer(q, q)) % DM)
    a1 = th * ((np.outer(q, 2 * q + 1)) % DM)
    s1f = -np.sin(a1)
    s1f[0, :] = -np.cos(np.pi * q)
    mperm = 16 * (q // 16) + ((q % 16) >> 1) + 8 * (q & 1)
    fwd = [np.cos(a0), np.cos(a1), -np.sin(a0), s1f]
    cs = np.stack([_pack_rows_u32(m[:, mperm]) for m in fwd])
    cs = np.ascontiguousarray(cs.reshape(4, 128, 2, 128).transpose(0, 2, 1, 3)).reshape(8, 128, 128)

    i16 = np.arange(16)
    i128 = np.arange(128)
    d128 = np.exp(-2j * np.pi * ((np.outer(i128, i128)) % 128) / 128.0)
    dc = np.conj(d128)
    small = np.stack([d128.real, d128.imag]).astype(np.float32)
    tw_f = np.exp(-2j * np.pi * np.outer(i16, i128) / 2048.0)
    tw = np.concatenate([tw_f.real, tw_f.imag]).astype(np.float32)
    twb = np.exp(2j * np.pi * np.outer(i16, np.arange(8)) / 2048.0)
    tws = np.exp(2j * np.pi * 8 * np.outer(i16, i16) / 2048.0)
    tws = np.concatenate([tws.real.reshape(-1), tws.imag.reshape(-1),
                          twb.real.reshape(-1), twb.imag.reshape(-1)]).astype(np.float32)
    return cs, tws, small, tw


_CS, _TWS, _SMALL, _TW = _make_consts()
NU = 16


def _lo_pair(a, b):
    return (a & np.uint32(0xFFFF)) | (b << 16)


def _hi_pair(a, b):
    return (a >> 16) | (b & np.uint32(0xFFFF0000))


def _cmul_const(x, c):
    re, im = x
    cr, ci = float(np.real(c)), float(np.imag(c))
    if abs(ci) < 1e-9:
        return (re, im) if cr > 0 else (-re, -im)
    if abs(cr) < 1e-9:
        return (-im, re) if ci > 0 else (im, -re)
    if abs(abs(cr) - abs(ci)) < 1e-9:
        a = abs(cr)
        sr, si = (1.0 if cr > 0 else -1.0), (1.0 if ci > 0 else -1.0)
        nr = (re if sr > 0 else -re) - (im if si > 0 else -im)
        ni = (re if si > 0 else -re) + (im if sr > 0 else -im)
        return (nr * a, ni * a)
    return (re * cr - im * ci, re * ci + im * cr)


def _dft4(x, sign):
    (ar, ai), (br, bi), (cr, ci), (dr, di) = x
    s0r, s0i = ar + cr, ai + ci
    s1r, s1i = ar - cr, ai - ci
    s2r, s2i = br + dr, bi + di
    s3r, s3i = br - dr, bi - di
    if sign < 0:
        return [(s0r + s2r, s0i + s2i), (s1r + s3i, s1i - s3r), (s0r - s2r, s0i - s2i), (s1r - s3i, s1i + s3r)]
    return [(s0r + s2r, s0i + s2i), (s1r - s3i, s1i + s3r), (s0r - s2r, s0i - s2i), (s1r + s3i, s1i - s3r)]


def _dft16(x, sign):
    w = np.exp(sign * 2j * np.pi / 16.0)
    t = [[None] * 4 for _ in range(4)]
    for b in range(4):
        col = _dft4([x[4 * a + b] for a in range(4)], sign)
        for c in range(4):
            t[b][c] = col[c] if b * c == 0 else _cmul_const(col[c], w ** (b * c))
    out = [None] * 16
    for c in range(4):
        row = _dft4([t[b][c] for b in range(4)], sign)
        for d in range(4):
            out[c + 4 * d] = row[d]
    return out


def _kernel(x_hbm, mem_hbm, wq_hbm, wk_hbm, wv_hbm, wo_hbm, wr_hbm, wi_hbm, gw_hbm,
            cs_hbm, tws_hbm, small_hbm, tw_hbm,
            out_hbm,
            mem_ref, gw_ref, gw_row, twb_ref, tws_ref, small_ref, tw_ref, perm_ref,
            x_v, cs_v, wrt_v, wit_v, wrn_v, win_v, wp_v, wqkv, wo_v, z1, z2, u0, u1, bt_scr, up_scr, wa_scr, a_scr, out_v,
            sem_x, sem_c, sem_s, sem_in, sem_w, sem_wo, sem_out):
    w32_hbm = tuple(w.bitcast(u32) for w in (wq_hbm, wk_hbm, wv_hbm))
    nt_dims = (((1,), (1,)), ((), ()))

    def cp_x(i):
        r0 = pl.multiple_of(i * 256, 256)
        return pltpu.make_async_copy(x_hbm.at[pl.ds(r0, 256)], x_v.at[pl.ds(r0, 256)], sem_x.at[i])

    cp_cs = pltpu.make_async_copy(cs_hbm, cs_v, sem_c)
    cp_wt = []
    for i, (src, dst, dstn) in enumerate(((wr_hbm, wrt_v, wrn_v), (wi_hbm, wit_v, win_v))):
        cp_wt.append(pltpu.make_async_copy(src.at[pl.ds(0, 512)], dst, sem_in.at[2 * i]))
        cp_wt.append(pltpu.make_async_copy(src.at[pl.ds(512, 1)], dstn, sem_in.at[2 * i + 1]))

    def cp_wo(n):
        return pltpu.make_async_copy(wo_hbm.at[:, pl.ds(n * 128, 128)], wo_v.at[n], sem_wo.at[n])

    def cp_w(p, par, which):
        t = 2 * p + par
        return pltpu.make_async_copy(w32_hbm[which].at[:, par * 16 + p], wqkv.at[3 * t + which],
                                     sem_w.at[3 * t + which])

    def unit_start(p):
        for par in range(2):
            for which in range(3):
                cp_w(p, par, which).start()

    def unit_repack(p):
        for par in range(2):
            for which in range(3):
                cp_w(p, par, which).wait()
        for which in range(3):
            ta = 6 * p + which
            tb = 6 * p + 3 + which
            for r in range(0, 512, 64):
                a = wqkv[ta, r:r + 64, :]
                b = wqkv[tb, r:r + 64, :]
                wqkv[ta, r:r + 64, :] = _lo_pair(a, b)
                wqkv[tb, r:r + 64, :] = _hi_pair(a, b)

    C0, C1, S0, S1F = range(4)

    def qdot(lhs, mat, nt):
        return jnp.dot(lhs, pltpu.bitcast(cs_v[2 * mat + nt], bf16), preferred_element_type=f32)

    def qdot_t(lhs, mat, dt):
        rows = jnp.concatenate([cs_v[2 * mat + kt, dt * 64:(dt + 1) * 64, :] for kt in range(2)], axis=1)
        return jax.lax.dot_general(lhs, pltpu.bitcast(rows, bf16), nt_dims, preferred_element_type=f32)

    def rev(t, first):
        return jnp.where(lane0, first, jnp.dot(t, perm_ref[1], preferred_element_type=f32))

    cp_small = [pltpu.make_async_copy(src, dst, sem_s.at[i]) for i, (src, dst) in enumerate((
        (tws_hbm, tws_ref), (small_hbm, small_ref.at[pl.ds(0, 2)]), (tw_hbm, tw_ref),
        (mem_hbm, mem_ref), (gw_hbm, gw_ref)))]
    cp_cs.start()
    cp_x(0).start()
    cp_x(1).start()
    for cp in cp_small:
        cp.start()
    ri = jax.lax.broadcasted_iota(jnp.int32, (128, 128), 0)
    ci = jax.lax.broadcasted_iota(jnp.int32, (128, 128), 1)
    perm_ref[0] = (ci == (ri >> 3) + 16 * (ri & 7)).astype(f32)
    perm_ref[1] = ((ri + ci == 128) & (ci >= 1)).astype(f32)

    lane_i = jax.lax.broadcasted_iota(jnp.int32, (1, 128), 1)
    lane0 = lane_i == 0
    sgn = (1 - 2 * (lane_i & 1)).astype(f32)
    sgn_m = (1 - 2 * ((lane_i >> 1) & 1)).astype(f32)

    def pro1(c, carry):
        @pl.when(c < 3)
        def _():
            cp_x(2 * c + 2).start()
            cp_x(2 * c + 3).start()

        @pl.when(c == 3)
        def _():
            for cp in cp_wt:
                cp.start()

        @pl.when(c >= 4)
        def _():
            unit_start(c - 4)

        cp_x(c).wait()
        r0 = pl.multiple_of(c * 256, 256)
        xt = [x_v[pl.ds(r0, 256), j * 128:(j + 1) * 128].astype(f32) for j in range(8)]
        zero = jnp.zeros((256, 128), f32)
        r1 = [rev(xt[7], zero), rev(xt[6], xt[7])]
        r2 = [rev(xt[3], zero), rev(xt[2], xt[3])]
        ee, eo, oe, oo = [], [], [], []
        for T in range(2):
            e1, o1 = xt[T] + r1[T], xt[T] - r1[T]
            e2, o2 = r2[T] + xt[4 + T], r2[T] - xt[4 + T]
            ee.append(e1 + e2)
            eo.append(e1 - e2)
            oe.append(o1 - o2)
            oo.append(o1 + o2)
        oo[0] = jnp.where(lane0, xt[2] - xt[6], oo[0])
        e256 = (xt[2] + xt[6])[:, 0:1]
        mid = jnp.broadcast_to(e256, (256, 128)) * sgn_m
        nyq = jnp.sum((ee[0] + ee[1]) * sgn, axis=1, keepdims=True) + e256
        ee, eo, oe, oo = (jnp.concatenate(v, axis=1) for v in (ee, eo, oe, oo))
        rr = pl.ds(2 * c, 2)
        for t in range(2):
            z1[0, rr, :, :, t * 128:(t + 1) * 128] = (qdot(ee, C0, t) + mid).reshape(2, 16, 8, 128)
            z1[0, rr, :, :, (2 + t) * 128:(3 + t) * 128] = qdot(eo, C1, t).reshape(2, 16, 8, 128)
            z1[1, rr, :, :, t * 128:(t + 1) * 128] = qdot(oe, S0, t).reshape(2, 16, 8, 128)
            z1[1, rr, :, :, (2 + t) * 128:(3 + t) * 128] = qdot(oo, S1F, t).reshape(2, 16, 8, 128)
        z1[0, rr, :, :, 512:640] = jnp.where(lane0, nyq, 0.0).reshape(2, 16, 8, 128)
        z1[1, rr, :, :, 512:640] = jnp.zeros((2, 16, 8, 128), f32)
        return carry

    cp_cs.wait()
    jax.lax.fori_loop(0, 8, pro1, 0)

    def stage_a(hi):
        for t in range(5):
            sl = slice(t * 128, (t + 1) * 128)
            xin = [(z1[0, s2, hi, :, sl], z1[1, s2, hi, :, sl]) for s2 in range(16)]
            xo = _dft16(xin, -1)
            for k2 in range(16):
                z2[0, k2, hi, :, sl] = xo[k2][0]
                z2[1, k2, hi, :, sl] = xo[k2][1]

    norm = 1.0 / (S_LEN * DM)
    cscale = [jnp.where(lane0, norm, 2.0 * norm).astype(f32)] + [2.0 * norm] * 3 + [norm]

    def wperm(c, carry):
        @pl.when(c % 3 == 0)
        def _():
            unit_start(6 + c // 3)

        for bb in range(2):
            blk_i = 2 * c + bb
            l0 = pl.multiple_of(blk_i * 128, 128)
            for i, (wt, wn) in enumerate(((wrt_v.bitcast(u32), wrn_v), (wit_v.bitcast(u32), win_v))):
                for t in range(5):
                    if t < 4:
                        w = wt[(t % 2) * 128:(t % 2 + 1) * 128, pl.ds(l0, 128)].reshape(8, 16, 128)
                        pk = (_lo_pair if t < 2 else _hi_pair)(w[:, :8, :], w[:, 8:, :])
                        blk = pltpu.bitcast(pk.reshape(64, 128), bf16)
                    else:
                        blk = jnp.broadcast_to(wn[:, pl.ds(l0, 128)], (128, 128))
                    o = jax.lax.dot_general(perm_ref[0], blk, nt_dims, preferred_element_type=f32)
                    wp_v[i, :, blk_i, :, t * 128:(t + 1) * 128] = (o * cscale[t]).reshape(16, 8, 128)
        return carry

    def stage_a_loop(hi, carry):
        @pl.when(hi % 8 == 0)
        def _():
            unit_start(4 + hi // 8)

        stage_a(hi)
        return carry

    for cp in cp_small:
        cp.wait()
    small_ref[2] = small_ref[0] - small_ref[1]
    small_ref[3] = -small_ref[1] - small_ref[0]
    sub = jax.lax.broadcasted_iota(jnp.int32, (8, 128), 0)
    for part in range(2):
        for k2 in range(1, 16):
            v = jnp.zeros((8, 128), f32)
            for j in range(8):
                v = jnp.where(sub == j, tws_ref[512 + part * 128 + k2 * 8 + j], v)
            twb_ref[part, k2] = v
    gw_row[...] = gw_ref[...].astype(f32)
    jax.lax.fori_loop(0, 16, stage_a_loop, 0)

    for cp in cp_wt:
        cp.wait()
    jax.lax.fori_loop(0, 8, wperm, 0)

    def cdot3(m1, m2, m3, zr, zi):
        k1 = jnp.dot(m1, (zr + zi).astype(bf16), preferred_element_type=f32)
        k2 = jnp.dot(m2, zi.astype(bf16), preferred_element_type=f32)
        k3 = jnp.dot(m3, zr.astype(bf16), preferred_element_type=f32)
        return k1 - k2, k1 + k3

    def b_fwd(k2):
        tr, ti = tw_ref[pl.ds(k2, 1), :], tw_ref[pl.ds(16 + k2, 1), :]
        mr = small_ref[0] * tr - small_ref[1] * ti
        mi = small_ref[0] * ti + small_ref[1] * tr
        return cdot3(mr, mr + mi, mi - mr, z2[0, k2].reshape(128, 640), z2[1, k2].reshape(128, 640))

    def b_inv(k2, x):
        xr, xi = x
        wr = wp_v[0, k2].reshape(128, 640)
        wi = wp_v[1, k2].reshape(128, 640)
        pr = xr * wr - xi * wi
        pi = xr * wi + xi * wr
        gr, gi = cdot3(small_ref[0], small_ref[2], small_ref[3], pr, pi)
        z1[0, k2] = gr.reshape(16, 8, 640)
        z1[1, k2] = gi.reshape(16, 8, 640)

    def stage_b2(j, carry):
        @pl.when(j < 7)
        def _():
            unit_start(9 + j)

        xa = b_fwd(2 * j)
        xb = b_fwd(2 * j + 1)
        b_inv(2 * j, xa)
        b_inv(2 * j + 1, xb)
        return carry

    jax.lax.fori_loop(0, 8, stage_b2, 0)

    lane0a = jax.lax.broadcasted_iota(jnp.int32, (8, 128), 1) == 0

    def inv_twiddles(hi):
        tw_inv = [None]
        for k2 in range(1, 16):
            cr, ci = tws_ref[hi * 16 + k2], tws_ref[256 + hi * 16 + k2]
            br, bi = twb_ref[0, k2], twb_ref[1, k2]
            tw_inv.append((br * cr - bi * ci, br * ci + bi * cr))
        return tw_inv

    def a_inv_tile(hi, t, tw_inv, u_dst):
        sl = slice(t * 128, (t + 1) * 128)
        w = np.exp(2j * np.pi / 16.0)
        tmp = bt_scr.at[t % 2]
        for b in range(4):
            xin = []
            for a in range(4):
                k2 = 4 * a + b
                gr, gi = z1[0, k2, hi, :, sl], z1[1, k2, hi, :, sl]
                if k2 > 0:
                    tr, ti = tw_inv[k2]
                    gr, gi = gr * tr - gi * ti, gr * ti + gi * tr
                xin.append((gr, gi))
            col = _dft4(xin, +1)
            for c in range(4):
                v = col[c] if b * c == 0 else _cmul_const(col[c], w ** (b * c))
                tmp[0, b, c] = v[0]
                tmp[1, b, c] = v[1]
        for c in range(4):
            row = _dft4([(tmp[0, b, c], tmp[1, b, c]) for b in range(4)], +1)
            for d in range(4):
                s2 = c + 4 * d
                u_dst[s2, :, sl] = row[d][0]
                if t < 4:
                    u_dst[s2, :, 640 + t * 128:640 + (t + 1) * 128] = row[d][1]

    def stage_c2(m, carry):
        @pl.when(jnp.logical_and(m >= 2, m < 6))
        def _():
            cp_wo(2 * (m - 2)).start()
            cp_wo(2 * (m - 2) + 1).start()

        stage_c(2 * m, 2 * m + 1, u0, u1)
        stage_c(2 * m + 1, jnp.minimum(2 * m + 2, 15), u1, u0)
        return carry

    def stage_c(hi, nxt, u_src, u_dst):
        tw_inv = inv_twiddles(nxt)
        unit_repack(hi)
        for t in range(5):
            a_inv_tile(nxt, t, tw_inv, u_dst)
        nyq = u_src[:, :, 512:513].reshape(128, 1)
        n = jnp.broadcast_to(nyq, (128, 128)) * sgn
        ue_r = u_src[:, :, 0:256].reshape(128, 256)
        uo_r = u_src[:, :, 256:512].reshape(128, 256)
        ue_i = u_src[:, :, 640:896].reshape(128, 256)
        uo_i = u_src[:, :, 896:1152].reshape(128, 256)
        for T in range(2):
            a0 = qdot_t(ue_r, C0, T) + n
            a1 = qdot_t(uo_r, C1, T)
            b0 = qdot_t(ue_i, S0, T)
            b1 = qdot_t(uo_i, S1F, T)
            if T == 0:
                b1 = jnp.where(lane0, 0.0, b1)
            p, q, pm, qm = a0 + a1, b0 + b1, a0 - a1, b0 - b1
            z2[0, :, hi, :, T * 128:(T + 1) * 128] = (p + q).reshape(16, 8, 128)
            z2[1, :, hi, :, T * 128:(T + 1) * 128] = (pm + qm).reshape(16, 8, 128)
            up_scr[T] = p - q
            up_scr[2 + T] = pm - qm
        s_e = jnp.sum((ue_r[:, :128] + ue_r[:, 128:]) * sgn_m, axis=1, keepdims=True) + nyq
        s_o = jnp.sum((uo_i[:, :128] + uo_i[:, 128:]) * sgn_m, axis=1, keepdims=True)
        z2[1, :, hi, :, 384:512] = rev(up_scr[0], up_scr[1]).reshape(16, 8, 128)
        z2[1, :, hi, :, 256:384] = rev(up_scr[1], s_e + s_o).reshape(16, 8, 128)
        z2[0, :, hi, :, 384:512] = rev(up_scr[2], up_scr[3]).reshape(16, 8, 128)
        z2[0, :, hi, :, 256:384] = rev(up_scr[3], s_e - s_o).reshape(16, 8, 128)

    tw0 = inv_twiddles(0)
    for t in range(5):
        a_inv_tile(0, t, tw0, u0)
    jax.lax.fori_loop(0, 8, stage_c2, 0)

    scale = DH ** -0.5
    rows = jax.lax.broadcasted_iota(jnp.int32, (L, L), 0)
    cols = jax.lax.broadcasted_iota(jnp.int32, (L, L), 1)
    mask = (rows < M) | (rows >= cols)
    wo32 = wo_v.bitcast(u32)

    def qkv_head(h, hd):
        return tuple(jnp.dot(h, pltpu.bitcast(wqkv[3 * hd + j], bf16), preferred_element_type=f32)
                     for j in range(3))

    def scores(qkv):
        return jax.lax.dot_general(qkv[0], qkv[1].astype(bf16), nt_dims, preferred_element_type=f32)

    def softmax(s):
        s = jnp.where(mask, s * scale, -1e9)
        m = jnp.max(s, axis=-1, keepdims=True)
        p = jnp.exp(s - m)
        l = jnp.sum(p, axis=-1, keepdims=True)
        return p / l

    def pv(p, qkv):
        return jnp.dot(p, qkv[2].astype(bf16), preferred_element_type=f32)

    def cp_out(seg0, nseg):
        r0 = pl.multiple_of(seg0 * SEG, SEG)
        return pltpu.make_async_copy(out_v.at[pl.ds(r0, nseg * SEG)], out_hbm.at[pl.ds(r0, nseg * SEG)], sem_out)

    def mix(seg):
        r0 = pl.multiple_of(seg * SEG, SEG)
        xs = x_v[pl.ds(r0, SEG), :].astype(f32)
        gate = jax.nn.sigmoid(jnp.sum(xs * gw_row[...], axis=-1, keepdims=True))
        s2 = seg // 4
        hi0 = (seg % 4) * 4
        b = jnp.concatenate([z2[0, s2, pl.ds(hi0, 4), :, 0:512].reshape(SEG, 512),
                             z2[1, s2, pl.ds(hi0, 4), :, 0:512].reshape(SEG, 512)], axis=1)
        res = gate * a_scr[...] + (1.0 - gate) * b
        out_v[pl.ds(r0, SEG), :] = res.astype(out_v.dtype)


    def wo_part(h0, h1, n, lhs):
        w = pltpu.bitcast(wo32[n, h0 * (DH // 2):h1 * (DH // 2), :], bf16)
        return jnp.dot(lhs, w, preferred_element_type=f32)

    def step(s, mem, first=False):
        r0 = s * SEG if first else pl.multiple_of(s * SEG, SEG)
        xs = x_v[pl.ds(r0, SEG), :].astype(f32)
        h = jnp.concatenate([mem, xs], axis=0)
        qkvs, sc, ps, oh = {}, {}, {}, {}

        def wo_a(n):
            if first:
                cp_wo(n).wait()
            wa_scr[:, n * 128:(n + 1) * 128] = wo_part(0, HA, n, oa)

        for i in range(QL):
            qkvs[i] = qkv_head(h, i)
        sc[0] = scores(qkvs[0])
        sc[1] = scores(qkvs[1])
        ps[0] = softmax(sc.pop(0))
        if not first:
            mix(s - 1)
        for hd in range(H):
            if hd + QL < H:
                qkvs[hd + QL] = qkv_head(h, hd + QL)
            for n in WO_SCHED.get((hd, 0), ()):
                wo_a(n)
            if hd + 2 < H:
                sc[hd + 2] = scores(qkvs[hd + 2])
            if hd + 1 < H:
                ps[hd + 1] = softmax(sc.pop(hd + 1))
            oh[hd] = pv(ps.pop(hd), qkvs.pop(hd))
            if hd == HA - 1:
                oa = jnp.concatenate([oh.pop(i) for i in range(HA)], axis=1)
            for n in WO_SCHED.get((hd, 1), ()):
                wo_a(n)
        ob = jnp.concatenate([oh.pop(i) for i in range(HA, H)], axis=1)
        out = wa_scr[...] + jnp.concatenate([wo_part(HA, H, n, ob) for n in range(8)], axis=1)
        a_scr[...] = out[M:]
        if not first:
            @pl.when(s % 3 == 0)
            def _():
                cp_out(s - 3, 3).start()

        return out[:M]

    mem1 = step(0, mem_ref[...].astype(f32), first=True)
    jax.lax.fori_loop(1, NSEG, step, mem1, unroll=UNROLL)
    mix(NSEG - 1)
    last = ((NSEG - 1) // 3) * 3
    cp_out(last, NSEG - last).start()
    pltpu.make_async_copy(out_v.at[pl.ds(0, NSEG * SEG)], out_hbm.at[pl.ds(0, NSEG * SEG)], sem_out).wait()


@jax.jit
def _run(A_x, A_mem0, A_Wq, A_Wk, A_Wv, A_Wo, B_w_r, B_w_i, gate_w):
    any_spec = pl.BlockSpec(memory_space=pl.ANY)
    out = pl.pallas_call(
        _kernel,
        out_shape=jax.ShapeDtypeStruct((S_LEN, DM), A_x.dtype),
        in_specs=[any_spec] * 13,
        out_specs=any_spec,
        scratch_shapes=[
            pltpu.VMEM((M, DM), bf16),
            pltpu.VMEM((1, DM), bf16),
            pltpu.VMEM((1, DM), f32),
            pltpu.VMEM((2, 16, 8, 128), f32),
            pltpu.SMEM((768,), f32),
            pltpu.VMEM((4, 128, 128), f32),
            pltpu.VMEM((32, 128), f32),
            pltpu.VMEM((2, 128, 128), f32),
            pltpu.VMEM((S_LEN, DM), bf16),
            pltpu.VMEM((8, 128, 128), u32),
            pltpu.VMEM((DM // 2, S_LEN), bf16),
            pltpu.VMEM((DM // 2, S_LEN), bf16),
            pltpu.VMEM((1, S_LEN), bf16),
            pltpu.VMEM((1, S_LEN), bf16),
            pltpu.VMEM((2, 16, 16, 8, 640), f32),
            pltpu.VMEM((3 * H, DM // 2, DH), u32),
            pltpu.VMEM((8, H * DH, 128), bf16),
            pltpu.VMEM((2, 16, 16, 8, 640), f32),
            pltpu.VMEM((2, 16, 16, 8, 640), f32),
            pltpu.VMEM((16, 8, 1152), f32),
            pltpu.VMEM((16, 8, 1152), f32),
            pltpu.VMEM((2, 2, 4, 4, 8, 128), f32),
            pltpu.VMEM((4, 128, 128), f32),
            pltpu.VMEM((L, DM), f32),
            pltpu.VMEM((SEG, DM), f32),
            pltpu.VMEM((S_LEN, DM), bf16),
            pltpu.SemaphoreType.DMA((8,)),
            pltpu.SemaphoreType.DMA(()),
            pltpu.SemaphoreType.DMA((5,)),
            pltpu.SemaphoreType.DMA((4,)),
            pltpu.SemaphoreType.DMA((3 * H,)),
            pltpu.SemaphoreType.DMA((8,)),
            pltpu.SemaphoreType.DMA(()),
        ],
        compiler_params=pltpu.CompilerParams(vmem_limit_bytes=100 * 1024 * 1024),
    )(A_x.reshape(S_LEN, DM), A_mem0.reshape(M, DM),
      A_Wq.reshape(512, 64, DH), A_Wk.reshape(512, 64, DH), A_Wv.reshape(512, 64, DH),
      A_Wo.reshape(H * DH, DM), B_w_r.T, B_w_i.T, gate_w.reshape(1, DM),
      _CS, _TWS, _SMALL, _TW)
    return out.reshape(A_x.shape)


def pallas_gated_mix__memory_aug_recurrent_mem_tr__spectral_gfnet__prompt_kernel(
    A_x, A_mem0, A_Wq, A_Wk, A_Wv, A_Wo, A_seg_len, B_x, B_w_r, B_w_i, gate_w,
):
    del B_x
    assert int(A_seg_len) == SEG and A_x.shape == (1, S_LEN, DM)
    return _run(A_x, A_mem0, A_Wq, A_Wk, A_Wv, A_Wo, B_w_r, B_w_i, gate_w)
```

```python
import numpy as np
import ml_dtypes

import jax
import jax.numpy as jnp
import jax.experimental.pallas as pl
import jax.experimental.pallas.tpu as pltpu

S_LEN, DM, H, DH, M, SEG = 2048, 1024, 32, 128, 8, 32
L = M + SEG
NSEG = S_LEN // SEG
DF = DM // 2 + 1
f32 = jnp.float32
bf16 = jnp.bfloat16
u32 = jnp.uint32
UNROLL = 4
QL = 4
HA = 26
WO_SCHED = {(27, 1): (0,), (28, 0): (1,), (28, 1): (2,), (29, 0): (3,), (29, 1): (4,), (30, 1): (5, 6), (31, 1): (7,)}


def _bf16_np(a):
    return np.asarray(a, np.float32).astype(ml_dtypes.bfloat16)


def _pack_rows_u32(a):
    b = _bf16_np(a).view(np.uint16).astype(np.uint32)
    return b[0::2] | (b[1::2] << 16)


def _make_consts():
    q = np.arange(DM // 4)
    th = 2.0 * np.pi / DM
    a0 = th * ((2 * np.outer(q, q)) % DM)
    a1 = th * ((np.outer(q, 2 * q + 1)) % DM)
    s1f = -np.sin(a1)
    s1f[0, :] = -np.cos(np.pi * q)
    mperm = 16 * (q // 16) + ((q % 16) >> 1) + 8 * (q & 1)
    fwd = [np.cos(a0), np.cos(a1), -np.sin(a0), s1f]
    cs = np.stack([_pack_rows_u32(m[:, mperm]) for m in fwd])
    cs = np.ascontiguousarray(cs.reshape(4, 128, 2, 128).transpose(0, 2, 1, 3)).reshape(8, 128, 128)

    i16 = np.arange(16)
    i128 = np.arange(128)
    d128 = np.exp(-2j * np.pi * ((np.outer(i128, i128)) % 128) / 128.0)
    dc = np.conj(d128)
    small = np.stack([d128.real, d128.imag]).astype(np.float32)
    tw_f = np.exp(-2j * np.pi * np.outer(i16, i128) / 2048.0)
    tw = np.concatenate([tw_f.real, tw_f.imag]).astype(np.float32)
    twb = np.exp(2j * np.pi * np.outer(i16, np.arange(8)) / 2048.0)
    tws = np.exp(2j * np.pi * 8 * np.outer(i16, i16) / 2048.0)
    tws = np.concatenate([tws.real.reshape(-1), tws.imag.reshape(-1),
                          twb.real.reshape(-1), twb.imag.reshape(-1)]).astype(np.float32)
    return cs, tws, small, tw


_CS, _TWS, _SMALL, _TW = _make_consts()
NU = 16


def _lo_pair(a, b):
    return (a & np.uint32(0xFFFF)) | (b << 16)


def _hi_pair(a, b):
    return (a >> 16) | (b & np.uint32(0xFFFF0000))


def _cmul_const(x, c):
    re, im = x
    cr, ci = float(np.real(c)), float(np.imag(c))
    if abs(ci) < 1e-9:
        return (re, im) if cr > 0 else (-re, -im)
    if abs(cr) < 1e-9:
        return (-im, re) if ci > 0 else (im, -re)
    if abs(abs(cr) - abs(ci)) < 1e-9:
        a = abs(cr)
        sr, si = (1.0 if cr > 0 else -1.0), (1.0 if ci > 0 else -1.0)
        nr = (re if sr > 0 else -re) - (im if si > 0 else -im)
        ni = (re if si > 0 else -re) + (im if sr > 0 else -im)
        return (nr * a, ni * a)
    return (re * cr - im * ci, re * ci + im * cr)


def _dft4(x, sign):
    (ar, ai), (br, bi), (cr, ci), (dr, di) = x
    s0r, s0i = ar + cr, ai + ci
    s1r, s1i = ar - cr, ai - ci
    s2r, s2i = br + dr, bi + di
    s3r, s3i = br - dr, bi - di
    if sign < 0:
        return [(s0r + s2r, s0i + s2i), (s1r + s3i, s1i - s3r), (s0r - s2r, s0i - s2i), (s1r - s3i, s1i + s3r)]
    return [(s0r + s2r, s0i + s2i), (s1r - s3i, s1i + s3r), (s0r - s2r, s0i - s2i), (s1r + s3i, s1i - s3r)]


def _dft16(x, sign):
    w = np.exp(sign * 2j * np.pi / 16.0)
    t = [[None] * 4 for _ in range(4)]
    for b in range(4):
        col = _dft4([x[4 * a + b] for a in range(4)], sign)
        for c in range(4):
            t[b][c] = col[c] if b * c == 0 else _cmul_const(col[c], w ** (b * c))
    out = [None] * 16
    for c in range(4):
        row = _dft4([t[b][c] for b in range(4)], sign)
        for d in range(4):
            out[c + 4 * d] = row[d]
    return out


def _kernel(x_hbm, mem_hbm, wq_hbm, wk_hbm, wv_hbm, wo_hbm, wr_hbm, wi_hbm, gw_hbm,
            cs_hbm, tws_hbm, small_hbm, tw_hbm,
            out_hbm,
            mem_ref, gw_ref, gw_row, twb_ref, tws_ref, small_ref, tw_ref, perm_ref,
            x_v, cs_v, wrt_v, wit_v, wrn_v, win_v, wp_v, wqkv, wo_v, z1, z2, u0, u1, bt_scr, up_scr, wa_scr, a_scr, out_v, xpre, pre,
            sem_x, sem_c, sem_s, sem_in, sem_w, sem_wo, sem_out):
    w32_hbm = tuple(w.bitcast(u32) for w in (wq_hbm, wk_hbm, wv_hbm))
    nt_dims = (((1,), (1,)), ((), ()))

    def cp_x(i):
        r0 = pl.multiple_of(i * 256, 256)
        return pltpu.make_async_copy(x_hbm.at[pl.ds(r0, 256)], x_v.at[pl.ds(r0, 256)], sem_x.at[i])

    cp_cs = pltpu.make_async_copy(cs_hbm, cs_v, sem_c)
    cp_wt = []
    for i, (src, dst, dstn) in enumerate(((wr_hbm, wrt_v, wrn_v), (wi_hbm, wit_v, win_v))):
        cp_wt.append(pltpu.make_async_copy(src.at[pl.ds(0, 512)], dst, sem_in.at[2 * i]))
        cp_wt.append(pltpu.make_async_copy(src.at[pl.ds(512, 1)], dstn, sem_in.at[2 * i + 1]))

    def cp_wo(n):
        return pltpu.make_async_copy(wo_hbm.at[:, pl.ds(n * 128, 128)], wo_v.at[n], sem_wo.at[n])

    def cp_w(p, par, which):
        t = 2 * p + par
        return pltpu.make_async_copy(w32_hbm[which].at[:, par * 16 + p], wqkv.at[3 * t + which],
                                     sem_w.at[3 * t + which])

    def unit_start(p):
        for par in range(2):
            for which in range(3):
                cp_w(p, par, which).start()

    def unit_repack(p):
        for par in range(2):
            for which in range(3):
                cp_w(p, par, which).wait()
        for which in range(3):
            ta = 6 * p + which
            tb = 6 * p + 3 + which
            for r in range(0, 512, 64):
                a = wqkv[ta, r:r + 64, :]
                b = wqkv[tb, r:r + 64, :]
                wqkv[ta, r:r + 64, :] = _lo_pair(a, b)
                wqkv[tb, r:r + 64, :] = _hi_pair(a, b)

    C0, C1, S0, S1F = range(4)

    def qdot(lhs, mat, nt):
        return jnp.dot(lhs, pltpu.bitcast(cs_v[2 * mat + nt], bf16), preferred_element_type=f32)

    def qdot_t(lhs, mat, dt):
        rows = jnp.concatenate([cs_v[2 * mat + kt, dt * 64:(dt + 1) * 64, :] for kt in range(2)], axis=1)
        return jax.lax.dot_general(lhs, pltpu.bitcast(rows, bf16), nt_dims, preferred_element_type=f32)

    def rev(t, first):
        return jnp.where(lane0, first, jnp.dot(t, perm_ref[1], preferred_element_type=f32))

    cp_small = [pltpu.make_async_copy(src, dst, sem_s.at[i]) for i, (src, dst) in enumerate((
        (tws_hbm, tws_ref), (small_hbm, small_ref.at[pl.ds(0, 2)]), (tw_hbm, tw_ref),
        (mem_hbm, mem_ref), (gw_hbm, gw_ref)))]
    cp_cs.start()
    cp_x(0).start()
    cp_x(1).start()
    for cp in cp_small:
        cp.start()
    ri = jax.lax.broadcasted_iota(jnp.int32, (128, 128), 0)
    ci = jax.lax.broadcasted_iota(jnp.int32, (128, 128), 1)
    perm_ref[0] = (ci == (ri >> 3) + 16 * (ri & 7)).astype(f32)
    perm_ref[1] = ((ri + ci == 128) & (ci >= 1)).astype(f32)

    lane_i = jax.lax.broadcasted_iota(jnp.int32, (1, 128), 1)
    lane0 = lane_i == 0
    sgn = (1 - 2 * (lane_i & 1)).astype(f32)
    sgn_m = (1 - 2 * ((lane_i >> 1) & 1)).astype(f32)

    def pro1(c, carry):
        @pl.when(c < 3)
        def _():
            cp_x(2 * c + 2).start()
            cp_x(2 * c + 3).start()

        @pl.when(c == 3)
        def _():
            for cp in cp_wt:
                cp.start()

        @pl.when(c >= 4)
        def _():
            unit_start(c - 4)

        cp_x(c).wait()
        r0 = pl.multiple_of(c * 256, 256)
        xt = [x_v[pl.ds(r0, 256), j * 128:(j + 1) * 128].astype(f32) for j in range(8)]
        zero = jnp.zeros((256, 128), f32)
        r1 = [rev(xt[7], zero), rev(xt[6], xt[7])]
        r2 = [rev(xt[3], zero), rev(xt[2], xt[3])]
        ee, eo, oe, oo = [], [], [], []
        for T in range(2):
            e1, o1 = xt[T] + r1[T], xt[T] - r1[T]
            e2, o2 = r2[T] + xt[4 + T], r2[T] - xt[4 + T]
            ee.append(e1 + e2)
            eo.append(e1 - e2)
            oe.append(o1 - o2)
            oo.append(o1 + o2)
        oo[0] = jnp.where(lane0, xt[2] - xt[6], oo[0])
        e256 = (xt[2] + xt[6])[:, 0:1]
        mid = jnp.broadcast_to(e256, (256, 128)) * sgn_m
        nyq = jnp.sum((ee[0] + ee[1]) * sgn, axis=1, keepdims=True) + e256
        ee, eo, oe, oo = (jnp.concatenate(v, axis=1) for v in (ee, eo, oe, oo))
        rr = pl.ds(2 * c, 2)
        for t in range(2):
            z1[0, rr, :, :, t * 128:(t + 1) * 128] = (qdot(ee, C0, t) + mid).reshape(2, 16, 8, 128)
            z1[0, rr, :, :, (2 + t) * 128:(3 + t) * 128] = qdot(eo, C1, t).reshape(2, 16, 8, 128)
            z1[1, rr, :, :, t * 128:(t + 1) * 128] = qdot(oe, S0, t).reshape(2, 16, 8, 128)
            z1[1, rr, :, :, (2 + t) * 128:(3 + t) * 128] = qdot(oo, S1F, t).reshape(2, 16, 8, 128)
        z1[0, rr, :, :, 512:640] = jnp.where(lane0, nyq, 0.0).reshape(2, 16, 8, 128)
        z1[1, rr, :, :, 512:640] = jnp.zeros((2, 16, 8, 128), f32)
        return carry

    cp_cs.wait()
    jax.lax.fori_loop(0, 8, pro1, 0)

    def stage_a(hi):
        for t in range(5):
            sl = slice(t * 128, (t + 1) * 128)
            xin = [(z1[0, s2, hi, :, sl], z1[1, s2, hi, :, sl]) for s2 in range(16)]
            xo = _dft16(xin, -1)
            for k2 in range(16):
                z2[0, k2, hi, :, sl] = xo[k2][0]
                z2[1, k2, hi, :, sl] = xo[k2][1]

    norm = 1.0 / (S_LEN * DM)
    cscale = [jnp.where(lane0, norm, 2.0 * norm).astype(f32)] + [2.0 * norm] * 3 + [norm]

    def wperm(c, carry):
        @pl.when(c < 5)
        def _():
            unit_start(4 + c)

        for bb in range(2):
            blk_i = 2 * c + bb
            l0 = pl.multiple_of(blk_i * 128, 128)
            for i, (wt, wn) in enumerate(((wrt_v.bitcast(u32), wrn_v), (wit_v.bitcast(u32), win_v))):
                for t in range(5):
                    if t < 4:
                        w = wt[(t % 2) * 128:(t % 2 + 1) * 128, pl.ds(l0, 128)].reshape(8, 16, 128)
                        pk = (_lo_pair if t < 2 else _hi_pair)(w[:, :8, :], w[:, 8:, :])
                        blk = pltpu.bitcast(pk.reshape(64, 128), bf16)
                    else:
                        blk = jnp.broadcast_to(wn[:, pl.ds(l0, 128)], (128, 128))
                    o = jax.lax.dot_general(perm_ref[0], blk, nt_dims, preferred_element_type=f32)
                    wp_v[i, :, blk_i, :, t * 128:(t + 1) * 128] = (o * cscale[t]).reshape(16, 8, 128)
            stage_a(blk_i)
        return carry

    def build_xpre(sg, carry):
        r0 = pl.multiple_of(sg * SEG, SEG)
        xpre[pl.ds(pl.multiple_of(sg * 8, 8), 8), :] = x_v[pl.ds(r0, 16), :].astype(f32)[:8]
        return carry

    jax.lax.fori_loop(0, NSEG, build_xpre, 0, unroll=4)

    def precompute(p):
        for hd in (2 * p, 2 * p + 1):
            pre[hd] = jnp.dot(xpre[...], pltpu.bitcast(wqkv[3 * hd], bf16), preferred_element_type=f32)

    for cp in cp_small:
        cp.wait()
    small_ref[2] = small_ref[0] - small_ref[1]
    small_ref[3] = -small_ref[1] - small_ref[0]
    sub = jax.lax.broadcasted_iota(jnp.int32, (8, 128), 0)
    for part in range(2):
        for k2 in range(1, 16):
            v = jnp.zeros((8, 128), f32)
            for j in range(8):
                v = jnp.where(sub == j, tws_ref[512 + part * 128 + k2 * 8 + j], v)
            twb_ref[part, k2] = v
    gw_row[...] = gw_ref[...].astype(f32)

    for cp in cp_wt:
        cp.wait()
    jax.lax.fori_loop(0, 8, wperm, 0)

    def cdot3(m1, m2, m3, zr, zi):
        k1 = jnp.dot(m1, (zr + zi).astype(bf16), preferred_element_type=f32)
        k2 = jnp.dot(m2, zi.astype(bf16), preferred_element_type=f32)
        k3 = jnp.dot(m3, zr.astype(bf16), preferred_element_type=f32)
        return k1 - k2, k1 + k3

    def b_fwd(k2):
        tr, ti = tw_ref[pl.ds(k2, 1), :], tw_ref[pl.ds(16 + k2, 1), :]
        mr = small_ref[0] * tr - small_ref[1] * ti
        mi = small_ref[0] * ti + small_ref[1] * tr
        return cdot3(mr, mr + mi, mi - mr, z2[0, k2].reshape(128, 640), z2[1, k2].reshape(128, 640))

    def b_inv(k2, x):
        xr, xi = x
        wr = wp_v[0, k2].reshape(128, 640)
        wi = wp_v[1, k2].reshape(128, 640)
        pr = xr * wr - xi * wi
        pi = xr * wi + xi * wr
        gr, gi = cdot3(small_ref[0], small_ref[2], small_ref[3], pr, pi)
        z1[0, k2] = gr.reshape(16, 8, 640)
        z1[1, k2] = gi.reshape(16, 8, 640)

    def stage_b2(j, carry):
        @pl.when(j < 7)
        def _():
            unit_start(9 + j)

        xa = b_fwd(2 * j)
        xb = b_fwd(2 * j + 1)
        b_inv(2 * j, xa)
        b_inv(2 * j + 1, xb)
        return carry

    jax.lax.fori_loop(0, 8, stage_b2, 0)

    lane0a = jax.lax.broadcasted_iota(jnp.int32, (8, 128), 1) == 0

    def inv_twiddles(hi):
        tw_inv = [None]
        for k2 in range(1, 16):
            cr, ci = tws_ref[hi * 16 + k2], tws_ref[256 + hi * 16 + k2]
            br, bi = twb_ref[0, k2], twb_ref[1, k2]
            tw_inv.append((br * cr - bi * ci, br * ci + bi * cr))
        return tw_inv

    def a_inv_tile(hi, t, tw_inv, u_dst):
        sl = slice(t * 128, (t + 1) * 128)
        w = np.exp(2j * np.pi / 16.0)
        tmp = bt_scr.at[t % 2]
        for b in range(4):
            xin = []
            for a in range(4):
                k2 = 4 * a + b
                gr, gi = z1[0, k2, hi, :, sl], z1[1, k2, hi, :, sl]
                if k2 > 0:
                    tr, ti = tw_inv[k2]
                    gr, gi = gr * tr - gi * ti, gr * ti + gi * tr
                xin.append((gr, gi))
            col = _dft4(xin, +1)
            for c in range(4):
                v = col[c] if b * c == 0 else _cmul_const(col[c], w ** (b * c))
                tmp[0, b, c] = v[0]
                tmp[1, b, c] = v[1]
        for c in range(4):
            row = _dft4([(tmp[0, b, c], tmp[1, b, c]) for b in range(4)], +1)
            for d in range(4):
                s2 = c + 4 * d
                u_dst[s2, :, sl] = row[d][0]
                if t < 4:
                    u_dst[s2, :, 640 + t * 128:640 + (t + 1) * 128] = row[d][1]

    def stage_c2(m, carry):
        @pl.when(jnp.logical_and(m >= 2, m < 6))
        def _():
            cp_wo(2 * (m - 2)).start()
            cp_wo(2 * (m - 2) + 1).start()

        stage_c(2 * m, 2 * m + 1, u0, u1)
        stage_c(2 * m + 1, jnp.minimum(2 * m + 2, 15), u1, u0)
        return carry

    def stage_c(hi, nxt, u_src, u_dst):
        tw_inv = inv_twiddles(nxt)
        unit_repack(hi)
        precompute(hi)
        for t in range(5):
            a_inv_tile(nxt, t, tw_inv, u_dst)
        nyq = u_src[:, :, 512:513].reshape(128, 1)
        n = jnp.broadcast_to(nyq, (128, 128)) * sgn
        ue_r = u_src[:, :, 0:256].reshape(128, 256)
        uo_r = u_src[:, :, 256:512].reshape(128, 256)
        ue_i = u_src[:, :, 640:896].reshape(128, 256)
        uo_i = u_src[:, :, 896:1152].reshape(128, 256)
        for T in range(2):
            a0 = qdot_t(ue_r, C0, T) + n
            a1 = qdot_t(uo_r, C1, T)
            b0 = qdot_t(ue_i, S0, T)
            b1 = qdot_t(uo_i, S1F, T)
            if T == 0:
                b1 = jnp.where(lane0, 0.0, b1)
            p, q, pm, qm = a0 + a1, b0 + b1, a0 - a1, b0 - b1
            z2[0, :, hi, :, T * 128:(T + 1) * 128] = (p + q).reshape(16, 8, 128)
            z2[1, :, hi, :, T * 128:(T + 1) * 128] = (pm + qm).reshape(16, 8, 128)
            up_scr[T] = p - q
            up_scr[2 + T] = pm - qm
        s_e = jnp.sum((ue_r[:, :128] + ue_r[:, 128:]) * sgn_m, axis=1, keepdims=True) + nyq
        s_o = jnp.sum((uo_i[:, :128] + uo_i[:, 128:]) * sgn_m, axis=1, keepdims=True)
        z2[1, :, hi, :, 384:512] = rev(up_scr[0], up_scr[1]).reshape(16, 8, 128)
        z2[1, :, hi, :, 256:384] = rev(up_scr[1], s_e + s_o).reshape(16, 8, 128)
        z2[0, :, hi, :, 384:512] = rev(up_scr[2], up_scr[3]).reshape(16, 8, 128)
        z2[0, :, hi, :, 256:384] = rev(up_scr[3], s_e - s_o).reshape(16, 8, 128)

    tw0 = inv_twiddles(0)
    for t in range(5):
        a_inv_tile(0, t, tw0, u0)
    jax.lax.fori_loop(0, 8, stage_c2, 0)

    scale = DH ** -0.5
    rows = jax.lax.broadcasted_iota(jnp.int32, (L, L), 0)
    cols = jax.lax.broadcasted_iota(jnp.int32, (L, L), 1)
    mask = (rows < M) | (rows >= cols)
    wo32 = wo_v.bitcast(u32)

    def qkv_head(h, hd, p0):
        out = []
        for j in range(3):
            if j == 0:
                new = jnp.dot(h[0], pltpu.bitcast(wqkv[3 * hd + j], bf16), preferred_element_type=f32)
                out.append(jnp.concatenate([new[:8], pre[hd, pl.ds(p0, 8), :], new[8:]], axis=0))
            else:
                out.append(jnp.dot(h[1], pltpu.bitcast(wqkv[3 * hd + j], bf16), preferred_element_type=f32))
        return tuple(out)

    def scores(qkv):
        return jax.lax.dot_general(qkv[0], qkv[1].astype(bf16), nt_dims, preferred_element_type=f32)

    def softmax(s):
        s = jnp.where(mask, s * scale, -1e9)
        m = jnp.max(s, axis=-1, keepdims=True)
        p = jnp.exp(s - m)
        l = jnp.sum(p, axis=-1, keepdims=True)
        return p / l

    def pv(p, qkv):
        return jnp.dot(p, qkv[2].astype(bf16), preferred_element_type=f32)

    def cp_out(seg0, nseg):
        r0 = pl.multiple_of(seg0 * SEG, SEG)
        return pltpu.make_async_copy(out_v.at[pl.ds(r0, nseg * SEG)], out_hbm.at[pl.ds(r0, nseg * SEG)], sem_out)

    def mix(seg):
        r0 = pl.multiple_of(seg * SEG, SEG)
        xs = x_v[pl.ds(r0, SEG), :].astype(f32)
        gate = jax.nn.sigmoid(jnp.sum(xs * gw_row[...], axis=-1, keepdims=True))
        s2 = seg // 4
        hi0 = (seg % 4) * 4
        b = jnp.concatenate([z2[0, s2, pl.ds(hi0, 4), :, 0:512].reshape(SEG, 512),
                             z2[1, s2, pl.ds(hi0, 4), :, 0:512].reshape(SEG, 512)], axis=1)
        res = gate * a_scr[...] + (1.0 - gate) * b
        out_v[pl.ds(r0, SEG), :] = res.astype(out_v.dtype)


    def wo_part(h0, h1, n, lhs):
        w = pltpu.bitcast(wo32[n, h0 * (DH // 2):h1 * (DH // 2), :], bf16)
        return jnp.dot(lhs, w, preferred_element_type=f32)

    def step(s, mem):
        r0 = pl.multiple_of(s * SEG, SEG)
        xs = x_v[pl.ds(r0, SEG), :].astype(f32)
        h = (jnp.concatenate([mem, xs[8:]], axis=0),
             jnp.concatenate([mem, xs], axis=0))
        p0 = pl.multiple_of(s * 8, 8)
        qkvs, sc, ps, oh = {}, {}, {}, {}

        def wo_a(n):
            wa_scr[:, n * 128:(n + 1) * 128] = wo_part(0, HA, n, oa)

        for i in range(QL):
            qkvs[i] = qkv_head(h, i, p0)
        sc[0] = scores(qkvs[0])
        sc[1] = scores(qkvs[1])
        ps[0] = softmax(sc.pop(0))
        mix(jnp.maximum(s - 1, 0))
        for hd in range(H):
            if hd + QL < H:
                qkvs[hd + QL] = qkv_head(h, hd + QL, p0)
            for n in WO_SCHED.get((hd, 0), ()):
                wo_a(n)
            if hd + 2 < H:
                sc[hd + 2] = scores(qkvs[hd + 2])
            if hd + 1 < H:
                ps[hd + 1] = softmax(sc.pop(hd + 1))
            oh[hd] = pv(ps.pop(hd), qkvs.pop(hd))
            if hd == HA - 1:
                oa = jnp.concatenate([oh.pop(i) for i in range(HA)], axis=1)
            for n in WO_SCHED.get((hd, 1), ()):
                wo_a(n)
        ob = jnp.concatenate([oh.pop(i) for i in range(HA, H)], axis=1)
        out = wa_scr[...] + jnp.concatenate([wo_part(HA, H, n, ob) for n in range(8)], axis=1)
        a_scr[...] = out[M:]
        @pl.when(jnp.logical_and(s > 0, s % 4 == 1))
        def _():
            @pl.when(s > 1)
            def _():
                cp_out(s - 5, 4).start()

        return out[:M]

    for n in range(8):
        cp_wo(n).wait()
    a_scr[...] = jnp.zeros(a_scr.shape, f32)
    jax.lax.fori_loop(0, NSEG, step, mem_ref[...].astype(f32), unroll=UNROLL)
    mix(NSEG - 1)
    cp_out(NSEG - 4, 4).start()
    pltpu.make_async_copy(out_v.at[pl.ds(0, NSEG * SEG)], out_hbm.at[pl.ds(0, NSEG * SEG)], sem_out).wait()


@jax.jit
def _run(A_x, A_mem0, A_Wq, A_Wk, A_Wv, A_Wo, B_w_r, B_w_i, gate_w):
    any_spec = pl.BlockSpec(memory_space=pl.ANY)
    out = pl.pallas_call(
        _kernel,
        out_shape=jax.ShapeDtypeStruct((S_LEN, DM), A_x.dtype),
        in_specs=[any_spec] * 13,
        out_specs=any_spec,
        scratch_shapes=[
            pltpu.VMEM((M, DM), bf16),
            pltpu.VMEM((1, DM), bf16),
            pltpu.VMEM((1, DM), f32),
            pltpu.VMEM((2, 16, 8, 128), f32),
            pltpu.SMEM((768,), f32),
            pltpu.VMEM((4, 128, 128), f32),
            pltpu.VMEM((32, 128), f32),
            pltpu.VMEM((2, 128, 128), f32),
            pltpu.VMEM((S_LEN, DM), bf16),
            pltpu.VMEM((8, 128, 128), u32),
            pltpu.VMEM((DM // 2, S_LEN), bf16),
            pltpu.VMEM((DM // 2, S_LEN), bf16),
            pltpu.VMEM((1, S_LEN), bf16),
            pltpu.VMEM((1, S_LEN), bf16),
            pltpu.VMEM((2, 16, 16, 8, 640), f32),
            pltpu.VMEM((3 * H, DM // 2, DH), u32),
            pltpu.VMEM((8, H * DH, 128), bf16),
            pltpu.VMEM((2, 16, 16, 8, 640), f32),
            pltpu.VMEM((2, 16, 16, 8, 640), f32),
            pltpu.VMEM((16, 8, 1152), f32),
            pltpu.VMEM((16, 8, 1152), f32),
            pltpu.VMEM((2, 2, 4, 4, 8, 128), f32),
            pltpu.VMEM((4, 128, 128), f32),
            pltpu.VMEM((L, DM), f32),
            pltpu.VMEM((SEG, DM), f32),
            pltpu.VMEM((S_LEN, DM), bf16),
            pltpu.VMEM((NSEG * 8, DM), f32),
            pltpu.VMEM((H, NSEG * 8, DH), f32),
            pltpu.SemaphoreType.DMA((8,)),
            pltpu.SemaphoreType.DMA(()),
            pltpu.SemaphoreType.DMA((5,)),
            pltpu.SemaphoreType.DMA((4,)),
            pltpu.SemaphoreType.DMA((3 * H,)),
            pltpu.SemaphoreType.DMA((8,)),
            pltpu.SemaphoreType.DMA(()),
        ],
        compiler_params=pltpu.CompilerParams(vmem_limit_bytes=120 * 1024 * 1024),
    )(A_x.reshape(S_LEN, DM), A_mem0.reshape(M, DM),
      A_Wq.reshape(512, 64, DH), A_Wk.reshape(512, 64, DH), A_Wv.reshape(512, 64, DH),
      A_Wo.reshape(H * DH, DM), B_w_r.T, B_w_i.T, gate_w.reshape(1, DM),
      _CS, _TWS, _SMALL, _TW)
    return out.reshape(A_x.shape)


def pallas_gated_mix__memory_aug_recurrent_mem_tr__spectral_gfnet__prompt_kernel(
    A_x, A_mem0, A_Wq, A_Wk, A_Wv, A_Wo, A_seg_len, B_x, B_w_r, B_w_i, gate_w,
):
    del B_x
    assert int(A_seg_len) == SEG and A_x.shape == (1, S_LEN, DM)
    return _run(A_x, A_mem0, A_Wq, A_Wk, A_Wv, A_Wo, B_w_r, B_w_i, gate_w)
```

```python
import numpy as np
import ml_dtypes

import jax
import jax.numpy as jnp
import jax.experimental.pallas as pl
import jax.experimental.pallas.tpu as pltpu

S_LEN, DM, H, DH, M, SEG = 2048, 1024, 32, 128, 8, 32
L = M + SEG
NSEG = S_LEN // SEG
f32 = jnp.float32
bf16 = jnp.bfloat16
u32 = jnp.uint32
UNROLL = 4
QL = 4
HA = 26
WO_SCHED = {(27, 1): (0,), (28, 0): (1,), (28, 1): (2,), (29, 0): (3,), (29, 1): (4,), (30, 1): (5, 6), (31, 1): (7,)}


def _bf16_np(a):
    return np.asarray(a, np.float32).astype(ml_dtypes.bfloat16)


def _pack_rows_u32(a):
    b = _bf16_np(a).view(np.uint16).astype(np.uint32)
    return b[0::2] | (b[1::2] << 16)


def _make_consts():
    q = np.arange(DM // 4)
    th = 2.0 * np.pi / DM
    a0 = th * ((2 * np.outer(q, q)) % DM)
    a1 = th * ((np.outer(q, 2 * q + 1)) % DM)
    s1f = -np.sin(a1)
    s1f[0, :] = -np.cos(np.pi * q)
    mperm = 16 * (q // 16) + ((q % 16) >> 1) + 8 * (q & 1)
    fwd = [np.cos(a0), np.cos(a1), -np.sin(a0), s1f]
    cs = np.stack([_pack_rows_u32(m[:, mperm]) for m in fwd])
    cs = np.ascontiguousarray(cs.reshape(4, 128, 2, 128).transpose(0, 2, 1, 3)).reshape(8, 128, 128)

    i16 = np.arange(16)
    i128 = np.arange(128)
    d128 = np.exp(-2j * np.pi * ((np.outer(i128, i128)) % 128) / 128.0)
    small = np.stack([d128.real, d128.imag]).astype(np.float32)
    tw_f = np.exp(-2j * np.pi * np.outer(i16, i128) / 2048.0)
    tw = np.concatenate([tw_f.real, tw_f.imag]).astype(np.float32)
    return cs, small, tw


_CS, _SMALL, _TW = _make_consts()
NU = 16


def _lo_pair(a, b):
    return (a & np.uint32(0xFFFF)) | (b << 16)


def _hi_pair(a, b):
    return (a >> 16) | (b & np.uint32(0xFFFF0000))


def _cmul_const(x, c):
    re, im = x
    cr, ci = float(np.real(c)), float(np.imag(c))
    if abs(ci) < 1e-9:
        return (re, im) if cr > 0 else (-re, -im)
    if abs(cr) < 1e-9:
        return (-im, re) if ci > 0 else (im, -re)
    if abs(abs(cr) - abs(ci)) < 1e-9:
        a = abs(cr)
        sr, si = (1.0 if cr > 0 else -1.0), (1.0 if ci > 0 else -1.0)
        nr = (re if sr > 0 else -re) - (im if si > 0 else -im)
        ni = (re if si > 0 else -re) + (im if sr > 0 else -im)
        return (nr * a, ni * a)
    return (re * cr - im * ci, re * ci + im * cr)


def _dft4(x, sign):
    (ar, ai), (br, bi), (cr, ci), (dr, di) = x
    s0r, s0i = ar + cr, ai + ci
    s1r, s1i = ar - cr, ai - ci
    s2r, s2i = br + dr, bi + di
    s3r, s3i = br - dr, bi - di
    if sign < 0:
        return [(s0r + s2r, s0i + s2i), (s1r + s3i, s1i - s3r), (s0r - s2r, s0i - s2i), (s1r - s3i, s1i + s3r)]
    return [(s0r + s2r, s0i + s2i), (s1r - s3i, s1i + s3r), (s0r - s2r, s0i - s2i), (s1r + s3i, s1i - s3r)]


def _dft16(x, sign):
    w = np.exp(sign * 2j * np.pi / 16.0)
    t = [[None] * 4 for _ in range(4)]
    for b in range(4):
        col = _dft4([x[4 * a + b] for a in range(4)], sign)
        for c in range(4):
            t[b][c] = col[c] if b * c == 0 else _cmul_const(col[c], w ** (b * c))
    out = [None] * 16
    for c in range(4):
        row = _dft4([t[b][c] for b in range(4)], sign)
        for d in range(4):
            out[c + 4 * d] = row[d]
    return out


def _kernel(x_hbm, mem_hbm, wq_hbm, wk_hbm, wv_hbm, wo_hbm, wr_hbm, wi_hbm, gw_hbm,
            cs_hbm, small_hbm, tw_hbm,
            out_hbm,
            mem_ref, gw_ref, gw_row, small_ref, tw_ref, perm_ref,
            x_v, cs_v, wrt_v, wit_v, wrn_v, win_v, wp_v, wqkv, wo_v, z1, z2, u0, u1, bt_scr, up_scr, wa_scr, a_scr, out_v, xpre, pre,
            sem_x, sem_c, sem_s, sem_in, sem_w, sem_wo, sem_out):
    w32_hbm = tuple(w.bitcast(u32) for w in (wq_hbm, wk_hbm, wv_hbm))
    nt_dims = (((1,), (1,)), ((), ()))

    def cp_x(i):
        r0 = pl.multiple_of(i * 256, 256)
        return pltpu.make_async_copy(x_hbm.at[pl.ds(r0, 256)], x_v.at[pl.ds(r0, 256)], sem_x.at[i])

    cp_cs = pltpu.make_async_copy(cs_hbm, cs_v, sem_c)
    cp_wt, cp_wt2 = [], []
    for i, (src, dst, dstn) in enumerate(((wr_hbm, wrt_v, wrn_v), (wi_hbm, wit_v, win_v))):
        cp_wt.append(pltpu.make_async_copy(src.at[pl.ds(0, 512), pl.ds(0, 1024)], dst.at[:, pl.ds(0, 1024)], sem_in.at[3 * i]))
        cp_wt.append(pltpu.make_async_copy(src.at[pl.ds(512, 1)], dstn, sem_in.at[3 * i + 1]))
        cp_wt2.append(pltpu.make_async_copy(src.at[pl.ds(0, 512), pl.ds(1024, 1024)], dst.at[:, pl.ds(1024, 1024)], sem_in.at[3 * i + 2]))

    def cp_wo(n):
        return pltpu.make_async_copy(wo_hbm.at[:, pl.ds(n * 128, 128)], wo_v.at[n], sem_wo.at[n])

    def cp_w(p, par, which):
        t = 2 * p + par
        return pltpu.make_async_copy(w32_hbm[which].at[:, par * 16 + p], wqkv.at[3 * t + which],
                                     sem_w.at[3 * t + which])

    def unit_start(p):
        for par in range(2):
            for which in range(3):
                cp_w(p, par, which).start()

    def unit_repack(p):
        for par in range(2):
            for which in range(3):
                cp_w(p, par, which).wait()
        for which in range(3):
            ta = 6 * p + which
            tb = 6 * p + 3 + which
            for r in range(0, 512, 64):
                a = wqkv[ta, r:r + 64, :]
                b = wqkv[tb, r:r + 64, :]
                wqkv[ta, r:r + 64, :] = _lo_pair(a, b)
                wqkv[tb, r:r + 64, :] = _hi_pair(a, b)

    C0, C1, S0, S1F = range(4)

    def qdot(lhs, mat, nt):
        return jnp.dot(lhs, pltpu.bitcast(cs_v[2 * mat + nt], bf16), preferred_element_type=f32)

    def qdot_t(lhs, mat, dt):
        rows = jnp.concatenate([cs_v[2 * mat + kt, dt * 64:(dt + 1) * 64, :] for kt in range(2)], axis=1)
        return jax.lax.dot_general(lhs, pltpu.bitcast(rows, bf16), nt_dims, preferred_element_type=f32)

    def rev(t, first):
        return jnp.where(lane0, first, jnp.dot(t, perm_ref[1], preferred_element_type=f32))

    cp_small = [pltpu.make_async_copy(src, dst, sem_s.at[i]) for i, (src, dst) in enumerate((
        (small_hbm, small_ref), (tw_hbm, tw_ref),
        (mem_hbm, mem_ref), (gw_hbm, gw_ref)))]
    cp_cs.start()
    cp_x(0).start()
    cp_x(1).start()
    for cp in cp_small:
        cp.start()
    ri = jax.lax.broadcasted_iota(jnp.int32, (128, 128), 0)
    ci = jax.lax.broadcasted_iota(jnp.int32, (128, 128), 1)
    perm_ref[0] = (ci == (ri >> 3) + 16 * (ri & 7)).astype(f32) * (2.0 / (S_LEN * DM))
    perm_ref[1] = ((ri + ci == 128) & (ci >= 1)).astype(f32)

    lane_i = jax.lax.broadcasted_iota(jnp.int32, (1, 128), 1)
    lane0 = lane_i == 0
    sgn = (1 - 2 * (lane_i & 1)).astype(f32)
    half0 = jnp.where(lane0, 0.5, 1.0).astype(f32)
    sgn_m = (1 - 2 * ((lane_i >> 1) & 1)).astype(f32)

    def pro1(c, carry):
        @pl.when(c < 3)
        def _():
            cp_x(2 * c + 2).start()
            cp_x(2 * c + 3).start()

        @pl.when(c == 2)
        def _():
            for cp in cp_wt:
                cp.start()

        @pl.when(c == 4)
        def _():
            for cp in cp_wt2:
                cp.start()

        @pl.when(c >= 4)
        def _():
            unit_start(c - 4)

        cp_x(c).wait()
        r0 = pl.multiple_of(c * 256, 256)
        xt = [x_v[pl.ds(r0, 256), j * 128:(j + 1) * 128].astype(f32) for j in range(8)]
        zero = jnp.zeros((256, 128), f32)
        r1 = [rev(xt[7], zero), rev(xt[6], xt[7])]
        r2 = [rev(xt[3], zero), rev(xt[2], xt[3])]
        ee, eo, oe, oo = [], [], [], []
        for T in range(2):
            e1, o1 = xt[T] + r1[T], xt[T] - r1[T]
            e2, o2 = r2[T] + xt[4 + T], r2[T] - xt[4 + T]
            ee.append(e1 + e2)
            eo.append(e1 - e2)
            oe.append(o1 - o2)
            oo.append(o1 + o2)
        oo[0] = jnp.where(lane0, xt[2] - xt[6], oo[0])
        e256 = (xt[2] + xt[6])[:, 0:1]
        mid = jnp.broadcast_to(e256, (256, 128)) * sgn_m
        nyq = jnp.sum((ee[0] + ee[1]) * sgn, axis=1, keepdims=True) + e256
        ee, eo, oe, oo = (jnp.concatenate(v, axis=1) for v in (ee, eo, oe, oo))
        rr = pl.ds(2 * c, 2)
        for t in range(2):
            y0 = qdot(ee, C0, t) + mid
            if t == 0:
                y0 = y0 * half0
            z1[0, rr, :, :, t * 128:(t + 1) * 128] = y0.reshape(2, 16, 8, 128)
            z1[0, rr, :, :, (2 + t) * 128:(3 + t) * 128] = qdot(eo, C1, t).reshape(2, 16, 8, 128)
            z1[1, rr, :, :, t * 128:(t + 1) * 128] = qdot(oe, S0, t).reshape(2, 16, 8, 128)
            z1[1, rr, :, :, (2 + t) * 128:(3 + t) * 128] = qdot(oo, S1F, t).reshape(2, 16, 8, 128)
        z1[0, rr, :, :, 512:640] = jnp.where(lane0, 0.5 * nyq, 0.0).reshape(2, 16, 8, 128)
        z1[1, rr, :, :, 512:640] = jnp.zeros((2, 16, 8, 128), f32)
        return carry

    cp_cs.wait()
    jax.lax.fori_loop(0, 8, pro1, 0)

    def stage_a(hi):
        for t in range(5):
            sl = slice(t * 128, (t + 1) * 128)
            xin = [(z1[0, s2, hi, :, sl], z1[1, s2, hi, :, sl]) for s2 in range(16)]
            xo = _dft16(xin, -1)
            for k2 in range(16):
                z2[0, k2, hi, :, sl] = xo[k2][0]
                z2[1, k2, hi, :, sl] = xo[k2][1]


    def wperm(c, carry):
        @pl.when(c < 5)
        def _():
            unit_start(4 + c)

        @pl.when(c == 4)
        def _():
            for cp in cp_wt2:
                cp.wait()

        for bb in range(2):
            blk_i = 2 * c + bb
            l0 = pl.multiple_of(blk_i * 128, 128)
            for i, (wt, wn) in enumerate(((wrt_v.bitcast(u32), wrn_v), (wit_v.bitcast(u32), win_v))):
                for t in range(5):
                    if t < 4:
                        w = wt[(t % 2) * 128:(t % 2 + 1) * 128, pl.ds(l0, 128)].reshape(8, 16, 128)
                        pk = (_lo_pair if t < 2 else _hi_pair)(w[:, :8, :], w[:, 8:, :])
                        blk = pltpu.bitcast(pk.reshape(64, 128), bf16)
                    else:
                        blk = jnp.broadcast_to(wn[:, pl.ds(l0, 128)], (128, 128))
                    o = jax.lax.dot_general(perm_ref[0], blk, nt_dims, preferred_element_type=f32)
                    wp_v[i, :, blk_i, :, t * 128:(t + 1) * 128] = o.reshape(16, 8, 128)
            stage_a(blk_i)
        return carry

    def build_xpre(sg, carry):
        r0 = pl.multiple_of(sg * SEG, SEG)
        xpre[pl.ds(pl.multiple_of(sg * 8, 8), 8), :] = x_v[pl.ds(r0, 16), :].astype(f32)[:8]
        return carry

    jax.lax.fori_loop(0, NSEG, build_xpre, 0, unroll=4)

    def precompute(p):
        for hd in (2 * p, 2 * p + 1):
            pre[hd] = jnp.dot(xpre[...], pltpu.bitcast(wqkv[3 * hd], bf16), preferred_element_type=f32)

    for cp in cp_small:
        cp.wait()
    gw_row[...] = gw_ref[...].astype(f32)

    for cp in cp_wt:
        cp.wait()
    jax.lax.fori_loop(0, 8, wperm, 0)

    def cdot3(m1, m2, m3, zr, zi, dims=(((1,), (0,)), ((), ()))):
        k1 = jax.lax.dot_general(m1, (zr + zi).astype(bf16), dims, preferred_element_type=f32)
        k2 = jax.lax.dot_general(m2, zi.astype(bf16), dims, preferred_element_type=f32)
        k3 = jax.lax.dot_general(m3, zr.astype(bf16), dims, preferred_element_type=f32)
        return k1 - k2, k1 + k3

    def b_fwd(k2):
        tr, ti = tw_ref[pl.ds(k2, 1), :], tw_ref[pl.ds(16 + k2, 1), :]
        mr = small_ref[0] * tr - small_ref[1] * ti
        mi = small_ref[0] * ti + small_ref[1] * tr
        return cdot3(mr, mr + mi, mi - mr, z2[0, k2].reshape(128, 640), z2[1, k2].reshape(128, 640)), (mr, mi)

    def b_inv(k2, x):
        (xr, xi), (mr, mi) = x
        wr = wp_v[0, k2].reshape(128, 640)
        wi = wp_v[1, k2].reshape(128, 640)
        pr = xr * wr - xi * wi
        pi = xr * wi + xi * wr
        gr, gi = cdot3(mr, mr - mi, -mi - mr, pr, pi, (((0,), (0,)), ((), ())))
        z1[0, k2] = gr.reshape(16, 8, 640)
        z1[1, k2] = gi.reshape(16, 8, 640)

    def stage_b2(j, carry):
        for u in range(2):
            @pl.when(9 + 2 * j + u < NU)
            def _():
                unit_start(9 + 2 * j + u)

        k = 4 * j
        xa = b_fwd(k)
        xb = b_fwd(k + 1)
        b_inv(k, xa)
        xc = b_fwd(k + 2)
        b_inv(k + 1, xb)
        xd = b_fwd(k + 3)
        b_inv(k + 2, xc)
        b_inv(k + 3, xd)
        return carry

    jax.lax.fori_loop(0, 4, stage_b2, 0)

    def a_inv_tile(hi, t, u_dst):
        sl = slice(t * 128, (t + 1) * 128)
        w = np.exp(2j * np.pi / 16.0)
        tmp = bt_scr.at[t % 2]
        for b in range(4):
            xin = []
            for a in range(4):
                k2 = 4 * a + b
                gr, gi = z1[0, k2, hi, :, sl], z1[1, k2, hi, :, sl]
                xin.append((gr, gi))
            col = _dft4(xin, +1)
            for c in range(4):
                v = col[c] if b * c == 0 else _cmul_const(col[c], w ** (b * c))
                tmp[0, b, c] = v[0]
                tmp[1, b, c] = v[1]
        for c in range(4):
            row = _dft4([(tmp[0, b, c], tmp[1, b, c]) for b in range(4)], +1)
            for d in range(4):
                s2 = c + 4 * d
                u_dst[s2, :, sl] = row[d][0]
                if t < 4:
                    u_dst[s2, :, 640 + t * 128:640 + (t + 1) * 128] = row[d][1]

    def stage_c2(m, carry):
        @pl.when(jnp.logical_and(m >= 2, m < 6))
        def _():
            cp_wo(2 * (m - 2)).start()
            cp_wo(2 * (m - 2) + 1).start()

        stage_c(2 * m, 2 * m + 1, u0, u1)
        stage_c(2 * m + 1, jnp.minimum(2 * m + 2, 15), u1, u0)
        return carry

    def stage_c(hi, nxt, u_src, u_dst):
        unit_repack(hi)
        precompute(hi)
        for t in range(5):
            a_inv_tile(nxt, t, u_dst)
        nyq = u_src[:, :, 512:513].reshape(128, 1)
        n = jnp.broadcast_to(nyq, (128, 128)) * sgn
        ue_r = u_src[:, :, 0:256].reshape(128, 256)
        uo_r = u_src[:, :, 256:512].reshape(128, 256)
        ue_i = u_src[:, :, 640:896].reshape(128, 256)
        uo_i = u_src[:, :, 896:1152].reshape(128, 256)
        for T in range(2):
            a0 = qdot_t(ue_r, C0, T) + n
            a1 = qdot_t(uo_r, C1, T)
            b0 = qdot_t(ue_i, S0, T)
            b1 = qdot_t(uo_i, S1F, T)
            if T == 0:
                b1 = jnp.where(lane0, 0.0, b1)
            p, q, pm, qm = a0 + a1, b0 + b1, a0 - a1, b0 - b1
            z2[0, :, hi, :, T * 128:(T + 1) * 128] = (p + q).reshape(16, 8, 128)
            z2[1, :, hi, :, T * 128:(T + 1) * 128] = (pm + qm).reshape(16, 8, 128)
            up_scr[T] = p - q
            up_scr[2 + T] = pm - qm
        s_e = jnp.sum((ue_r[:, :128] + ue_r[:, 128:]) * sgn_m, axis=1, keepdims=True) + nyq
        s_o = jnp.sum((uo_i[:, :128] + uo_i[:, 128:]) * sgn_m, axis=1, keepdims=True)
        z2[1, :, hi, :, 384:512] = rev(up_scr[0], up_scr[1]).reshape(16, 8, 128)
        z2[1, :, hi, :, 256:384] = rev(up_scr[1], s_e + s_o).reshape(16, 8, 128)
        z2[0, :, hi, :, 384:512] = rev(up_scr[2], up_scr[3]).reshape(16, 8, 128)
        z2[0, :, hi, :, 256:384] = rev(up_scr[3], s_e - s_o).reshape(16, 8, 128)

    for t in range(5):
        a_inv_tile(0, t, u0)
    jax.lax.fori_loop(0, 8, stage_c2, 0)

    scale = DH ** -0.5
    rows = jax.lax.broadcasted_iota(jnp.int32, (L, L), 0)
    cols = jax.lax.broadcasted_iota(jnp.int32, (L, L), 1)
    mask = (rows < M) | (rows >= cols)
    wo32 = wo_v.bitcast(u32)

    def qkv_head(h, hd, p0):
        out = []
        for j in range(3):
            if j == 0:
                new = jnp.dot(h[0], pltpu.bitcast(wqkv[3 * hd + j], bf16), preferred_element_type=f32)
                out.append(jnp.concatenate([new[:8], pre[hd, pl.ds(p0, 8), :], new[8:]], axis=0))
            else:
                out.append(jnp.dot(h[1], pltpu.bitcast(wqkv[3 * hd + j], bf16), preferred_element_type=f32))
        return tuple(out)

    def scores(qkv):
        return jax.lax.dot_general(qkv[0], qkv[1].astype(bf16), nt_dims, preferred_element_type=f32)

    def softmax(s):
        s = jnp.where(mask, s * scale, -1e9)
        m = jnp.max(s, axis=-1, keepdims=True)
        p = jnp.exp(s - m)
        l = jnp.sum(p, axis=-1, keepdims=True)
        return p / l

    def pv(p, qkv):
        return jnp.dot(p, qkv[2].astype(bf16), preferred_element_type=f32)

    def cp_out(seg0, nseg):
        r0 = pl.multiple_of(seg0 * SEG, SEG)
        return pltpu.make_async_copy(out_v.at[pl.ds(r0, nseg * SEG)], out_hbm.at[pl.ds(r0, nseg * SEG)], sem_out)

    def mix(seg):
        r0 = pl.multiple_of(seg * SEG, SEG)
        xs = x_v[pl.ds(r0, SEG), :].astype(f32)
        gate = jax.nn.sigmoid(jnp.sum(xs * gw_row[...], axis=-1, keepdims=True))
        s2 = seg // 4
        hi0 = (seg % 4) * 4
        b = jnp.concatenate([z2[0, s2, pl.ds(hi0, 4), :, 0:512].reshape(SEG, 512),
                             z2[1, s2, pl.ds(hi0, 4), :, 0:512].reshape(SEG, 512)], axis=1)
        res = gate * a_scr[...] + (1.0 - gate) * b
        out_v[pl.ds(r0, SEG), :] = res.astype(out_v.dtype)


    def wo_part(h0, h1, n, lhs):
        w = pltpu.bitcast(wo32[n, h0 * (DH // 2):h1 * (DH // 2), :], bf16)
        return jnp.dot(lhs, w, preferred_element_type=f32)

    def step(s, mem):
        r0 = pl.multiple_of(s * SEG, SEG)
        xs = x_v[pl.ds(r0, SEG), :].astype(f32)
        h = (jnp.concatenate([mem, xs[8:]], axis=0),
             jnp.concatenate([mem, xs], axis=0))
        p0 = pl.multiple_of(s * 8, 8)
        qkvs, sc, ps, oh = {}, {}, {}, {}

        def wo_a(n):
            wa_scr[:, n * 128:(n + 1) * 128] = wo_part(0, HA, n, oa)

        for i in range(QL):
            qkvs[i] = qkv_head(h, i, p0)
        sc[0] = scores(qkvs[0])
        sc[1] = scores(qkvs[1])
        ps[0] = softmax(sc.pop(0))
        mix(jnp.maximum(s - 1, 0))

        @pl.when(s == NSEG - 1)
        def _():
            cp_out(NSEG - 4, 3).start()

        for hd in range(H):
            if hd + QL < H:
                qkvs[hd + QL] = qkv_head(h, hd + QL, p0)
            for n in WO_SCHED.get((hd, 0), ()):
                wo_a(n)
            if hd + 2 < H:
                sc[hd + 2] = scores(qkvs[hd + 2])
            if hd + 1 < H:
                ps[hd + 1] = softmax(sc.pop(hd + 1))
            oh[hd] = pv(ps.pop(hd), qkvs.pop(hd))
            if hd == HA - 1:
                oa = jnp.concatenate([oh.pop(i) for i in range(HA)], axis=1)
            for n in WO_SCHED.get((hd, 1), ()):
                wo_a(n)
        ob = jnp.concatenate([oh.pop(i) for i in range(HA, H)], axis=1)
        out = wa_scr[...] + jnp.concatenate([wo_part(HA, H, n, ob) for n in range(8)], axis=1)
        a_scr[...] = out[M:]
        @pl.when(jnp.logical_and(s > 0, s % 4 == 1))
        def _():
            @pl.when(s > 1)
            def _():
                cp_out(s - 5, 4).start()

        return out[:M]

    for n in range(8):
        cp_wo(n).wait()
    a_scr[...] = jnp.zeros(a_scr.shape, f32)
    jax.lax.fori_loop(0, NSEG, step, mem_ref[...].astype(f32), unroll=UNROLL)
    mix(NSEG - 1)
    cp_out(NSEG - 1, 1).start()
    pltpu.make_async_copy(out_v.at[pl.ds(0, NSEG * SEG)], out_hbm.at[pl.ds(0, NSEG * SEG)], sem_out).wait()


@jax.jit
def _run(A_x, A_mem0, A_Wq, A_Wk, A_Wv, A_Wo, B_w_r, B_w_i, gate_w):
    any_spec = pl.BlockSpec(memory_space=pl.ANY)
    out = pl.pallas_call(
        _kernel,
        out_shape=jax.ShapeDtypeStruct((S_LEN, DM), A_x.dtype),
        in_specs=[any_spec] * 12,
        out_specs=any_spec,
        scratch_shapes=[
            pltpu.VMEM((M, DM), bf16),
            pltpu.VMEM((1, DM), bf16),
            pltpu.VMEM((1, DM), f32),
            pltpu.VMEM((2, 128, 128), f32),
            pltpu.VMEM((32, 128), f32),
            pltpu.VMEM((2, 128, 128), f32),
            pltpu.VMEM((S_LEN, DM), bf16),
            pltpu.VMEM((8, 128, 128), u32),
            pltpu.VMEM((DM // 2, S_LEN), bf16),
            pltpu.VMEM((DM // 2, S_LEN), bf16),
            pltpu.VMEM((1, S_LEN), bf16),
            pltpu.VMEM((1, S_LEN), bf16),
            pltpu.VMEM((2, 16, 16, 8, 640), f32),
            pltpu.VMEM((3 * H, DM // 2, DH), u32),
            pltpu.VMEM((8, H * DH, 128), bf16),
            pltpu.VMEM((2, 16, 16, 8, 640), f32),
            pltpu.VMEM((2, 16, 16, 8, 640), f32),
            pltpu.VMEM((16, 8, 1152), f32),
            pltpu.VMEM((16, 8, 1152), f32),
            pltpu.VMEM((2, 2, 4, 4, 8, 128), f32),
            pltpu.VMEM((4, 128, 128), f32),
            pltpu.VMEM((L, DM), f32),
            pltpu.VMEM((SEG, DM), f32),
            pltpu.VMEM((S_LEN, DM), bf16),
            pltpu.VMEM((NSEG * 8, DM), f32),
            pltpu.VMEM((H, NSEG * 8, DH), f32),
            pltpu.SemaphoreType.DMA((8,)),
            pltpu.SemaphoreType.DMA(()),
            pltpu.SemaphoreType.DMA((4,)),
            pltpu.SemaphoreType.DMA((6,)),
            pltpu.SemaphoreType.DMA((3 * H,)),
            pltpu.SemaphoreType.DMA((8,)),
            pltpu.SemaphoreType.DMA(()),
        ],
        compiler_params=pltpu.CompilerParams(vmem_limit_bytes=120 * 1024 * 1024),
    )(A_x.reshape(S_LEN, DM), A_mem0.reshape(M, DM),
      A_Wq.reshape(512, 64, DH), A_Wk.reshape(512, 64, DH), A_Wv.reshape(512, 64, DH),
      A_Wo.reshape(H * DH, DM), B_w_r.T, B_w_i.T, gate_w.reshape(1, DM),
      _CS, _SMALL, _TW)
    return out.reshape(A_x.shape)


def pallas_gated_mix__memory_aug_recurrent_mem_tr__spectral_gfnet__prompt_kernel(
    A_x, A_mem0, A_Wq, A_Wk, A_Wv, A_Wo, A_seg_len, B_x, B_w_r, B_w_i, gate_w,
):
    del B_x
    assert int(A_seg_len) == SEG and A_x.shape == (1, S_LEN, DM)
    return _run(A_x, A_mem0, A_Wq, A_Wk, A_Wv, A_Wo, B_w_r, B_w_i, gate_w)
```

```python
import numpy as np
import ml_dtypes

import jax
import jax.numpy as jnp
import jax.experimental.pallas as pl
import jax.experimental.pallas.tpu as pltpu

S_LEN, DM, H, DH, M, SEG = 2048, 1024, 32, 128, 8, 32
L = M + SEG
NSEG = S_LEN // SEG
f32 = jnp.float32
bf16 = jnp.bfloat16
u32 = jnp.uint32
UNROLL = 4
QL = 4
HA = 26
WO_SCHED = {(27, 1): (0,), (28, 0): (1,), (28, 1): (2,), (29, 0): (3,), (29, 1): (4,), (30, 1): (5, 6), (31, 1): (7,)}


def _bf16_np(a):
    return np.asarray(a, np.float32).astype(ml_dtypes.bfloat16)


def _pack_rows_u32(a):
    b = _bf16_np(a).view(np.uint16).astype(np.uint32)
    return b[0::2] | (b[1::2] << 16)


def _make_consts():
    q = np.arange(DM // 4)
    th = 2.0 * np.pi / DM
    a0 = th * ((2 * np.outer(q, q)) % DM)
    a1 = th * ((np.outer(q, 2 * q + 1)) % DM)
    s1f = -np.sin(a1)
    s1f[0, :] = -np.cos(np.pi * q)
    mperm = 16 * (q // 16) + ((q % 16) >> 1) + 8 * (q & 1)
    fwd = [np.cos(a0), np.cos(a1), -np.sin(a0), s1f]
    cs = np.stack([_pack_rows_u32(m[:, mperm]) for m in fwd])
    cs = np.ascontiguousarray(cs.reshape(4, 128, 2, 128).transpose(0, 2, 1, 3)).reshape(8, 128, 128)

    i16 = np.arange(16)
    i128 = np.arange(128)
    d128 = np.exp(-2j * np.pi * ((np.outer(i128, i128)) % 128) / 128.0)
    small = np.stack([d128.real, d128.imag]).astype(np.float32)
    tw_f = np.exp(-2j * np.pi * np.outer(i16, i128) / 2048.0)
    tw = np.concatenate([tw_f.real, tw_f.imag]).astype(np.float32)
    return cs, small, tw


_CS, _SMALL, _TW = _make_consts()
NU = 16


def _lo_pair(a, b):
    return (a & np.uint32(0xFFFF)) | (b << 16)


def _hi_pair(a, b):
    return (a >> 16) | (b & np.uint32(0xFFFF0000))


def _is0(a):
    return isinstance(a, int) and a == 0


def _neg(a):
    return 0 if _is0(a) else -a


def _add(a, b):
    return b if _is0(a) else a if _is0(b) else a + b


def _sub(a, b):
    return _neg(b) if _is0(a) else a if _is0(b) else a - b


def _mul(a, c):
    return 0 if _is0(a) else a * c


def _cmul_const(x, c):
    re, im = x
    cr, ci = float(np.real(c)), float(np.imag(c))
    if abs(ci) < 1e-9:
        return (re, im) if cr > 0 else (_neg(re), _neg(im))
    if abs(cr) < 1e-9:
        return (_neg(im), re) if ci > 0 else (im, _neg(re))
    if abs(abs(cr) - abs(ci)) < 1e-9:
        a = abs(cr)
        if cr > 0:
            nr, ni = (_sub(re, im), _add(re, im)) if ci > 0 else (_add(re, im), _sub(im, re))
            return (_mul(nr, a), _mul(ni, a))
        nr, ni = (_add(re, im), _sub(im, re)) if ci > 0 else (_sub(im, re), _add(re, im))
        return (_mul(nr, -a), _mul(ni, -a)) if ci > 0 else (_mul(nr, a), _mul(ni, -a))
    return (_sub(_mul(re, cr), _mul(im, ci)), _add(_mul(re, ci), _mul(im, cr)))


def _dft4(x, sign):
    (ar, ai), (br, bi), (cr, ci), (dr, di) = x
    s0r, s0i = _add(ar, cr), _add(ai, ci)
    s1r, s1i = _sub(ar, cr), _sub(ai, ci)
    s2r, s2i = _add(br, dr), _add(bi, di)
    s3r, s3i = _sub(br, dr), _sub(bi, di)
    even, odd = (_add(s0r, s2r), _add(s0i, s2i)), (_sub(s0r, s2r), _sub(s0i, s2i))
    if sign < 0:
        return [even, (_add(s1r, s3i), _sub(s1i, s3r)), odd, (_sub(s1r, s3i), _add(s1i, s3r))]
    return [even, (_sub(s1r, s3i), _add(s1i, s3r)), odd, (_add(s1r, s3i), _sub(s1i, s3r))]


def _dft16(x, sign):
    w = np.exp(sign * 2j * np.pi / 16.0)
    t = [[None] * 4 for _ in range(4)]
    for b in range(4):
        col = _dft4([x[4 * a + b] for a in range(4)], sign)
        for c in range(4):
            t[b][c] = col[c] if b * c == 0 else _cmul_const(col[c], w ** (b * c))
    out = [None] * 16
    for c in range(4):
        row = _dft4([t[b][c] for b in range(4)], sign)
        for d in range(4):
            out[c + 4 * d] = row[d]
    return out


def _kernel(x_hbm, mem_hbm, wq_hbm, wk_hbm, wv_hbm, wo_hbm, wr_hbm, wi_hbm, gw_hbm,
            cs_hbm, small_hbm, tw_hbm,
            out_hbm,
            mem_ref, gw_ref, gw_row, small_ref, tw_ref, perm_ref,
            x_v, cs_v, wrt_v, wit_v, wrn_v, win_v, wp_v, wqkv, wo_v, z1, z2, u0, u1, bt_scr, up_scr, wa_scr, a_scr, out_v, xpre, pre,
            sem_x, sem_c, sem_s, sem_in, sem_w, sem_wo, sem_out):
    w32_hbm = tuple(w.bitcast(u32) for w in (wq_hbm, wk_hbm, wv_hbm))
    nt_dims = (((1,), (1,)), ((), ()))

    def cp_x(i):
        r0 = pl.multiple_of(i * 256, 256)
        return pltpu.make_async_copy(x_hbm.at[pl.ds(r0, 256)], x_v.at[pl.ds(r0, 256)], sem_x.at[i])

    cp_cs = pltpu.make_async_copy(cs_hbm, cs_v, sem_c)
    cp_wt, cp_wt2 = [], []
    for i, (src, dst, dstn) in enumerate(((wr_hbm, wrt_v, wrn_v), (wi_hbm, wit_v, win_v))):
        cp_wt.append(pltpu.make_async_copy(src.at[pl.ds(0, 512), pl.ds(0, 1024)], dst.at[:, pl.ds(0, 1024)], sem_in.at[3 * i]))
        cp_wt.append(pltpu.make_async_copy(src.at[pl.ds(512, 1)], dstn, sem_in.at[3 * i + 1]))
        cp_wt2.append(pltpu.make_async_copy(src.at[pl.ds(0, 512), pl.ds(1024, 1024)], dst.at[:, pl.ds(1024, 1024)], sem_in.at[3 * i + 2]))

    def cp_wo(n):
        return pltpu.make_async_copy(wo_hbm.at[:, pl.ds(n * 128, 128)], wo_v.at[n], sem_wo.at[n])

    def cp_w(p, par, which):
        t = 2 * p + par
        return pltpu.make_async_copy(w32_hbm[which].at[:, par * 16 + p], wqkv.at[3 * t + which],
                                     sem_w.at[3 * t + which])

    def unit_start(p):
        for par in range(2):
            for which in range(3):
                cp_w(p, par, which).start()

    def unit_repack(p):
        for par in range(2):
            for which in range(3):
                cp_w(p, par, which).wait()
        for which in range(3):
            ta = 6 * p + which
            tb = 6 * p + 3 + which
            for r in range(0, 512, 64):
                a = wqkv[ta, r:r + 64, :]
                b = wqkv[tb, r:r + 64, :]
                wqkv[ta, r:r + 64, :] = _lo_pair(a, b)
                wqkv[tb, r:r + 64, :] = _hi_pair(a, b)

    C0, C1, S0, S1F = range(4)

    def qdot(lhs, mat, nt):
        return jnp.dot(lhs, pltpu.bitcast(cs_v[2 * mat + nt], bf16), preferred_element_type=f32)

    def qdot_t(lhs, mat, dt):
        rows = jnp.concatenate([cs_v[2 * mat + kt, dt * 64:(dt + 1) * 64, :] for kt in range(2)], axis=1)
        return jax.lax.dot_general(lhs, pltpu.bitcast(rows, bf16), nt_dims, preferred_element_type=f32)

    def rev(t, first):
        return jnp.where(lane0, first, jnp.dot(t, perm_ref[1], preferred_element_type=f32))

    cp_small = [pltpu.make_async_copy(src, dst, sem_s.at[i]) for i, (src, dst) in enumerate((
        (small_hbm, small_ref), (tw_hbm, tw_ref),
        (mem_hbm, mem_ref), (gw_hbm, gw_ref)))]
    cp_cs.start()
    cp_x(0).start()
    cp_x(1).start()
    for cp in cp_small:
        cp.start()
    ri = jax.lax.broadcasted_iota(jnp.int32, (128, 128), 0)
    ci = jax.lax.broadcasted_iota(jnp.int32, (128, 128), 1)
    perm_ref[0] = (ci == (ri >> 3) + 16 * (ri & 7)).astype(f32) * (2.0 / (S_LEN * DM))
    perm_ref[1] = ((ri + ci == 128) & (ci >= 1)).astype(f32)

    lane_i = jax.lax.broadcasted_iota(jnp.int32, (1, 128), 1)
    lane0 = lane_i == 0
    sgn = (1 - 2 * (lane_i & 1)).astype(f32)
    half0 = jnp.where(lane0, 0.5, 1.0).astype(f32)
    sgn_m = (1 - 2 * ((lane_i >> 1) & 1)).astype(f32)

    def pro1(c, carry):
        @pl.when(c < 3)
        def _():
            cp_x(2 * c + 2).start()
            cp_x(2 * c + 3).start()

        @pl.when(c == 2)
        def _():
            for cp in cp_wt:
                cp.start()

        @pl.when(c == 4)
        def _():
            for cp in cp_wt2:
                cp.start()

        @pl.when(c >= 4)
        def _():
            unit_start(c - 4)

        cp_x(c).wait()
        r0 = pl.multiple_of(c * 256, 256)
        xt = [x_v[pl.ds(r0, 256), j * 128:(j + 1) * 128].astype(f32) for j in range(8)]
        for j in range(8):
            xpre[pl.ds(pl.multiple_of(c * 64, 64), 64), j * 128:(j + 1) * 128] = (
                xt[j].reshape(8, 32, 128)[:, :8, :].reshape(64, 128))
        zero = jnp.zeros((256, 128), f32)
        r1 = [rev(xt[7], zero), rev(xt[6], xt[7])]
        r2 = [rev(xt[3], zero), rev(xt[2], xt[3])]
        ee, eo, oe, oo = [], [], [], []
        for T in range(2):
            e1, o1 = xt[T] + r1[T], xt[T] - r1[T]
            e2, o2 = r2[T] + xt[4 + T], r2[T] - xt[4 + T]
            ee.append(e1 + e2)
            eo.append(e1 - e2)
            oe.append(o1 - o2)
            oo.append(o1 + o2)
        oo[0] = jnp.where(lane0, xt[2] - xt[6], oo[0])
        e256 = (xt[2] + xt[6])[:, 0:1]
        mid = jnp.broadcast_to(e256, (256, 128)) * sgn_m
        nyq = jnp.sum((ee[0] + ee[1]) * sgn, axis=1, keepdims=True) + e256
        ee, eo, oe, oo = (jnp.concatenate(v, axis=1) for v in (ee, eo, oe, oo))
        rr = pl.ds(2 * c, 2)
        for t in range(2):
            y0 = qdot(ee, C0, t) + mid
            if t == 0:
                y0 = y0 * half0
            z1[0, rr, :, :, t * 128:(t + 1) * 128] = y0.reshape(2, 16, 8, 128)
            z1[0, rr, :, :, (2 + t) * 128:(3 + t) * 128] = qdot(eo, C1, t).reshape(2, 16, 8, 128)
            z1[1, rr, :, :, t * 128:(t + 1) * 128] = qdot(oe, S0, t).reshape(2, 16, 8, 128)
            z1[1, rr, :, :, (2 + t) * 128:(3 + t) * 128] = qdot(oo, S1F, t).reshape(2, 16, 8, 128)
        z1[0, rr, :, :, 512:640] = jnp.where(lane0, 0.5 * nyq, 0.0).reshape(2, 16, 8, 128)
        return carry

    cp_cs.wait()
    jax.lax.fori_loop(0, 8, pro1, 0)

    def stage_a(hi):
        for t in range(5):
            sl = slice(t * 128, (t + 1) * 128)
            xin = [(z1[0, s2, hi, :, sl], z1[1, s2, hi, :, sl] if t < 4 else 0) for s2 in range(16)]
            xo = _dft16(xin, -1)
            for k2 in range(16):
                z2[0, k2, hi, :, sl] = xo[k2][0]
                z2[1, k2, hi, :, sl] = jnp.zeros((8, 128), f32) if _is0(xo[k2][1]) else xo[k2][1]


    def wperm(c, carry):
        @pl.when(c < 5)
        def _():
            unit_start(4 + c)

        @pl.when(c == 4)
        def _():
            for cp in cp_wt2:
                cp.wait()

        for bb in range(2):
            blk_i = 2 * c + bb
            l0 = pl.multiple_of(blk_i * 128, 128)
            for i, (wt, wn) in enumerate(((wrt_v.bitcast(u32), wrn_v), (wit_v.bitcast(u32), win_v))):
                for t in range(5):
                    if t < 4:
                        w = wt[(t % 2) * 128:(t % 2 + 1) * 128, pl.ds(l0, 128)].reshape(8, 16, 128)
                        pk = (_lo_pair if t < 2 else _hi_pair)(w[:, :8, :], w[:, 8:, :])
                        blk = pltpu.bitcast(pk.reshape(64, 128), bf16)
                    else:
                        blk = jnp.broadcast_to(wn[:, pl.ds(l0, 128)], (128, 128))
                    o = jax.lax.dot_general(perm_ref[0], blk, nt_dims, preferred_element_type=f32)
                    wp_v[i, :, blk_i, :, t * 128:(t + 1) * 128] = o.reshape(16, 8, 128)
            stage_a(blk_i)
        return carry

    def precompute(p):
        for hd in (2 * p, 2 * p + 1):
            pre[hd] = jnp.dot(xpre[...], pltpu.bitcast(wqkv[3 * hd], bf16), preferred_element_type=f32)

    for cp in cp_small:
        cp.wait()
    gw_row[...] = gw_ref[...].astype(f32)

    for cp in cp_wt:
        cp.wait()
    jax.lax.fori_loop(0, 8, wperm, 0)

    def cdot3(m1, m2, m3, zr, zi, dims=(((1,), (0,)), ((), ()))):
        k1 = jax.lax.dot_general(m1, (zr + zi).astype(bf16), dims, preferred_element_type=f32)
        k2 = jax.lax.dot_general(m2, zi.astype(bf16), dims, preferred_element_type=f32)
        k3 = jax.lax.dot_general(m3, zr.astype(bf16), dims, preferred_element_type=f32)
        return k1 - k2, k1 + k3

    def b_fwd(k2):
        tr, ti = tw_ref[pl.ds(k2, 1), :], tw_ref[pl.ds(16 + k2, 1), :]
        mr = small_ref[0] * tr - small_ref[1] * ti
        mi = small_ref[0] * ti + small_ref[1] * tr
        return cdot3(mr, mr + mi, mi - mr, z2[0, k2].reshape(128, 640), z2[1, k2].reshape(128, 640)), (mr, mi)

    def b_inv(k2, x):
        (xr, xi), (mr, mi) = x
        wr = wp_v[0, k2].reshape(128, 640)
        wi = wp_v[1, k2].reshape(128, 640)
        pr = xr * wr - xi * wi
        pi = xr * wi + xi * wr
        gr, gi = cdot3(mr, mr - mi, -mi - mr, pr, pi, (((0,), (0,)), ((), ())))
        z1[0, k2] = gr.reshape(16, 8, 640)
        z1[1, k2] = gi.reshape(16, 8, 640)

    def stage_b2(j, carry):
        for u in range(2):
            @pl.when(9 + 2 * j + u < NU)
            def _():
                unit_start(9 + 2 * j + u)

        k = 4 * j
        xa = b_fwd(k)
        xb = b_fwd(k + 1)
        b_inv(k, xa)
        xc = b_fwd(k + 2)
        b_inv(k + 1, xb)
        xd = b_fwd(k + 3)
        b_inv(k + 2, xc)
        b_inv(k + 3, xd)
        return carry

    jax.lax.fori_loop(0, 4, stage_b2, 0)

    def a_inv_tile(hi, t, u_dst):
        sl = slice(t * 128, (t + 1) * 128)
        w = np.exp(2j * np.pi / 16.0)
        tmp = bt_scr.at[t % 2]
        for b in range(4):
            xin = []
            for a in range(4):
                k2 = 4 * a + b
                gr, gi = z1[0, k2, hi, :, sl], z1[1, k2, hi, :, sl]
                xin.append((gr, gi))
            col = _dft4(xin, +1)
            for c in range(4):
                v = col[c] if b * c == 0 else _cmul_const(col[c], w ** (b * c))
                tmp[0, b, c] = v[0]
                tmp[1, b, c] = v[1]
        for c in range(4):
            row = _dft4([(tmp[0, b, c], tmp[1, b, c]) for b in range(4)], +1)
            for d in range(4):
                s2 = c + 4 * d
                u_dst[s2, :, sl] = row[d][0]
                if t < 4:
                    u_dst[s2, :, 640 + t * 128:640 + (t + 1) * 128] = row[d][1]

    def stage_c2(m, carry):
        @pl.when(jnp.logical_and(m >= 2, m < 6))
        def _():
            cp_wo(2 * (m - 2)).start()
            cp_wo(2 * (m - 2) + 1).start()

        stage_c(2 * m, 2 * m + 1, u0, u1)
        stage_c(2 * m + 1, jnp.minimum(2 * m + 2, 15), u1, u0)
        return carry

    def stage_c(hi, nxt, u_src, u_dst):
        unit_repack(hi)
        precompute(hi)
        for t in range(5):
            a_inv_tile(nxt, t, u_dst)
        nyq = u_src[:, :, 512:513].reshape(128, 1)
        n = jnp.broadcast_to(nyq, (128, 128)) * sgn
        ue_r = u_src[:, :, 0:256].reshape(128, 256)
        uo_r = u_src[:, :, 256:512].reshape(128, 256)
        ue_i = u_src[:, :, 640:896].reshape(128, 256)
        uo_i = u_src[:, :, 896:1152].reshape(128, 256)
        for T in range(2):
            a0 = qdot_t(ue_r, C0, T) + n
            a1 = qdot_t(uo_r, C1, T)
            b0 = qdot_t(ue_i, S0, T)
            b1 = qdot_t(uo_i, S1F, T)
            if T == 0:
                b1 = jnp.where(lane0, 0.0, b1)
            p, q, pm, qm = a0 + a1, b0 + b1, a0 - a1, b0 - b1
            z2[0, :, hi, :, T * 128:(T + 1) * 128] = (p + q).reshape(16, 8, 128)
            z2[1, :, hi, :, T * 128:(T + 1) * 128] = (pm + qm).reshape(16, 8, 128)
            up_scr[T] = p - q
            up_scr[2 + T] = pm - qm
        s_e = jnp.sum((ue_r[:, :128] + ue_r[:, 128:]) * sgn_m, axis=1, keepdims=True) + nyq
        s_o = jnp.sum((uo_i[:, :128] + uo_i[:, 128:]) * sgn_m, axis=1, keepdims=True)
        z2[1, :, hi, :, 384:512] = rev(up_scr[0], up_scr[1]).reshape(16, 8, 128)
        z2[1, :, hi, :, 256:384] = rev(up_scr[1], s_e + s_o).reshape(16, 8, 128)
        z2[0, :, hi, :, 384:512] = rev(up_scr[2], up_scr[3]).reshape(16, 8, 128)
        z2[0, :, hi, :, 256:384] = rev(up_scr[3], s_e - s_o).reshape(16, 8, 128)

    for t in range(5):
        a_inv_tile(0, t, u0)
    jax.lax.fori_loop(0, 8, stage_c2, 0)

    scale = DH ** -0.5
    rows = jax.lax.broadcasted_iota(jnp.int32, (L, L), 0)
    cols = jax.lax.broadcasted_iota(jnp.int32, (L, L), 1)
    mask = (rows < M) | (rows >= cols)
    wo32 = wo_v.bitcast(u32)

    def qkv_head(h, hd, p0):
        out = []
        for j in range(3):
            if j == 0:
                new = jnp.dot(h[0], pltpu.bitcast(wqkv[3 * hd + j], bf16), preferred_element_type=f32)
                out.append(jnp.concatenate([new[:8], pre[hd, pl.ds(p0, 8), :], new[8:]], axis=0))
            else:
                out.append(jnp.dot(h[1], pltpu.bitcast(wqkv[3 * hd + j], bf16), preferred_element_type=f32))
        return tuple(out)

    def scores(qkv):
        return jax.lax.dot_general(qkv[0], qkv[1].astype(bf16), nt_dims, preferred_element_type=f32)

    def softmax(s):
        s = jnp.where(mask, s * scale, -1e9)
        m = jnp.max(s, axis=-1, keepdims=True)
        p = jnp.exp(s - m)
        l = jnp.sum(p, axis=-1, keepdims=True)
        return p / l

    def pv(p, qkv):
        return jnp.dot(p, qkv[2].astype(bf16), preferred_element_type=f32)

    def cp_out(seg0, nseg):
        r0 = pl.multiple_of(seg0 * SEG, SEG)
        return pltpu.make_async_copy(out_v.at[pl.ds(r0, nseg * SEG)], out_hbm.at[pl.ds(r0, nseg * SEG)], sem_out)

    def mix(seg):
        r0 = pl.multiple_of(seg * SEG, SEG)
        xs = x_v[pl.ds(r0, SEG), :].astype(f32)
        gate = jax.nn.sigmoid(jnp.sum(xs * gw_row[...], axis=-1, keepdims=True))
        s2 = seg // 4
        hi0 = (seg % 4) * 4
        b = jnp.concatenate([z2[0, s2, pl.ds(hi0, 4), :, 0:512].reshape(SEG, 512),
                             z2[1, s2, pl.ds(hi0, 4), :, 0:512].reshape(SEG, 512)], axis=1)
        res = gate * a_scr[...] + (1.0 - gate) * b
        out_v[pl.ds(r0, SEG), :] = res.astype(out_v.dtype)


    def wo_part(h0, h1, n, lhs):
        w = pltpu.bitcast(wo32[n, h0 * (DH // 2):h1 * (DH // 2), :], bf16)
        return jnp.dot(lhs, w, preferred_element_type=f32)

    def step(s, mem):
        r0 = pl.multiple_of(s * SEG, SEG)
        xs = x_v[pl.ds(r0, SEG), :].astype(f32)
        h = (jnp.concatenate([mem, xs[8:]], axis=0),
             jnp.concatenate([mem, xs], axis=0))
        p0 = pl.multiple_of(s * 8, 8)
        qkvs, sc, ps, oh = {}, {}, {}, {}

        def wo_a(n):
            wa_scr[:, n * 128:(n + 1) * 128] = wo_part(0, HA, n, oa)

        for i in range(QL):
            qkvs[i] = qkv_head(h, i, p0)
        sc[0] = scores(qkvs[0])
        sc[1] = scores(qkvs[1])
        ps[0] = softmax(sc.pop(0))
        mix(jnp.maximum(s - 1, 0))

        @pl.when(s == NSEG - 1)
        def _():
            cp_out(NSEG - 4, 3).start()

        for hd in range(H):
            if hd + QL < H:
                qkvs[hd + QL] = qkv_head(h, hd + QL, p0)
            for n in WO_SCHED.get((hd, 0), ()):
                wo_a(n)
            if hd + 2 < H:
                sc[hd + 2] = scores(qkvs[hd + 2])
            if hd + 1 < H:
                ps[hd + 1] = softmax(sc.pop(hd + 1))
            oh[hd] = pv(ps.pop(hd), qkvs.pop(hd))
            if hd == HA - 1:
                oa = jnp.concatenate([oh.pop(i) for i in range(HA)], axis=1)
            for n in WO_SCHED.get((hd, 1), ()):
                wo_a(n)
        ob = jnp.concatenate([oh.pop(i) for i in range(HA, H)], axis=1)
        out = wa_scr[...] + jnp.concatenate([wo_part(HA, H, n, ob) for n in range(8)], axis=1)
        a_scr[...] = out[M:]
        @pl.when(jnp.logical_and(s > 0, s % 4 == 1))
        def _():
            @pl.when(s > 1)
            def _():
                cp_out(s - 5, 4).start()

        return out[:M]

    for n in range(8):
        cp_wo(n).wait()
    a_scr[...] = jnp.zeros(a_scr.shape, f32)
    jax.lax.fori_loop(0, NSEG, step, mem_ref[...].astype(f32), unroll=UNROLL)
    mix(NSEG - 1)
    cp_out(NSEG - 1, 1).start()
    pltpu.make_async_copy(out_v.at[pl.ds(0, NSEG * SEG)], out_hbm.at[pl.ds(0, NSEG * SEG)], sem_out).wait()


@jax.jit
def _run(A_x, A_mem0, A_Wq, A_Wk, A_Wv, A_Wo, B_w_r, B_w_i, gate_w):
    any_spec = pl.BlockSpec(memory_space=pl.ANY)
    out = pl.pallas_call(
        _kernel,
        out_shape=jax.ShapeDtypeStruct((S_LEN, DM), A_x.dtype),
        in_specs=[any_spec] * 12,
        out_specs=any_spec,
        scratch_shapes=[
            pltpu.VMEM((M, DM), bf16),
            pltpu.VMEM((1, DM), bf16),
            pltpu.VMEM((1, DM), f32),
            pltpu.VMEM((2, 128, 128), f32),
            pltpu.VMEM((32, 128), f32),
            pltpu.VMEM((2, 128, 128), f32),
            pltpu.VMEM((S_LEN, DM), bf16),
            pltpu.VMEM((8, 128, 128), u32),
            pltpu.VMEM((DM // 2, S_LEN), bf16),
            pltpu.VMEM((DM // 2, S_LEN), bf16),
            pltpu.VMEM((1, S_LEN), bf16),
            pltpu.VMEM((1, S_LEN), bf16),
            pltpu.VMEM((2, 16, 16, 8, 640), f32),
            pltpu.VMEM((3 * H, DM // 2, DH), u32),
            pltpu.VMEM((8, H * DH, 128), bf16),
            pltpu.VMEM((2, 16, 16, 8, 640), f32),
            pltpu.VMEM((2, 16, 16, 8, 640), f32),
            pltpu.VMEM((16, 8, 1152), f32),
            pltpu.VMEM((16, 8, 1152), f32),
            pltpu.VMEM((2, 2, 4, 4, 8, 128), f32),
            pltpu.VMEM((4, 128, 128), f32),
            pltpu.VMEM((L, DM), f32),
            pltpu.VMEM((SEG, DM), f32),
            pltpu.VMEM((S_LEN, DM), bf16),
            pltpu.VMEM((NSEG * 8, DM), f32),
            pltpu.VMEM((H, NSEG * 8, DH), f32),
            pltpu.SemaphoreType.DMA((8,)),
            pltpu.SemaphoreType.DMA(()),
            pltpu.SemaphoreType.DMA((4,)),
            pltpu.SemaphoreType.DMA((6,)),
            pltpu.SemaphoreType.DMA((3 * H,)),
            pltpu.SemaphoreType.DMA((8,)),
            pltpu.SemaphoreType.DMA(()),
        ],
        compiler_params=pltpu.CompilerParams(vmem_limit_bytes=120 * 1024 * 1024),
    )(A_x.reshape(S_LEN, DM), A_mem0.reshape(M, DM),
      A_Wq.reshape(512, 64, DH), A_Wk.reshape(512, 64, DH), A_Wv.reshape(512, 64, DH),
      A_Wo.reshape(H * DH, DM), B_w_r.T, B_w_i.T, gate_w.reshape(1, DM),
      _CS, _SMALL, _TW)
    return out.reshape(A_x.shape)


def pallas_gated_mix__memory_aug_recurrent_mem_tr__spectral_gfnet__prompt_kernel(
    A_x, A_mem0, A_Wq, A_Wk, A_Wv, A_Wo, A_seg_len, B_x, B_w_r, B_w_i, gate_w,
):
    del B_x
    assert int(A_seg_len) == SEG and A_x.shape == (1, S_LEN, DM)
    return _run(A_x, A_mem0, A_Wq, A_Wk, A_Wv, A_Wo, B_w_r, B_w_i, gate_w)
```

```python
import numpy as np
import ml_dtypes

import jax
import jax.numpy as jnp
import jax.experimental.pallas as pl
import jax.experimental.pallas.tpu as pltpu

S_LEN, DM, H, DH, M, SEG = 2048, 1024, 32, 128, 8, 32
L = M + SEG
NSEG = S_LEN // SEG
f32 = jnp.float32
bf16 = jnp.bfloat16
u32 = jnp.uint32
UNROLL = 4
QL = 4
HA = 26
WO_SCHED = {(27, 1): (0,), (28, 0): (1,), (28, 1): (2,), (29, 0): (3,), (29, 1): (4,), (30, 1): (5, 6), (31, 1): (7,)}


def _bf16_np(a):
    return np.asarray(a, np.float32).astype(ml_dtypes.bfloat16)


def _pack_rows_u32(a):
    b = _bf16_np(a).view(np.uint16).astype(np.uint32)
    return b[0::2] | (b[1::2] << 16)


def _make_consts():
    q = np.arange(DM // 4)
    th = 2.0 * np.pi / DM
    a0 = th * ((2 * np.outer(q, q)) % DM)
    a1 = th * ((np.outer(q, 2 * q + 1)) % DM)
    s1f = -np.sin(a1)
    s1f[0, :] = -np.cos(np.pi * q)
    mperm = 16 * (q // 16) + ((q % 16) >> 1) + 8 * (q & 1)
    fwd = [np.cos(a0), np.cos(a1), -np.sin(a0), s1f]
    cs = np.stack([_pack_rows_u32(m[:, mperm]) for m in fwd])
    cs = np.ascontiguousarray(cs.reshape(4, 128, 2, 128).transpose(0, 2, 1, 3)).reshape(8, 128, 128)

    i16 = np.arange(16)
    i128 = np.arange(128)
    d128 = np.exp(-2j * np.pi * ((np.outer(i128, i128)) % 128) / 128.0)
    small = np.stack([d128.real, d128.imag]).astype(np.float32)
    tw_f = np.exp(-2j * np.pi * np.outer(i16, i128) / 2048.0)
    tw = np.concatenate([tw_f.real, tw_f.imag]).astype(np.float32)
    return cs, small, tw


_CS, _SMALL, _TW = _make_consts()
NU = 16


def _lo_pair(a, b):
    return (a & np.uint32(0xFFFF)) | (b << 16)


def _hi_pair(a, b):
    return (a >> 16) | (b & np.uint32(0xFFFF0000))


def _is0(a):
    return isinstance(a, int) and a == 0


def _neg(a):
    return 0 if _is0(a) else -a


def _add(a, b):
    return b if _is0(a) else a if _is0(b) else a + b


def _sub(a, b):
    return _neg(b) if _is0(a) else a if _is0(b) else a - b


def _mul(a, c):
    return 0 if _is0(a) else a * c


def _cmul_const(x, c):
    re, im = x
    cr, ci = float(np.real(c)), float(np.imag(c))
    if abs(ci) < 1e-9:
        return (re, im) if cr > 0 else (_neg(re), _neg(im))
    if abs(cr) < 1e-9:
        return (_neg(im), re) if ci > 0 else (im, _neg(re))
    if abs(abs(cr) - abs(ci)) < 1e-9:
        a = abs(cr)
        if cr > 0:
            nr, ni = (_sub(re, im), _add(re, im)) if ci > 0 else (_add(re, im), _sub(im, re))
            return (_mul(nr, a), _mul(ni, a))
        nr, ni = (_add(re, im), _sub(im, re)) if ci > 0 else (_sub(im, re), _add(re, im))
        return (_mul(nr, -a), _mul(ni, -a)) if ci > 0 else (_mul(nr, a), _mul(ni, -a))
    return (_sub(_mul(re, cr), _mul(im, ci)), _add(_mul(re, ci), _mul(im, cr)))


def _dft4(x, sign):
    (ar, ai), (br, bi), (cr, ci), (dr, di) = x
    s0r, s0i = _add(ar, cr), _add(ai, ci)
    s1r, s1i = _sub(ar, cr), _sub(ai, ci)
    s2r, s2i = _add(br, dr), _add(bi, di)
    s3r, s3i = _sub(br, dr), _sub(bi, di)
    even, odd = (_add(s0r, s2r), _add(s0i, s2i)), (_sub(s0r, s2r), _sub(s0i, s2i))
    if sign < 0:
        return [even, (_add(s1r, s3i), _sub(s1i, s3r)), odd, (_sub(s1r, s3i), _add(s1i, s3r))]
    return [even, (_sub(s1r, s3i), _add(s1i, s3r)), odd, (_add(s1r, s3i), _sub(s1i, s3r))]


def _dft16(x, sign):
    w = np.exp(sign * 2j * np.pi / 16.0)
    t = [[None] * 4 for _ in range(4)]
    for b in range(4):
        col = _dft4([x[4 * a + b] for a in range(4)], sign)
        for c in range(4):
            t[b][c] = col[c] if b * c == 0 else _cmul_const(col[c], w ** (b * c))
    out = [None] * 16
    for c in range(4):
        row = _dft4([t[b][c] for b in range(4)], sign)
        for d in range(4):
            out[c + 4 * d] = row[d]
    return out


def _kernel(x_hbm, mem_hbm, wq_hbm, wk_hbm, wv_hbm, wo_hbm, wr_hbm, wi_hbm, gw_hbm,
            cs_hbm, small_hbm, tw_hbm,
            out_hbm,
            mem_ref, gw_ref, gw_row, small_ref, tw_ref, perm_ref,
            x_v, cs_v, wrt_v, wit_v, wrn_v, win_v, wp_v, wqkv, wo_v, z1, z2, u0, u1, bt_scr, up_scr, wa_scr, a_scr, out_v, xpre, pre,
            sem_x, sem_c, sem_s, sem_in, sem_w, sem_wo, sem_out):
    w32_hbm = tuple(w.bitcast(u32) for w in (wq_hbm, wk_hbm, wv_hbm))
    nt_dims = (((1,), (1,)), ((), ()))

    def cp_x(i):
        r0 = pl.multiple_of(i * 256, 256)
        return pltpu.make_async_copy(x_hbm.at[pl.ds(r0, 256)], x_v.at[pl.ds(r0, 256)], sem_x.at[i])

    cp_cs = pltpu.make_async_copy(cs_hbm, cs_v, sem_c)
    cp_wt, cp_wt2 = [], []
    for i, (src, dst, dstn) in enumerate(((wr_hbm, wrt_v, wrn_v), (wi_hbm, wit_v, win_v))):
        cp_wt.append(pltpu.make_async_copy(src.at[pl.ds(0, 512), pl.ds(0, 1024)], dst.at[:, pl.ds(0, 1024)], sem_in.at[3 * i]))
        cp_wt.append(pltpu.make_async_copy(src.at[pl.ds(512, 1)], dstn, sem_in.at[3 * i + 1]))
        cp_wt2.append(pltpu.make_async_copy(src.at[pl.ds(0, 512), pl.ds(1024, 1024)], dst.at[:, pl.ds(1024, 1024)], sem_in.at[3 * i + 2]))

    def cp_wo(n):
        return pltpu.make_async_copy(wo_hbm.at[:, pl.ds(n * 128, 128)], wo_v.at[n], sem_wo.at[n])

    def cp_w(p, par, which):
        t = 2 * p + par
        return pltpu.make_async_copy(w32_hbm[which].at[:, par * 16 + p], wqkv.at[3 * t + which],
                                     sem_w.at[3 * t + which])

    def unit_start(p):
        for par in range(2):
            for which in range(3):
                cp_w(p, par, which).start()

    def unit_repack(p):
        for par in range(2):
            for which in range(3):
                cp_w(p, par, which).wait()
        for which in range(3):
            ta = 6 * p + which
            tb = 6 * p + 3 + which
            for r in range(0, 512, 64):
                a = wqkv[ta, r:r + 64, :]
                b = wqkv[tb, r:r + 64, :]
                wqkv[ta, r:r + 64, :] = _lo_pair(a, b)
                wqkv[tb, r:r + 64, :] = _hi_pair(a, b)

    C0, C1, S0, S1F = range(4)

    def qdot(lhs, mat, nt):
        return jnp.dot(lhs, pltpu.bitcast(cs_v[2 * mat + nt], bf16), preferred_element_type=f32)

    def qdot_t(lhs, mat, dt):
        rows = jnp.concatenate([cs_v[2 * mat + kt, dt * 64:(dt + 1) * 64, :] for kt in range(2)], axis=1)
        return jax.lax.dot_general(lhs, pltpu.bitcast(rows, bf16), nt_dims, preferred_element_type=f32)

    def rev(t, first):
        return jnp.where(lane0, first, jnp.dot(t, perm_ref[1], preferred_element_type=f32))

    cp_small = [pltpu.make_async_copy(src, dst, sem_s.at[i]) for i, (src, dst) in enumerate((
        (small_hbm, small_ref), (tw_hbm, tw_ref),
        (mem_hbm, mem_ref), (gw_hbm, gw_ref)))]
    cp_cs.start()
    cp_x(0).start()
    cp_x(1).start()
    for cp in cp_small:
        cp.start()
    ri = jax.lax.broadcasted_iota(jnp.int32, (128, 128), 0)
    ci = jax.lax.broadcasted_iota(jnp.int32, (128, 128), 1)
    perm_ref[0] = (ci == (ri >> 3) + 16 * (ri & 7)).astype(f32) * (2.0 / (S_LEN * DM))
    perm_ref[1] = ((ri + ci == 128) & (ci >= 1)).astype(f32)

    lane_i = jax.lax.broadcasted_iota(jnp.int32, (1, 128), 1)
    lane0 = lane_i == 0
    sgn = (1 - 2 * (lane_i & 1)).astype(f32)
    half0 = jnp.where(lane0, 0.5, 1.0).astype(f32)
    sgn_m = (1 - 2 * ((lane_i >> 1) & 1)).astype(f32)

    def pro1(c, carry):
        @pl.when(c < 3)
        def _():
            cp_x(2 * c + 2).start()
            cp_x(2 * c + 3).start()

        @pl.when(c == 2)
        def _():
            for cp in cp_wt:
                cp.start()

        @pl.when(c == 4)
        def _():
            for cp in cp_wt2:
                cp.start()

        @pl.when(c >= 4)
        def _():
            unit_start(c - 4)

        cp_x(c).wait()
        r0 = pl.multiple_of(c * 256, 256)
        xt = [x_v[pl.ds(r0, 256), j * 128:(j + 1) * 128].astype(f32) for j in range(8)]
        for j in range(8):
            xpre[pl.ds(pl.multiple_of(c * 64, 64), 64), j * 128:(j + 1) * 128] = (
                xt[j].reshape(8, 32, 128)[:, :8, :].reshape(64, 128))
        zero = jnp.zeros((256, 128), f32)
        r1 = [rev(xt[7], zero), rev(xt[6], xt[7])]
        r2 = [rev(xt[3], zero), rev(xt[2], xt[3])]
        ee, eo, oe, oo = [], [], [], []
        for T in range(2):
            e1, o1 = xt[T] + r1[T], xt[T] - r1[T]
            e2, o2 = r2[T] + xt[4 + T], r2[T] - xt[4 + T]
            ee.append(e1 + e2)
            eo.append(e1 - e2)
            oe.append(o1 - o2)
            oo.append(o1 + o2)
        oo[0] = jnp.where(lane0, xt[2] - xt[6], oo[0])
        e256 = (xt[2] + xt[6])[:, 0:1]
        mid = jnp.broadcast_to(e256, (256, 128)) * sgn_m
        nyq = jnp.sum((ee[0] + ee[1]) * sgn, axis=1, keepdims=True) + e256
        ee, eo, oe, oo = (jnp.concatenate(v, axis=1) for v in (ee, eo, oe, oo))
        rr = pl.ds(2 * c, 2)
        for t in range(2):
            y0 = qdot(ee, C0, t) + mid
            if t == 0:
                y0 = y0 * half0
            z1[0, rr, :, :, t * 128:(t + 1) * 128] = y0.reshape(2, 16, 8, 128)
            z1[0, rr, :, :, (2 + t) * 128:(3 + t) * 128] = qdot(eo, C1, t).reshape(2, 16, 8, 128)
            z1[1, rr, :, :, t * 128:(t + 1) * 128] = qdot(oe, S0, t).reshape(2, 16, 8, 128)
            z1[1, rr, :, :, (2 + t) * 128:(3 + t) * 128] = qdot(oo, S1F, t).reshape(2, 16, 8, 128)
        z1[0, rr, :, :, 512:640] = jnp.where(lane0, 0.5 * nyq, 0.0).reshape(2, 16, 8, 128)
        return carry

    cp_cs.wait()
    jax.lax.fori_loop(0, 8, pro1, 0)

    def stage_a(hi):
        for t in range(5):
            sl = slice(t * 128, (t + 1) * 128)
            xin = [(z1[0, s2, hi, :, sl], z1[1, s2, hi, :, sl] if t < 4 else 0) for s2 in range(16)]
            xo = _dft16(xin, -1)
            for k2 in range(16):
                z2[0, k2, hi, :, sl] = xo[k2][0]
                z2[1, k2, hi, :, sl] = jnp.zeros((8, 128), f32) if _is0(xo[k2][1]) else xo[k2][1]


    def wperm(c, carry):
        @pl.when(c < 5)
        def _():
            unit_start(4 + c)

        @pl.when(c == 4)
        def _():
            for cp in cp_wt2:
                cp.wait()

        for bb in range(2):
            blk_i = 2 * c + bb
            l0 = pl.multiple_of(blk_i * 128, 128)
            for i, (wt, wn) in enumerate(((wrt_v.bitcast(u32), wrn_v), (wit_v.bitcast(u32), win_v))):
                blks = []
                for t in range(5):
                    if t < 4:
                        w = wt[(t % 2) * 128:(t % 2 + 1) * 128, pl.ds(l0, 128)].reshape(8, 16, 128)
                        pk = (_lo_pair if t < 2 else _hi_pair)(w[:, :8, :], w[:, 8:, :])
                        blks.append(pltpu.bitcast(pk.reshape(64, 128), bf16))
                    else:
                        blks.append(jnp.broadcast_to(wn[:, pl.ds(l0, 128)], (128, 128)))
                o = jax.lax.dot_general(perm_ref[0], jnp.concatenate(blks, axis=0), nt_dims,
                                        preferred_element_type=f32)
                wp_v[i, :, blk_i] = o.reshape(16, 8, 640)
            stage_a(blk_i)
        return carry

    def precompute(p):
        for hd in (2 * p, 2 * p + 1):
            pre[hd] = jnp.dot(xpre[...], pltpu.bitcast(wqkv[3 * hd], bf16), preferred_element_type=f32)

    for cp in cp_small:
        cp.wait()
    gw_row[...] = gw_ref[...].astype(f32)

    for cp in cp_wt:
        cp.wait()
    jax.lax.fori_loop(0, 8, wperm, 0)

    def cdot3(m1, m2, m3, zr, zi, dims=(((1,), (0,)), ((), ()))):
        k1 = jax.lax.dot_general(m1, (zr + zi).astype(bf16), dims, preferred_element_type=f32)
        k2 = jax.lax.dot_general(m2, zi.astype(bf16), dims, preferred_element_type=f32)
        k3 = jax.lax.dot_general(m3, zr.astype(bf16), dims, preferred_element_type=f32)
        return k1 - k2, k1 + k3

    def b_fwd(k2):
        tr, ti = tw_ref[pl.ds(k2, 1), :], tw_ref[pl.ds(16 + k2, 1), :]
        mr = small_ref[0] * tr - small_ref[1] * ti
        mi = small_ref[0] * ti + small_ref[1] * tr
        m2, m3 = mr + mi, mi - mr
        return cdot3(mr, m2, m3, z2[0, k2].reshape(128, 640), z2[1, k2].reshape(128, 640)), (mr, m2, m3)

    def b_inv(k2, x):
        (xr, xi), (mr, m2, m3) = x
        wr = wp_v[0, k2].reshape(128, 640)
        wi = wp_v[1, k2].reshape(128, 640)
        pr = xr * wr - xi * wi
        pi = xr * wi + xi * wr
        tn = (((0,), (0,)), ((), ()))
        k1 = jax.lax.dot_general(mr, (pr + pi).astype(bf16), tn, preferred_element_type=f32)
        k2_ = jax.lax.dot_general(m3, pi.astype(bf16), tn, preferred_element_type=f32)
        k3 = jax.lax.dot_general(m2, pr.astype(bf16), tn, preferred_element_type=f32)
        gr, gi = k1 + k2_, k1 - k3
        z1[0, k2] = gr.reshape(16, 8, 640)
        z1[1, k2] = gi.reshape(16, 8, 640)

    def stage_b2(j, carry):
        for u in range(2):
            @pl.when(9 + 2 * j + u < NU)
            def _():
                unit_start(9 + 2 * j + u)

        k = 4 * j
        xa = b_fwd(k)
        xb = b_fwd(k + 1)
        b_inv(k, xa)
        xc = b_fwd(k + 2)
        b_inv(k + 1, xb)
        xd = b_fwd(k + 3)
        b_inv(k + 2, xc)
        b_inv(k + 3, xd)
        return carry

    jax.lax.fori_loop(0, 4, stage_b2, 0)

    def a_inv_tile(hi, t, u_dst):
        sl = slice(t * 128, (t + 1) * 128)
        w = np.exp(2j * np.pi / 16.0)
        tmp = bt_scr.at[t % 2]
        for b in range(4):
            xin = []
            for a in range(4):
                k2 = 4 * a + b
                gr, gi = z1[0, k2, hi, :, sl], z1[1, k2, hi, :, sl]
                xin.append((gr, gi))
            col = _dft4(xin, +1)
            for c in range(4):
                v = col[c] if b * c == 0 else _cmul_const(col[c], w ** (b * c))
                tmp[0, b, c] = v[0]
                tmp[1, b, c] = v[1]
        for c in range(4):
            row = _dft4([(tmp[0, b, c], tmp[1, b, c]) for b in range(4)], +1)
            for d in range(4):
                s2 = c + 4 * d
                u_dst[s2, :, sl] = row[d][0]
                if t < 4:
                    u_dst[s2, :, 640 + t * 128:640 + (t + 1) * 128] = row[d][1]

    def stage_c2(m, carry):
        @pl.when(jnp.logical_and(m >= 2, m < 6))
        def _():
            cp_wo(2 * (m - 2)).start()
            cp_wo(2 * (m - 2) + 1).start()

        stage_c(2 * m, 2 * m + 1, u0, u1)
        stage_c(2 * m + 1, jnp.minimum(2 * m + 2, 15), u1, u0)
        return carry

    def stage_c(hi, nxt, u_src, u_dst):
        unit_repack(hi)
        precompute(hi)
        for t in range(5):
            a_inv_tile(nxt, t, u_dst)
        nyq = u_src[:, :, 512:513].reshape(128, 1)
        n = jnp.broadcast_to(nyq, (128, 128)) * sgn
        ue_r = u_src[:, :, 0:256].reshape(128, 256)
        uo_r = u_src[:, :, 256:512].reshape(128, 256)
        ue_i = u_src[:, :, 640:896].reshape(128, 256)
        uo_i = u_src[:, :, 896:1152].reshape(128, 256)
        for T in range(2):
            a0 = qdot_t(ue_r, C0, T) + n
            a1 = qdot_t(uo_r, C1, T)
            b0 = qdot_t(ue_i, S0, T)
            b1 = qdot_t(uo_i, S1F, T)
            if T == 0:
                b1 = jnp.where(lane0, 0.0, b1)
            p, q, pm, qm = a0 + a1, b0 + b1, a0 - a1, b0 - b1
            z2[0, :, hi, :, T * 128:(T + 1) * 128] = (p + q).reshape(16, 8, 128)
            z2[1, :, hi, :, T * 128:(T + 1) * 128] = (pm + qm).reshape(16, 8, 128)
            up_scr[T] = p - q
            up_scr[2 + T] = pm - qm
        s_e = jnp.sum((ue_r[:, :128] + ue_r[:, 128:]) * sgn_m, axis=1, keepdims=True) + nyq
        s_o = jnp.sum((uo_i[:, :128] + uo_i[:, 128:]) * sgn_m, axis=1, keepdims=True)
        z2[1, :, hi, :, 384:512] = rev(up_scr[0], up_scr[1]).reshape(16, 8, 128)
        z2[1, :, hi, :, 256:384] = rev(up_scr[1], s_e + s_o).reshape(16, 8, 128)
        z2[0, :, hi, :, 384:512] = rev(up_scr[2], up_scr[3]).reshape(16, 8, 128)
        z2[0, :, hi, :, 256:384] = rev(up_scr[3], s_e - s_o).reshape(16, 8, 128)

    for t in range(5):
        a_inv_tile(0, t, u0)
    jax.lax.fori_loop(0, 8, stage_c2, 0)

    scale = DH ** -0.5
    rows = jax.lax.broadcasted_iota(jnp.int32, (L, L), 0)
    cols = jax.lax.broadcasted_iota(jnp.int32, (L, L), 1)
    mask = (rows < M) | (rows >= cols)
    wo32 = wo_v.bitcast(u32)

    def qkv_head(h, hd, p0):
        out = []
        for j in range(3):
            if j == 0:
                new = jnp.dot(h[0], pltpu.bitcast(wqkv[3 * hd + j], bf16), preferred_element_type=f32)
                out.append(jnp.concatenate([new[:8], pre[hd, pl.ds(p0, 8), :], new[8:]], axis=0))
            else:
                out.append(jnp.dot(h[1], pltpu.bitcast(wqkv[3 * hd + j], bf16), preferred_element_type=f32))
        return tuple(out)

    def scores(qkv):
        return jax.lax.dot_general(qkv[0], qkv[1].astype(bf16), nt_dims, preferred_element_type=f32)

    def softmax(s):
        s = jnp.where(mask, s * scale, -1e9)
        m = jnp.max(s, axis=-1, keepdims=True)
        p = jnp.exp(s - m)
        l = jnp.sum(p, axis=-1, keepdims=True)
        return p / l

    def pv(p, qkv):
        return jnp.dot(p, qkv[2].astype(bf16), preferred_element_type=f32)

    def cp_out(seg0, nseg):
        r0 = pl.multiple_of(seg0 * SEG, SEG)
        return pltpu.make_async_copy(out_v.at[pl.ds(r0, nseg * SEG)], out_hbm.at[pl.ds(r0, nseg * SEG)], sem_out)

    def mix(seg):
        r0 = pl.multiple_of(seg * SEG, SEG)
        xs = x_v[pl.ds(r0, SEG), :].astype(f32)
        gate = jax.nn.sigmoid(jnp.sum(xs * gw_row[...], axis=-1, keepdims=True))
        s2 = seg // 4
        hi0 = (seg % 4) * 4
        b = jnp.concatenate([z2[0, s2, pl.ds(hi0, 4), :, 0:512].reshape(SEG, 512),
                             z2[1, s2, pl.ds(hi0, 4), :, 0:512].reshape(SEG, 512)], axis=1)
        res = gate * a_scr[...] + (1.0 - gate) * b
        out_v[pl.ds(r0, SEG), :] = res.astype(out_v.dtype)


    def wo_part(h0, h1, n, lhs):
        w = pltpu.bitcast(wo32[n, h0 * (DH // 2):h1 * (DH // 2), :], bf16)
        return jnp.dot(lhs, w, preferred_element_type=f32)

    def step(s, mem):
        r0 = pl.multiple_of(s * SEG, SEG)
        xs = x_v[pl.ds(r0, SEG), :].astype(f32)
        h = (jnp.concatenate([mem, xs[8:]], axis=0),
             jnp.concatenate([mem, xs], axis=0))
        p0 = pl.multiple_of(s * 8, 8)
        qkvs, sc, ps, oh = {}, {}, {}, {}

        def wo_a(n):
            wa_scr[:, n * 128:(n + 1) * 128] = wo_part(0, HA, n, oa)

        for i in range(QL):
            qkvs[i] = qkv_head(h, i, p0)
        sc[0] = scores(qkvs[0])
        sc[1] = scores(qkvs[1])
        ps[0] = softmax(sc.pop(0))
        mix(jnp.maximum(s - 1, 0))

        @pl.when(s == NSEG - 1)
        def _():
            cp_out(NSEG - 4, 3).start()

        for hd in range(H):
            if hd + QL < H:
                qkvs[hd + QL] = qkv_head(h, hd + QL, p0)
            for n in WO_SCHED.get((hd, 0), ()):
                wo_a(n)
            if hd + 2 < H:
                sc[hd + 2] = scores(qkvs[hd + 2])
            if hd + 1 < H:
                ps[hd + 1] = softmax(sc.pop(hd + 1))
            oh[hd] = pv(ps.pop(hd), qkvs.pop(hd))
            if hd == HA - 1:
                oa = jnp.concatenate([oh.pop(i) for i in range(HA)], axis=1)
            for n in WO_SCHED.get((hd, 1), ()):
                wo_a(n)
        ob = jnp.concatenate([oh.pop(i) for i in range(HA, H)], axis=1)
        out = wa_scr[...] + jnp.concatenate([wo_part(HA, H, n, ob) for n in range(8)], axis=1)
        a_scr[...] = out[M:]
        @pl.when(jnp.logical_and(s > 0, s % 4 == 1))
        def _():
            @pl.when(s > 1)
            def _():
                cp_out(s - 5, 4).start()

        return out[:M]

    for n in range(8):
        cp_wo(n).wait()
    a_scr[...] = jnp.zeros(a_scr.shape, f32)
    jax.lax.fori_loop(0, NSEG, step, mem_ref[...].astype(f32), unroll=UNROLL)
    mix(NSEG - 1)
    cp_out(NSEG - 1, 1).start()
    pltpu.make_async_copy(out_v.at[pl.ds(0, NSEG * SEG)], out_hbm.at[pl.ds(0, NSEG * SEG)], sem_out).wait()


@jax.jit
def _run(A_x, A_mem0, A_Wq, A_Wk, A_Wv, A_Wo, B_w_r, B_w_i, gate_w):
    any_spec = pl.BlockSpec(memory_space=pl.ANY)
    out = pl.pallas_call(
        _kernel,
        out_shape=jax.ShapeDtypeStruct((S_LEN, DM), A_x.dtype),
        in_specs=[any_spec] * 12,
        out_specs=any_spec,
        scratch_shapes=[
            pltpu.VMEM((M, DM), bf16),
            pltpu.VMEM((1, DM), bf16),
            pltpu.VMEM((1, DM), f32),
            pltpu.VMEM((2, 128, 128), f32),
            pltpu.VMEM((32, 128), f32),
            pltpu.VMEM((2, 128, 128), f32),
            pltpu.VMEM((S_LEN, DM), bf16),
            pltpu.VMEM((8, 128, 128), u32),
            pltpu.VMEM((DM // 2, S_LEN), bf16),
            pltpu.VMEM((DM // 2, S_LEN), bf16),
            pltpu.VMEM((1, S_LEN), bf16),
            pltpu.VMEM((1, S_LEN), bf16),
            pltpu.VMEM((2, 16, 16, 8, 640), f32),
            pltpu.VMEM((3 * H, DM // 2, DH), u32),
            pltpu.VMEM((8, H * DH, 128), bf16),
            pltpu.VMEM((2, 16, 16, 8, 640), f32),
            pltpu.VMEM((2, 16, 16, 8, 640), f32),
            pltpu.VMEM((16, 8, 1152), f32),
            pltpu.VMEM((16, 8, 1152), f32),
            pltpu.VMEM((2, 2, 4, 4, 8, 128), f32),
            pltpu.VMEM((4, 128, 128), f32),
            pltpu.VMEM((L, DM), f32),
            pltpu.VMEM((SEG, DM), f32),
            pltpu.VMEM((S_LEN, DM), bf16),
            pltpu.VMEM((NSEG * 8, DM), f32),
            pltpu.VMEM((H, NSEG * 8, DH), f32),
            pltpu.SemaphoreType.DMA((8,)),
            pltpu.SemaphoreType.DMA(()),
            pltpu.SemaphoreType.DMA((4,)),
            pltpu.SemaphoreType.DMA((6,)),
            pltpu.SemaphoreType.DMA((3 * H,)),
            pltpu.SemaphoreType.DMA((8,)),
            pltpu.SemaphoreType.DMA(()),
        ],
        compiler_params=pltpu.CompilerParams(vmem_limit_bytes=120 * 1024 * 1024),
    )(A_x.reshape(S_LEN, DM), A_mem0.reshape(M, DM),
      A_Wq.reshape(512, 64, DH), A_Wk.reshape(512, 64, DH), A_Wv.reshape(512, 64, DH),
      A_Wo.reshape(H * DH, DM), B_w_r.T, B_w_i.T, gate_w.reshape(1, DM),
      _CS, _SMALL, _TW)
    return out.reshape(A_x.shape)


def pallas_gated_mix__memory_aug_recurrent_mem_tr__spectral_gfnet__prompt_kernel(
    A_x, A_mem0, A_Wq, A_Wk, A_Wv, A_Wo, A_seg_len, B_x, B_w_r, B_w_i, gate_w,
):
    del B_x
    assert int(A_seg_len) == SEG and A_x.shape == (1, S_LEN, DM)
    return _run(A_x, A_mem0, A_Wq, A_Wk, A_Wv, A_Wo, B_w_r, B_w_i, gate_w)
```
